```python
import os as _os
_os.environ.setdefault('JAX_PLATFORMS', 'cpu')
import jax
import jax.numpy as jnp

def _softmax(x, axis=-1):
    return jax.nn.softmax(x, axis=axis)

def _gelu(x):
    return jax.nn.gelu(x, approximate=True)

def _silu(x):
    return jax.nn.silu(x)

def _sigmoid(x):
    return jax.nn.sigmoid(x)

def _layernorm(x, axis=-1, eps=1e-05):
    m = jnp.mean(x, axis=axis, keepdims=True)
    v = jnp.var(x, axis=axis, keepdims=True)
    return (x - m) / jnp.sqrt(v + eps)

def _scatter_add(tgt, idx, src, axis=0):
    return tgt.at[idx].add(src)

def _segment_sum(src, seg, n):
    return jax.ops.segment_sum(src, seg, n)

class _Rng:

    def __init__(self, key):
        self._k = key

    def _next(self):
        self._k, sub = jax.random.split(self._k)
        return sub

    def normal(self, shape):
        return jax.random.normal(self._next(), shape, dtype=jnp.bfloat16)

    def randint(self, lo, hi, shape):
        return jax.random.randint(self._next(), shape, lo, hi, dtype=jnp.int32)

    def uniform(self, shape, lo=0.0, hi=1.0):
        return jax.random.uniform(self._next(), shape, jnp.bfloat16, lo, hi)

    def permutation(self, n):
        return jax.random.permutation(self._next(), n)
kernel_name = 'concat_heads__spectral_gfnet__memory_aug_recurrent_mem_tr__prompt'

def setup_inputs():
    _rng = _Rng(jax.random.key(int.from_bytes(__import__("os").urandom(4), "little")))
    _w = lambda a: (lambda t: t.astype(jnp.bfloat16) if jnp.issubdtype(t.dtype, jnp.floating) else t)(jnp.asarray(a))

    def _A_setup():
        B, S, D = (1, 2048, 512)
        Df = D // 2 + 1
        return {'x': _w((lambda *s: _rng.normal(s) * 0.05)(B, S, D)), 'w_r': _w((lambda *s: _rng.normal(s) * 0.05)(S, Df) * 0.02), 'w_i': _w((lambda *s: _rng.normal(s) * 0.05)(S, Df) * 0.02)}
    _A_in = _A_setup()

    def _B_setup():
        B, S, Dm = (1, 2048, 512)
        H, Dh = (32, 128)
        M, seg = (8, 32)
        seg = min(seg, S)
        S = S // seg * seg
        return {'x': _w((lambda *s: _rng.normal(s) * 0.05)(B, S, Dm)), 'mem0': _w((lambda *s: _rng.normal(s) * 0.4)(B, M, Dm)), 'Wq': _w((lambda *s: _rng.normal(s) * 3.2)(Dm, H, Dh) * Dm ** (-0.5)), 'Wk': _w((lambda *s: _rng.normal(s) * 3.2)(Dm, H, Dh) * Dm ** (-0.5)), 'Wv': _w((lambda *s: _rng.normal(s) * 0.4)(Dm, H, Dh) * Dm ** (-0.5)), 'Wo': _w((lambda *s: _rng.normal(s) * 0.4)(H, Dh, Dm) * (H * Dh) ** (-0.5)), 'seg_len': seg}
    _B_in = _B_setup()
    return {'A_x': _A_in['x'], 'A_w_r': _A_in['w_r'], 'A_w_i': _A_in['w_i'], 'B_x': _B_in['x'], 'B_mem0': _B_in['mem0'], 'B_Wq': _B_in['Wq'], 'B_Wk': _B_in['Wk'], 'B_Wv': _B_in['Wv'], 'B_Wo': _B_in['Wo'], 'B_seg_len': _B_in['seg_len']}

def reference(A_x, A_w_r, A_w_i, B_x, B_mem0, B_Wq, B_Wk, B_Wv, B_Wo, B_seg_len):

    def _A_ref(x, w_r, w_i):
        B, S, D = x.shape
        X = (lambda x, axes=(-2, -1): jnp.fft.rfft2(x.astype(jnp.float32), axes=axes))(x, axes=(-2, -1))
        W = w_r + 1j * w_i
        X = X * W
        y = (lambda x, s, axes=(-2, -1): jnp.fft.irfft2(x, s=s, axes=axes).astype(jnp.bfloat16))(X, (S, D), axes=(-2, -1))
        return y

    def _B_ref(x, mem0, Wq, Wk, Wv, Wo, seg_len):
        B, S, Dm = x.shape
        H, Dh = (Wq.shape[1], Wq.shape[2])
        M = mem0.shape[1]
        scale = Dh ** (-0.5)
        n_seg = S // seg_len
        L = M + seg_len
        idx = jnp.arange(L)
        mask = (idx[:, None] < M) | (idx[:, None] >= idx[None, :])
        mem = mem0
        outs = []
        for s in range(n_seg):
            xs = x[:, s * seg_len:(s + 1) * seg_len, :].copy()
            h = jnp.concatenate([mem, xs], axis=1)
            q = jnp.einsum('btd,dhe->bhte', h, Wq)
            k = jnp.einsum('btd,dhe->bhte', h, Wk)
            v = jnp.einsum('btd,dhe->bhte', h, Wv)
            scores = jnp.einsum('bhqe,bhke->bhqk', q, k) * scale
            scores = jnp.where(mask[None, None], scores, -1000000000.0)
            p = _softmax(scores, axis=-1)
            o = jnp.einsum('bhqk,bhke->bhqe', p, v)
            o = jnp.einsum('bhte,hed->btd', o, Wo)
            mem = o[:, :M, :].copy()
            outs.append(o[:, M:, :])
        return jnp.concatenate(outs, axis=1)
    a = _A_ref(A_x, A_w_r, A_w_i)
    b = _B_ref(B_x, B_mem0, B_Wq, B_Wk, B_Wv, B_Wo, B_seg_len)
    return jnp.concatenate([a, b], axis=-1)
```

```python
import jax
import jax.numpy as jnp
import ml_dtypes
import numpy as np
from jax import lax
import jax.experimental.pallas as pl
import jax.experimental.pallas.tpu as pltpu

S, D, H, E, M, SEG = 2048, 512, 32, 128, 8, 32
L = M + SEG
f32, bf16, u32 = jnp.float32, jnp.bfloat16, jnp.uint32
NN = (((1,), (0,)), ((), ()))
NT = (((1,), (1,)), ((), ()))


def _dot(a, b, dims=NN):
    return lax.dot_general(a, b, dims, preferred_element_type=f32)


def _lo(u):
    return pltpu.bitcast(u << 16, f32)


def _hi(u):
    return pltpu.bitcast(u & np.uint32(0xFFFF0000), f32)


SU = {1: (((0, 0), 1), ((1, 1), 1)), 2: (((1, 0), 1), ((1, 1), 1)), 3: (((0, 0), 1),), 4: (((1, 1), 1),),
      5: (((0, 0), 1), ((0, 1), 1)), 6: (((1, 0), 1), ((0, 0), -1)), 7: (((0, 1), 1), ((1, 1), -1))}
SV = {1: (((0, 0), 1), ((1, 1), 1)), 2: (((0, 0), 1),), 3: (((0, 1), 1), ((1, 1), -1)),
      4: (((1, 0), 1), ((0, 0), -1)), 5: (((1, 1), 1),), 6: (((0, 0), 1), ((0, 1), 1)),
      7: (((1, 0), 1), ((1, 1), 1))}
SW = {(0, 0): ((1, 1), (4, 1), (7, 1), (5, -1)), (0, 1): ((3, 1), (5, 1)), (1, 0): ((2, 1), (4, 1)),
      (1, 1): ((1, 1), (3, 1), (6, 1), (2, -1))}
PHASE = ((1, 3, 5, 7), (1, 2, 4, 6))


def _lin(terms):
    terms = [(v, c) for v, c in terms if v is not None]
    if not terms:
        return None
    pos = [v for v, c in terms if c > 0]
    neg = [v for v, c in terms if c < 0]
    if pos:
        acc = pos[0]
        for v in pos[1:]:
            acc = acc + v
    else:
        acc, neg = -neg[0], neg[1:]
    for v in neg:
        acc = acc - v
    return acc


def _pre(blocks, level, table, want):
    if level == 0:
        return {(): blocks.get((0, 0))}
    h = 2 ** (level - 1)
    out = {}
    for r in sorted({w[0] for w in want}):
        sub = {(i, k): _lin([(blocks.get((a * h + i, b * h + k)), c) for (a, b), c in table[r]])
               for i in range(h) for k in range(h)}
        for rr, v in _pre(sub, level - 1, table, sorted(w[1:] for w in want if w[0] == r)).items():
            out[(r,) + rr] = v
    return out


def _post(prods, level, rows=None):
    if level == 0:
        return {(0, 0): prods[()]}
    h = 2 ** (level - 1)
    subrows = None if rows is None else [i % h for i in rows]
    inner = {r: _post({w[1:]: v for w, v in prods.items() if w[0] == r}, level - 1, subrows)
             for r in sorted({w[0] for w in prods})}
    out = {}
    for (a, b), terms in SW.items():
        for i in range(h):
            if rows is not None and a * h + i not in rows:
                continue
            for n in range(h):
                v = _lin([(inner.get(r, {}).get((i, n)), c) for r, c in terms])
                if v is not None:
                    out[(a * h + i, b * h + n)] = v
    return out


def _all_products(level):
    out = [()]
    for _ in range(level):
        out = [o + (r,) for o in out for r in range(1, 8)]
    return out


def _phase_products(level, p):
    out = [()]
    for l in range(level):
        out = [o + (r,) for o in out for r in PHASE[(p >> (level - 1 - l)) & 1]]
    return out


def _assign(level):
    G = 2 ** level
    rows = {p: {} for p in range(G)}
    for r in _all_products(level):
        cand = [p for p in range(G) if r in _phase_products(level, p)]
        n = SEG // len(cand)
        for j, p in enumerate(cand):
            rows[p][r] = (j * n, (j + 1) * n)
    out = {}
    for p in range(G):
        prods = _phase_products(level, p)
        lng = [r for r in prods if rows[p][r][1] - rows[p][r][0] == SEG]
        sht = [r for r in prods if rows[p][r][1] - rows[p][r][0] < SEG]
        order, k = [], 0
        for j in range(len(prods)):
            if sht and (j + 1) * len(sht) // len(prods) > k:
                order.append(sht[k])
                k += 1
            else:
                order.append(lng[j - k])
        out[p] = [(r,) + rows[p][r] for r in order]
    return out


def _contrib(level, asg):
    c = {}
    for p in range(2 ** level):
        for (r, a, b) in asg[p]:
            for rb in range(a // 8, b // 8):
                for key in _post({r: np.zeros(1)}, level):
                    lst = c.setdefault(key + (rb,), [])
                    if p not in lst:
                        lst.append(p)
    return c


def _dft_constants():
    n = np.arange(128)[None, :]
    m = np.arange(64)[:, None]
    th = lambda k: 2 * np.pi * ((k * n) % 512) / 512
    fa = np.concatenate([np.cos(th(4 * m)), -np.sin(th(4 * m))])
    fa[64] = np.cos(np.pi * n[0])
    fb = np.concatenate([np.cos(th(4 * m + 2)), -np.sin(th(4 * m + 2))])
    c1, s1, c3, s3 = np.cos(th(4 * m + 1)), np.sin(th(4 * m + 1)), np.cos(th(4 * m + 3)), np.sin(th(4 * m + 3))
    f0 = np.concatenate([c1, -s1, c3, -s3])
    f1 = np.concatenate([-s1, -c1, s3, c3])
    a = np.arange(128)
    ph = 2 * np.pi * ((a[:, None] * a[None, :]) % 128) / 128
    mats = np.concatenate([fa, fb, f0, f1, np.cos(ph), -np.sin(ph)]).astype(np.float32)
    u = mats.astype(ml_dtypes.bfloat16).view(np.uint16).astype(np.uint32)
    tp = 2 * np.pi * (np.arange(16)[:, None] * a[None, :]) / S
    tw = np.concatenate([np.cos(tp), -np.sin(tp)]).astype(np.float32)
    return u[0::2] | (u[1::2] << 16), tw


_DFT_MATS, _DFT_TW = _dft_constants()
GRP = (0, 128, 256, 384)


def _fft4(a, b, c, d, sg):
    t0 = (a[0] + c[0], a[1] + c[1])
    t1 = (a[0] - c[0], a[1] - c[1])
    t2 = (b[0] + d[0], b[1] + d[1])
    t3 = (b[0] - d[0], b[1] - d[1])
    y0 = (t0[0] + t2[0], t0[1] + t2[1])
    y2 = (t0[0] - t2[0], t0[1] - t2[1])
    p = (t1[0] + t3[1], t1[1] - t3[0])
    q = (t1[0] - t3[1], t1[1] + t3[0])
    return (y0, p, y2, q) if sg < 0 else (y0, q, y2, p)


def _tw16(z, e, sg):
    if e == 0:
        return z
    r, i = z
    if e == 4:
        return (i, -r) if sg < 0 else (-i, r)
    h = np.float32(np.sqrt(0.5))
    if e == 2:
        return ((r + i) * h, (i - r) * h) if sg < 0 else ((r - i) * h, (r + i) * h)
    if e == 6:
        return ((i - r) * h, (r + i) * (-h)) if sg < 0 else ((r + i) * (-h), (r - i) * h)
    c = np.float32(np.cos(2 * np.pi * e / 16))
    s = np.float32(sg * np.sin(2 * np.pi * e / 16))
    return (r * c - i * s, r * s + i * c)


def _fft16(x, sg):
    col = [_fft4(x[n], x[4 + n], x[8 + n], x[12 + n], sg) for n in range(4)]
    y = [None] * 16
    for k1 in range(4):
        r = _fft4(*[_tw16(col[n][k1], n * k1, sg) for n in range(4)], sg)
        for k2 in range(4):
            y[k1 + 4 * k2] = r[k2]
    return y


def _make_kernel(lq=1, lo=1, lag=16, d1=1, d2=3, bnd=3, unroll=1, xpose=1, fuse=1):
    scale = E ** -0.5
    Gq, Go = 2 ** lq, 2 ** lo
    G = max(Gq, Go)
    ncyc = S // SEG // G
    NP = H // 2
    pq, po = _all_products(lq), _all_products(lo)
    iq = {r: i for i, r in enumerate(pq)}
    io = {r: i for i, r in enumerate(po)}
    aq, ao = _assign(lq), _assign(lo)
    cq, co = _contrib(lq, aq), _contrib(lo, ao)
    KQ, NO = D // Gq, D // Go
    NGq, NGo = H // Gq, H // Go
    XA = 256

    def kernel(ax_h, wr_h, wi_h, bx_h, mem_h, wq_h, wk_h, wv_h, wo_h, cm_h, tw_h, out_h,
               ax, wrv, wiv, wnr, wni, cm, twv, twb, xs, ts, ya,
               bx, memv, rq, rk, rv, ro, tq, to, qx, part, on, lb, outp, ob, sems):
        cp = pltpu.make_async_copy
        c_const = [cp(cm_h, cm, sems.at[0]), cp(tw_h, twv, sems.at[0])]
        c_ax = [cp(ax_h.at[:, pl.ds(128 * j, 128)], ax.at[pl.ds(j * S, S)], sems.at[0]) for j in range(4)]
        c_w = [cp(h.at[pl.ds(0, 256), pl.ds(128 * k, 128)], v.at[pl.ds(256 * k, 256)], sems.at[1])
               for k in range(16) for h, v in ((wr_h, wrv), (wi_h, wiv))]
        c_w += [cp(h.at[pl.ds(256, 1)], v, sems.at[1]) for h, v in ((wr_h, wnr), (wi_h, wni))]
        c_q = [cp(bx_h.at[pl.ds(0, XA)], bx.at[pl.ds(0, XA)], sems.at[2]), cp(mem_h, memv, sems.at[2]),
               cp(wq_h, rq, sems.at[2])]
        c_k = [cp(wk_h, rk, sems.at[3])]
        c_v = [cp(wv_h, rv, sems.at[4])]
        NWO = 4
        c_o = [cp(wo_h.at[pl.ds(j * (H * E // NWO), H * E // NWO)], ro.at[pl.ds(j * (H * E // NWO), H * E // NWO)],
                  sems.at[5 + j]) for j in range(NWO)]
        c_x = cp(bx_h.at[pl.ds(XA, S - XA)], bx.at[pl.ds(XA, S - XA)], sems.at[9])
        for c in c_const + c_ax + c_w + c_q + c_k + c_v + c_o + [c_x]:
            c.start()
        on[...] = jnp.zeros(on.shape, f32)

        for c in c_const + c_ax:
            c.wait()
        for s in range(32):
            twb[s] = jnp.broadcast_to(twv[s:s + 1, :], (8, 128))
        mat = lambda a, b: pltpu.bitcast(cm[a:b], bf16)
        fa, fb = mat(0, 64), mat(64, 128)
        fcd = jnp.concatenate([mat(128, 256), mat(256, 384)], axis=1)
        ax_u = ax.bitcast(u32)
        for j0 in range(8):
            u = [ax_u[pl.ds(j * (S // 2) + j0, 128, stride=8), :] for j in range(4)]
            for h, un in enumerate((_lo, _hi)):
                x0, x1, x2, x3 = (un(v) for v in u)
                s02, s13 = x0 + x2, x1 + x3
                s1 = 2 * j0 + h
                xs[s1, 0:128, :] = _dot(fa, (s02 + s13).astype(bf16), NT)
                xs[s1, 128:256, :] = _dot(fb, (s02 - s13).astype(bf16), NT)
                xs[s1, 256:512, :] = _dot(fcd, jnp.concatenate([x0 - x2, x1 - x3], axis=1).astype(bf16), NT)

        for c in c_w:
            c.wait()
        fr, fi = mat(384, 448), mat(448, 512)
        fc = jnp.concatenate([jnp.concatenate([fr, fi], axis=1), jnp.concatenate([-fi, fr], axis=1)], axis=0)
        row = lax.broadcasted_iota(jnp.int32, (8, 128), 0)
        c2 = np.float32(2.0 / (S * D))
        wr_u, wi_u = wrv.bitcast(u32), wiv.bitcast(u32)

        def spectral_filter(t, w, dst):
            z = [t[0]] + [(t[s][0] * twb[s] - t[s][1] * twb[16 + s], t[s][0] * twb[16 + s] + t[s][1] * twb[s])
                          for s in range(1, 16)]
            y = _fft16(z, -1)
            y = [(a * w[k][0] - b * w[k][1], a * w[k][1] + b * w[k][0]) for k, (a, b) in enumerate(y)]
            z = _fft16(y, +1)
            for s in range(16):
                a, b = z[s]
                if s:
                    a, b = a * twb[s] + b * twb[16 + s], b * twb[s] - a * twb[16 + s]
                ts[s, dst[0]:dst[0] + 8, :] = a
                ts[s, dst[1]:dst[1] + 8, :] = b

        for par in range(2):
            for mb in range(8):
                offs = [GRP[par] + 8 * mb, GRP[2 + par] + 8 * mb]
                first = par == 0 and mb == 0
                rows = []
                for s in range(16):
                    for gi, o in enumerate(offs):
                        xr, xi = xs[s, o:o + 8, :], xs[s, o + 64:o + 72, :]
                        if first and gi == 0:
                            nyq = xi
                            xi = jnp.where(row == 0, 0.0, xi)
                        rows.append(jnp.concatenate([xr, xi], axis=1))
                    if first:
                        rows.append(jnp.concatenate([nyq, jnp.zeros_like(nyq)], axis=1))
                nb = 3 if first else 2
                t = _dot(jnp.concatenate(rows, axis=0), fc)
                ur = [wr_u[pl.ds(128 * k + 16 * mb + par, 8, stride=2), :] for k in range(16)]
                ui = [wi_u[pl.ds(128 * k + 16 * mb + par, 8, stride=2), :] for k in range(16)]
                for gi in range(nb):
                    tt = [(t[(s * nb + gi) * 8:(s * nb + gi + 1) * 8, :128],
                           t[(s * nb + gi) * 8:(s * nb + gi + 1) * 8, 128:]) for s in range(16)]
                    if gi < 2:
                        un = (_lo, _hi)[gi]
                        c = jnp.where(row == 0, 0.5 * c2, c2) if (first and gi == 0) else c2
                        w = [(un(ur[k]) * c, un(ui[k]) * c) for k in range(16)]
                        spectral_filter(tt, w, (offs[gi], offs[gi] + 64))
                    else:
                        nr, ni = wnr[...].astype(f32) * (0.5 * c2), wni[...].astype(f32) * (0.5 * c2)
                        w = [(jnp.broadcast_to(nr[:, 128 * k:128 * (k + 1)], (8, 128)),
                              jnp.broadcast_to(ni[:, 128 * k:128 * (k + 1)], (8, 128))) for k in range(16)]
                        spectral_filter(tt, w, (512, 520))

        fl = jnp.concatenate([fr, fi], axis=1)
        y_u = ya.bitcast(u32)
        for j0 in range(8):
            ys = []
            for h in range(2):
                s1 = 2 * j0 + h
                rhs = []
                for g in GRP:
                    tr, ti = ts[s1, g:g + 64, :], ts[s1, g + 64:g + 128, :]
                    a, b = ti, -tr
                    if g == 0:
                        a = jnp.concatenate([jnp.where(row == 0, ts[s1, 512:520, :], a[:8]), a[8:]], axis=0)
                        b = jnp.concatenate([jnp.where(row == 0, ts[s1, 520:528, :], b[:8]), b[8:]], axis=0)
                    rhs += [jnp.concatenate([tr, ti], axis=1), jnp.concatenate([a, b], axis=1)]
                u = _dot(fl, jnp.concatenate(rhs, axis=0).astype(bf16), NT).astype(bf16)
                e0, e1, dd = _dot(u[:, 0:128], fa), _dot(u[:, 128:256], fb), _dot(u[:, 256:512], fcd)
                p, q = e0 + e1, e0 - e1
                y = [p + dd[:, :128], q + dd[:, 128:], p - dd[:, :128], q - dd[:, 128:]]
                ys.append([pltpu.bitcast(v.astype(bf16).astype(f32), u32) for v in y])
            for j in range(4):
                y_u[pl.ds(j * (S // 2) + j0, 128, stride=8), :] = (ys[0][j] >> 16) | ys[1][j]

        wq = lambda g, m, r: pltpu.bitcast(tq[(g * 3 + m) * len(pq) + iq[r]], bf16)

        def wo(g, r):
            return jnp.concatenate([pltpu.bitcast(to[(g * len(po) + io[r]) * (NO // 128) + n], bf16)
                                    for n in range(NO // 128)], axis=1)

        def transform_qkv(raw, m, d0):
            ru = raw.bitcast(u32)
            for jb in range(2):
                words = {}
                for k in range(Gq):
                    base = (k * KQ + d0) * 16
                    if xpose:
                        half = []
                        for dh in range(2):
                            v = jnp.stack([ru[base + (8 * dh + i) * 16 + 8 * jb:base + (8 * dh + i) * 16 + 8 * jb + 8, :]
                                           for i in range(8)])
                            half.append(jnp.swapaxes(v, 0, 1))
                        for j in range(8):
                            words[(k, 8 * jb + j)] = jnp.concatenate([half[0][j], half[1][j]], axis=0)
                    else:
                        for j in range(8 * jb, 8 * jb + 8):
                            words[(k, j)] = ru[pl.ds(base + j, 16, stride=16), :]
                for g in range(16 * jb // Gq, 16 * (jb + 1) // Gq):
                    blocks = {(k, n): (_lo, _hi)[(g * Gq + n) % 2](words[(k, (g * Gq + n) // 2)])
                              for k in range(Gq) for n in range(Gq)}
                    for r, v in _pre(blocks, lq, SV, pq).items():
                        tq[(g * 3 + m) * len(pq) + iq[r], d0 // 2:d0 // 2 + 8, :] = pltpu.bitcast(v.astype(bf16), u32)

        def transform_o(g):
            for e0 in range(0, E, 16):
                blocks = {(k, n): ro[(g * Go + k) * E + e0:(g * Go + k) * E + e0 + 16, n * NO:(n + 1) * NO].astype(f32)
                          for k in range(Go) for n in range(Go)}
                for r, v in _pre(blocks, lo, SV, po).items():
                    w = pltpu.bitcast(v.astype(bf16), u32)
                    for n in range(NO // 128):
                        to[(g * len(po) + io[r]) * (NO // 128) + n, e0 // 2:e0 // 2 + 8, :] = w[:, 128 * n:128 * (n + 1)]

        def x_lhs(c):
            start = c * (Gq * SEG)
            if not isinstance(c, int):
                start = pl.multiple_of(start, Gq * SEG)
            xv = bx[pl.ds(start, Gq * SEG), :].astype(f32)
            return _pre({(i, k): xv[i * SEG:(i + 1) * SEG, k * KQ:(k + 1) * KQ] for i in range(Gq) for k in range(Gq)},
                        lq, SU, pq)

        def prologue(lx0, m, g):
            for (i, n), v in _post({r: _dot(lx0[r], wq(g, m, r)) for r in pq}, lq).items():
                qx[m, g * Gq + n, i * SEG:(i + 1) * SEG, :] = v

        nd = KQ // 16
        for c in c_q:
            c.wait()
        for i in range(nd):
            transform_qkv(rq, 0, 16 * i)
        for m, (cps, raw) in enumerate(((c_k, rk), (c_v, rv))):
            if not fuse:
                lx0 = x_lhs(0)
                for g in range(NGq):
                    prologue(lx0, m, g)
            for c in cps:
                c.wait()
            lx0 = x_lhs(0)
            for i in range(nd):
                transform_qkv(raw, m + 1, 16 * i)
                if fuse:
                    for g in range(i * NGq // nd, (i + 1) * NGq // nd):
                        prologue(lx0, m, g)
        for j in range(NWO):
            if not fuse and j == 0:
                lx0 = x_lhs(0)
                for g in range(NGq):
                    prologue(lx0, 2, g)
            c_o[j].wait()
            lx0 = x_lhs(0)
            for g in range(j * NGo // NWO, (j + 1) * NGo // NWO):
                transform_o(g)
            if fuse:
                for g in range(j * NGq // NWO, (j + 1) * NGq // NWO):
                    prologue(lx0, 2, g)

        c_ya = [cp(ya.at[pl.ds(j * S, S)], out_h.at[:, pl.ds(128 * j, 128)], sems.at[10]) for j in range(4)]
        for c in c_ya:
            c.start()

        R = 2 * L
        ri = lax.broadcasted_iota(jnp.int32, (R, R), 0)
        ci = lax.broadcasted_iota(jnp.int32, (R, R), 1)
        rh, ch = (ri >= L).astype(jnp.int32), (ci >= L).astype(jnp.int32)
        rr, cc = ri - rh * L, ci - ch * L
        same = rh == ch
        allowed = same & ((rr < M) | (rr >= cc))
        fill = jnp.where(same, np.float32(-1e9), np.float32(-np.inf))

        def step(cyc, ph, mem, lx):
            p_q, p_o = ph % Gq, ph % Go
            lm = _pre({(p_q, k): mem[:, k * KQ:(k + 1) * KQ] for k in range(Gq)}, lq, SU, [e[0] for e in aq[p_q]])
            lhs = {r: jnp.concatenate([lm[r], lx[r][a:b]], axis=0) for (r, a, b) in aq[p_q]}
            qkv, pend, acc, lmo = {}, {}, {}, {}
            sc, om = [None] * NP, [None] * H

            def do_qkv(g):
                for m in range(3):
                    for (r, a, b) in aq[p_q]:
                        if (g, m, r) not in pend:
                            pend[(g, m, r)] = _dot(lhs[r], wq(g, m, r))
                    res = {r: pend.pop((g, m, r)) for (r, a, b) in aq[p_q]}
                    cmem = _post({r: v[:M] for r, v in res.items()}, lq, [p_q])
                    for n in range(Gq):
                        qkv[(m, g * Gq + n)] = (cmem[(p_q, n)], qx[m, g * Gq + n, p_q * SEG:(p_q + 1) * SEG, :])
                    for rb in range(SEG // 8):
                        cx = _post({r: res[r][M + rb * 8 - a:M + rb * 8 + 8 - a]
                                    for (r, a, b) in aq[p_q] if a <= rb * 8 < b}, lq)
                        for (i, n), v in cx.items():
                            phs = cq[(i, n, rb)]
                            sl = (m, g * Gq + n, slice(i * SEG + rb * 8, i * SEG + rb * 8 + 8), slice(None))
                            if p_q != phs[0]:
                                v = v + part[sl]
                            if p_q == phs[-1]:
                                assert p_q >= i
                                qx[sl] = v
                            else:
                                part[sl] = v

            def cat(m, j):
                return jnp.concatenate(qkv[(m, 2 * j)] + qkv[(m, 2 * j + 1)], axis=0)

            def do_scores(j):
                s = jnp.where(allowed, _dot(cat(0, j), cat(1, j), NT) * scale, fill)
                p = jnp.exp(s - jnp.max(s, axis=-1, keepdims=True))
                sc[j] = p * pl.reciprocal(jnp.sum(p, axis=-1, keepdims=True), approx=False)

            def do_pv(j):
                if p_o == 0:
                    for g in range((2 * j + Go - 1) // Go, (2 * j + 2 + Go - 1) // Go):
                        prev = {(i, k): on[g * Go + k, i * SEG:(i + 1) * SEG, :] for i in range(Go) for k in range(Go)}
                        for r, v in _pre(prev, lo, SU, po).items():
                            lb[g * len(po) + io[r]] = v
                o = _dot(sc[j], cat(2, j))
                for u in range(2):
                    om[2 * j + u] = o[u * L:u * L + M]
                    on[2 * j + u, p_o * SEG:(p_o + 1) * SEG, :] = o[u * L + M:(u + 1) * L]

            def do_wo(g, only=None):
                if g not in lmo:
                    lmo[g] = _pre({(p_o, k): om[g * Go + k] for k in range(Go)}, lo, SU, [e[0] for e in ao[p_o]])
                for (r, a, b) in ao[p_o]:
                    if only is None or r in only:
                        v = _dot(jnp.concatenate([lmo[g][r], lb[g * len(po) + io[r], a:b, :]], axis=0), wo(g, r))
                        acc[r] = v if r not in acc else acc[r] + v

            if bnd and lq == 1:
                for gm in range(bnd):
                    for r in (((1,), (3,)) if p_q == 0 else ((4,), (1,))):
                        pend[(gm // 3, gm % 3, r)] = _dot(lhs[r], wq(gm // 3, gm % 3, r))
            tail = bnd if lo == 1 else 0
            nxt = 0
            for t in range(NP + d2):
                if t < NP:
                    for g in range((2 * t + Gq - 1) // Gq, (2 * t + 2 + Gq - 1) // Gq):
                        do_qkv(g)
                if 0 <= t - d1 < NP:
                    do_scores(t - d1)
                if 0 <= t - d2 < NP:
                    do_pv(t - d2)
                avail = (t - d2) * 2 - lag
                if t >= NP - 1:
                    avail = min((t - d2) * 2, avail + (t - (NP - 2)) * lag // (d2 + 1))
                while (nxt + 1) * Go <= avail and nxt < NGo - tail:
                    do_wo(nxt)
                    nxt += 1
            while nxt < NGo - tail:
                do_wo(nxt)
                nxt += 1
            if tail:
                first = ((3,), (5,)) if p_o == 0 else ((2,), (4,))
                for g in range(nxt, NGo):
                    do_wo(g, first)
                for g in range(nxt, NGo):
                    do_wo(g, [e[0] for e in ao[p_o] if e[0] not in first])

            cmem = _post({r: v[:M] for r, v in acc.items()}, lo, [p_o])
            for rb in range(SEG // 8):
                cx = _post({r: acc[r][M + rb * 8 - a:M + rb * 8 + 8 - a]
                            for (r, a, b) in ao[p_o] if a <= rb * 8 < b}, lo)
                for (i, n), v in cx.items():
                    sl = (slice(i * SEG + rb * 8, i * SEG + rb * 8 + 8), slice(n * NO, (n + 1) * NO))
                    if p_o != co[(i, n, rb)][0]:
                        v = v + outp[sl]
                    outp[sl] = v
            if p_o == Go - 1:
                oc = jnp.maximum(cyc * (G // Go) + ph // Go - 1, 0)
                ob[pl.ds(pl.multiple_of(oc * (Go * SEG), Go * SEG), Go * SEG), :] = outp[...].astype(bf16)
            return jnp.concatenate([cmem[(p_o, n)] for n in range(Go)], axis=1)

        RB = G * SEG * unroll

        def out_copy(start, size):
            return cp(ob.at[pl.ds(start, size)], out_h.at[pl.ds(start, size), pl.ds(D, D)], sems.at[11])

        def iteration(it, mem):
            @pl.when(it == max(XA // RB - 1, 0))
            def _():
                c_x.wait()

            @pl.when(it >= 2)
            def _():
                out_copy(pl.multiple_of((it - 2) * RB, RB), RB).start()

            for u in range(unroll):
                cyc = it * unroll + u
                for ph in range(G):
                    if ph % Gq == 0:
                        lx = x_lhs(jnp.minimum(cyc * (G // Gq) + ph // Gq + 1, S // SEG // Gq - 1))
                    mem = step(cyc, ph, mem, lx)
            return mem

        nit = ncyc // unroll
        lax.fori_loop(0, nit, iteration, memv[...].astype(f32))

        los = [_pre({(i, k): on[g * Go + k, i * SEG:(i + 1) * SEG, :] for i in range(Go) for k in range(Go)}, lo, SU, po)
               for g in range(NGo)]
        last = {r: _dot(jnp.concatenate([los[g][r] for g in range(NGo)], axis=1),
                        jnp.concatenate([wo(g, r) for g in range(NGo)], axis=0)) for r in po}
        for (i, n), v in _post(last, lo).items():
            ob[S - (Go - i) * SEG:S - (Go - i - 1) * SEG, n * NO:(n + 1) * NO] = v.astype(bf16)
        out_copy((nit - 2) * RB, 2 * RB).start()
        for c in c_ya:
            c.wait()
        out_copy(0, S).wait()

    scratch = [
        pltpu.VMEM((4 * S, 128), bf16), pltpu.VMEM((16 * 256, 128), bf16), pltpu.VMEM((16 * 256, 128), bf16),
        pltpu.VMEM((1, S), bf16), pltpu.VMEM((1, S), bf16),
        pltpu.VMEM(_DFT_MATS.shape, u32), pltpu.VMEM(_DFT_TW.shape, f32), pltpu.VMEM((32, 8, 128), f32),
        pltpu.VMEM((16, 512, 128), f32), pltpu.VMEM((16, 528, 128), f32), pltpu.VMEM((4 * S, 128), bf16),
        pltpu.VMEM((S, D), bf16), pltpu.VMEM((M, D), bf16),
        pltpu.VMEM((D * H, E), bf16), pltpu.VMEM((D * H, E), bf16), pltpu.VMEM((D * H, E), bf16),
        pltpu.VMEM((H * E, D), bf16),
        pltpu.VMEM((NGq * 3 * len(pq), KQ // 2, E), u32),
        pltpu.VMEM((NGo * len(po) * (NO // 128), E // 2, 128), u32),
        pltpu.VMEM((3, H, Gq * SEG, E), f32), pltpu.VMEM((3, H, Gq * SEG, E), f32),
        pltpu.VMEM((H, Go * SEG, E), f32), pltpu.VMEM((NGo * len(po), SEG, E), f32),
        pltpu.VMEM((Go * SEG, D), f32), pltpu.VMEM((S, D), bf16),
        pltpu.SemaphoreType.DMA((12,)),
    ]
    return kernel, scratch


def _run(A_x, A_w_r, A_w_i, B_x, B_mem0, B_Wq, B_Wk, B_Wv, B_Wo, flags=None, **cfg):
    kernel, scratch = _make_kernel(**cfg)
    hbm = pl.BlockSpec(memory_space=pl.ANY)
    out = pl.pallas_call(
        kernel,
        out_shape=jax.ShapeDtypeStruct((S, 2 * D), bf16),
        in_specs=[hbm] * 11,
        out_specs=hbm,
        scratch_shapes=scratch,
        compiler_params=pltpu.CompilerParams(vmem_limit_bytes=120 * 2 ** 20, flags=flags),
    )(A_x.reshape(S, D), A_w_r.T, A_w_i.T, B_x.reshape(S, D), B_mem0.reshape(M, D),
      B_Wq.reshape(D * H, E), B_Wk.reshape(D * H, E), B_Wv.reshape(D * H, E), B_Wo.reshape(H * E, D),
      _DFT_MATS, _DFT_TW)
    return out.reshape(1, S, 2 * D)


@jax.jit
def pallas_concat_heads__spectral_gfnet__memory_aug_recurrent_mem_tr__prompt_kernel(
    A_x: jax.Array,
    A_w_r: jax.Array,
    A_w_i: jax.Array,
    B_x: jax.Array,
    B_mem0: jax.Array,
    B_Wq: jax.Array,
    B_Wk: jax.Array,
    B_Wv: jax.Array,
    B_Wo: jax.Array,
    B_seg_len: jax.Array,
):
    del B_seg_len
    return _run(A_x, A_w_r, A_w_i, B_x, B_mem0, B_Wq, B_Wk, B_Wv, B_Wo, xpose=0)
```

```python
import contextlib
import jax
import jax.numpy as jnp
import ml_dtypes
import numpy as np
from jax import lax
import jax.experimental.pallas as pl
import jax.experimental.pallas.tpu as pltpu

S, D, H, E, M, SEG = 2048, 512, 32, 128, 8, 32
L = M + SEG
f32, bf16, u32 = jnp.float32, jnp.bfloat16, jnp.uint32
NN = (((1,), (0,)), ((), ()))
NT = (((1,), (1,)), ((), ()))


def _dot(a, b, dims=NN):
    return lax.dot_general(a, b, dims, preferred_element_type=f32)


def _lo(u):
    return pltpu.bitcast(u << 16, f32)


def _hi(u):
    return pltpu.bitcast(u & np.uint32(0xFFFF0000), f32)


SU = {1: (((0, 0), 1), ((1, 1), 1)), 2: (((1, 0), 1), ((1, 1), 1)), 3: (((0, 0), 1),), 4: (((1, 1), 1),),
      5: (((0, 0), 1), ((0, 1), 1)), 6: (((1, 0), 1), ((0, 0), -1)), 7: (((0, 1), 1), ((1, 1), -1))}
SV = {1: (((0, 0), 1), ((1, 1), 1)), 2: (((0, 0), 1),), 3: (((0, 1), 1), ((1, 1), -1)),
      4: (((1, 0), 1), ((0, 0), -1)), 5: (((1, 1), 1),), 6: (((0, 0), 1), ((0, 1), 1)),
      7: (((1, 0), 1), ((1, 1), 1))}
SW = {(0, 0): ((1, 1), (4, 1), (7, 1), (5, -1)), (0, 1): ((3, 1), (5, 1)), (1, 0): ((2, 1), (4, 1)),
      (1, 1): ((1, 1), (3, 1), (6, 1), (2, -1))}
PHASE = ((1, 3, 5, 7), (1, 2, 4, 6))


def _lin(terms):
    terms = [(v, c) for v, c in terms if v is not None]
    if not terms:
        return None
    pos = [v for v, c in terms if c > 0]
    neg = [v for v, c in terms if c < 0]
    if pos:
        acc = pos[0]
        for v in pos[1:]:
            acc = acc + v
    else:
        acc, neg = -neg[0], neg[1:]
    for v in neg:
        acc = acc - v
    return acc


def _pre(blocks, level, table, want):
    if level == 0:
        return {(): blocks.get((0, 0))}
    h = 2 ** (level - 1)
    out = {}
    for r in sorted({w[0] for w in want}):
        sub = {(i, k): _lin([(blocks.get((a * h + i, b * h + k)), c) for (a, b), c in table[r]])
               for i in range(h) for k in range(h)}
        for rr, v in _pre(sub, level - 1, table, sorted(w[1:] for w in want if w[0] == r)).items():
            out[(r,) + rr] = v
    return out


def _post(prods, level, rows=None):
    if level == 0:
        return {(0, 0): prods[()]}
    h = 2 ** (level - 1)
    subrows = None if rows is None else [i % h for i in rows]
    inner = {r: _post({w[1:]: v for w, v in prods.items() if w[0] == r}, level - 1, subrows)
             for r in sorted({w[0] for w in prods})}
    out = {}
    for (a, b), terms in SW.items():
        for i in range(h):
            if rows is not None and a * h + i not in rows:
                continue
            for n in range(h):
                v = _lin([(inner.get(r, {}).get((i, n)), c) for r, c in terms])
                if v is not None:
                    out[(a * h + i, b * h + n)] = v
    return out


def _all_products(level):
    out = [()]
    for _ in range(level):
        out = [o + (r,) for o in out for r in range(1, 8)]
    return out


def _phase_products(level, p):
    out = [()]
    for l in range(level):
        out = [o + (r,) for o in out for r in PHASE[(p >> (level - 1 - l)) & 1]]
    return out


def _assign(level, mode=0, uneven=0):
    G = 2 ** level
    rows = {p: {} for p in range(G)}
    for r in _all_products(level):
        cand = [p for p in range(G) if r in _phase_products(level, p)]
        n = SEG // len(cand)
        if uneven and len(cand) == 2:
            big = min(cand, key=lambda p: (sum(b - a for a, b in rows[p].values()), p))
            for p in cand:
                rows[p][r] = (0, 24) if p == big else (24, 32)
            continue
        for j, p in enumerate(cand):
            rows[p][r] = (j * n, (j + 1) * n)
    out = {}
    for p in range(G):
        prods = _phase_products(level, p)
        lng = [r for r in prods if rows[p][r][1] - rows[p][r][0] == SEG]
        sht = [r for r in prods if rows[p][r][1] - rows[p][r][0] < SEG]
        order, k = [], 0
        for j in range(len(prods)):
            if sht and (j + 1) * len(sht) // len(prods) > k:
                order.append(sht[k])
                k += 1
            else:
                order.append(lng[j - k])
        if mode:
            rank = {1: {3: 0, 1: 1, 5: 2, 7: 3, 4: 0, 2: 1, 6: 3}, 2: {3: 0, 5: 1, 1: 2, 7: 3, 4: 0, 2: 1, 6: 3},
                    3: {1: 0, 3: 1, 5: 2, 7: 3, 2: 1, 4: 2, 6: 3}}[mode]
            order = sorted(prods, key=lambda r: tuple((rank[x], x) for x in r))
        out[p] = [(r,) + rows[p][r] for r in order]
    return out


def _contrib(level, asg):
    c = {}
    for p in range(2 ** level):
        for (r, a, b) in asg[p]:
            for rb in range(a // 8, b // 8):
                for key in _post({r: np.zeros(1)}, level):
                    lst = c.setdefault(key + (rb,), [])
                    if p not in lst:
                        lst.append(p)
    return c


def _dft_constants():
    n = np.arange(128)[None, :]
    m = np.arange(64)[:, None]
    th = lambda k: 2 * np.pi * ((k * n) % 512) / 512
    fa = np.concatenate([np.cos(th(4 * m)), -np.sin(th(4 * m))])
    fa[64] = np.cos(np.pi * n[0])
    fb = np.concatenate([np.cos(th(4 * m + 2)), -np.sin(th(4 * m + 2))])
    c1, s1, c3, s3 = np.cos(th(4 * m + 1)), np.sin(th(4 * m + 1)), np.cos(th(4 * m + 3)), np.sin(th(4 * m + 3))
    f0 = np.concatenate([c1, -s1, c3, -s3])
    f1 = np.concatenate([-s1, -c1, s3, c3])
    a = np.arange(128)
    ph = 2 * np.pi * ((a[:, None] * a[None, :]) % 128) / 128
    fwd = np.concatenate([fa, fb, f0, f1])
    gain = np.full((fwd.shape[0], 1), 2.0 / (S * D))
    gain[0] = gain[64] = 1.0 / (S * D)
    u = np.concatenate([fwd, fwd * gain]).astype(np.float32).astype(ml_dtypes.bfloat16).view(np.uint16).astype(np.uint32)
    tp = 2 * np.pi * (np.arange(16)[:, None] * a[None, :]) / S
    return (u[0::2] | (u[1::2] << 16), np.concatenate([np.cos(ph), -np.sin(ph)]).astype(np.float32),
            np.concatenate([np.cos(tp), -np.sin(tp)]).astype(np.float32))


_DFT_ROWS, _DFT_128, _DFT_TW = _dft_constants()


def _fft4(a, b, c, d, sg):
    t0 = (a[0] + c[0], a[1] + c[1])
    t1 = (a[0] - c[0], a[1] - c[1])
    t2 = (b[0] + d[0], b[1] + d[1])
    t3 = (b[0] - d[0], b[1] - d[1])
    y0 = (t0[0] + t2[0], t0[1] + t2[1])
    y2 = (t0[0] - t2[0], t0[1] - t2[1])
    p = (t1[0] + t3[1], t1[1] - t3[0])
    q = (t1[0] - t3[1], t1[1] + t3[0])
    return (y0, p, y2, q) if sg < 0 else (y0, q, y2, p)


def _tw16(z, e, sg):
    if e == 0:
        return z
    r, i = z
    if e == 4:
        return (i, -r) if sg < 0 else (-i, r)
    h = np.float32(np.sqrt(0.5))
    if e == 2:
        return ((r + i) * h, (i - r) * h) if sg < 0 else ((r - i) * h, (r + i) * h)
    if e == 6:
        return ((i - r) * h, (r + i) * (-h)) if sg < 0 else ((r + i) * (-h), (r - i) * h)
    c = np.float32(np.cos(2 * np.pi * e / 16))
    s = np.float32(sg * np.sin(2 * np.pi * e / 16))
    return (r * c - i * s, r * s + i * c)


def _fft16(x, sg):
    col = [_fft4(x[n], x[4 + n], x[8 + n], x[12 + n], sg) for n in range(4)]
    y = [None] * 16
    for k1 in range(4):
        r = _fft4(*[_tw16(col[n][k1], n * k1, sg) for n in range(4)], sg)
        for k2 in range(4):
            y[k1 + 4 * k2] = r[k2]
    return y


def _make_kernel(lq=2, lo=2, res=600, d1=200, d2=500, d3=150, gap=100, bnd=0, tail=0, unroll=1, xpose=0, fuse=1, scopes=0,
                 bonly=0, newton=1, kvbf=1, order=0, nh=1, dbuf=1, lref=0, wb=1, accref=1, pref=1, po_ord=0, dz=0, uneven=0, lbf=0, abf=0, o1=6, o2=6, o3=5, o4=4, blk=1, sp=3, defer=1, pord=0, ocut=3, f3u=1, st8=0, pun=4, gauss=1):
    stack = contextlib.ExitStack()

    def mark(name):
        if scopes:
            stack.close()
            if name:
                stack.enter_context(jax.named_scope('P_' + name))

    scale = E ** -0.5
    Gq, Go = 2 ** lq, 2 ** lo
    G = max(Gq, Go)
    ncyc = S // SEG // G
    NP = H // 2
    pq, po = _all_products(lq), _all_products(lo)
    iq = {r: i for i, r in enumerate(pq)}
    io = {r: i for i, r in enumerate(po)}
    aq, ao = _assign(lq, po_ord, uneven & 1), _assign(lo, po_ord, uneven & 2)
    cq, co = _contrib(lq, aq), _contrib(lo, ao)
    KQ, NO = D // Gq, D // Go
    NGq, NGo = H // Gq, H // Go
    XA = 256

    def kron(sets):
        out = [()]
        for st in sets:
            out = [o + (r,) for o in out for r in st]
        return out

    def schedule(ph):
        p_q, p_o = ph % Gq, ph % Go
        bits = lambda p, level: [(p >> (level - 1 - l)) & 1 for l in range(level)]
        size = {r: b - a for (r, a, b) in aq[p_q]}

        def mix(prods, size):
            lng = [r for r in prods if size[r] == SEG]
            sht = [r for r in prods if size[r] < SEG]
            out = []
            while lng or sht:
                if lng:
                    out.append(lng.pop(0))
                if sht and len(sht) >= len(lng) - 1:
                    out.append(sht.pop(0))
            return out

        early = []
        if bnd and lq == lo:
            early = kron([{(0, 1): (1, 3), (0, 0): (7,), (1, 1): (6,), (1, 0): (1, 4)}[(nb, pb)]
                          for nb, pb in zip(bits(p_q, lq), bits((ph - 1) % Go, lo))])
        prods = [e[0] for e in aq[p_q]]
        per = 4 // (KQ // 128)

        def qkv_block(groups, first):
            if first or blk == 0 or lq != 2:
                rs = mix([r for r in prods if r in early], size) + mix([r for r in prods if r not in early], size) \
                    if first else mix(prods, size)
                return [[('q', g, m, r) for (g, m) in groups[i:i + per]] for i in range(0, 4, per) for r in rs]
            lng = [r for r in prods if size[r] == SEG]
            sht = [r for r in prods if size[r] == SEG // 2]
            tiny = [r for r in prods if size[r] == SEG // 4]
            shared = lambda r: [('q', g, m, r) for (g, m) in groups]
            own = lambda i, rs: [('q',) + groups[i] + (r,) for r in rs]
            return [shared(lng[8]), shared(sht[4]), own(0, lng[:4]), shared(sht[5]), own(0, lng[4:8]), own(0, sht[:4]),
                    own(1, lng[:4]), shared(tiny[0]), own(1, lng[4:8]), own(1, sht[:4]),
                    own(2, lng[:4]), own(2, sht[:4]), own(2, lng[4:8]), own(3, lng[:4]), own(3, sht[:4]), own(3, lng[4:8])]

        flat = [(g, m) for g in range(NGq) for m in (0, 1)] + [(g, 2) for g in range(NGq)]
        rounds, done = [], {}
        for i in range(0, len(flat), 4):
            rounds += qkv_block(flat[i:i + 4], i == 0 and bnd)
        for t, rd in enumerate(rounds):
            for it in rd:
                done[it[1:3]] = t + 1
        size_o = {r: b - a for (r, a, b) in ao[p_o]}
        rows_o = {r: (a, b) for (r, a, b) in ao[p_o]}
        first = kron([((3, 5), (2, 4))[b] for b in bits(p_o, lo)]) if tail else []
        prods_o = [e[0] for e in ao[p_o]]
        wper = 4 // (NO // 128)
        nq = len(rounds)
        for g0 in range(0, NGo, wper):
            rs = mix(prods_o, size_o)
            if g0 + wper == NGo:
                rs = mix([r for r in prods_o if r in first], size_o) + mix([r for r in prods_o if r not in first], size_o)
            rounds += [[('w', tuple(range(g0, g0 + wper)), r) + rows_o[r]] for r in rs]
        NP = H // nh
        grp = lambda j: range(nh * j // Gq, (nh * j + nh - 1) // Gq + 1)
        ins, last = {}, -99
        t_s = {}
        for j0 in range(0, NP, 4):
            t = max(max(done[(g, m)] for j in range(j0, j0 + 4) for g in grp(j) for m in (0, 1)) + o1, last + sp)
            ins.setdefault(t, []).append([('s', j) for j in range(j0, j0 + 4)])
            last = t_s[j0] = t
        for j0 in range(0, NP, 4):
            t = max(max(done[(g, 2)] for j in range(j0, j0 + 4) for g in grp(j)) + o2, t_s[j0] + o3, last + sp)
            ins.setdefault(t, []).append([('p', j) for j in range(j0, j0 + 4)])
            last = t
        out = []
        for t, rd in enumerate(rounds):
            for extra in ins.get(t, []):
                out += extra
            out += rd
        return out

    def kernel(ax_h, wr_h, wi_h, bx_h, mem_h, wq_h, wk_h, wv_h, wo_h, cm_h, fm_h, tw_h, out_h,
               ax, wrv, wiv, wnr, wni, cm, fm, twv, gm, xs, ts, ya,
               bx, memv, rw, ro, tq, to, qx, part, lq_ref, lm_ref, on, lb, wacc, pbuf, outp, ob, sems, osem):
        cp = pltpu.make_async_copy
        c_const = [cp(fm_h, fm, sems.at[8]), cp(tw_h, twv, sems.at[8])]
        c_ax = [cp(cm_h.at[pl.ds(0, 384)], cm.at[pl.ds(0, 384)], sems.at[0])] + [cp(ax_h.at[:, pl.ds(128 * j, 128)], ax.at[pl.ds(j * S, S)], sems.at[0]) for j in range(4)]
        c_w = [cp(h.at[pl.ds(0, 256), pl.ds(128 * k, 128)], v.at[pl.ds(256 * k, 256)], sems.at[1])
               for k in range(16) for h, v in ((wr_h, wrv), (wi_h, wiv))]
        c_w += [cp(h.at[pl.ds(256, 1)], v, sems.at[1]) for h, v in ((wr_h, wnr), (wi_h, wni))]
        c_w += [cp(cm_h.at[pl.ds(384, 384)], cm.at[pl.ds(384, 384)], sems.at[1])]
        c_w += [cp(bx_h.at[pl.ds(0, XA)], bx.at[pl.ds(0, XA)], sems.at[1]), cp(mem_h, memv, sems.at[1])]
        aligned = lambda v, n: v if isinstance(v, int) else pl.multiple_of(v, n)

        def c_qkv(h, m):
            if st8:
                return [cp(h.bitcast(u32).at[:, pl.ds(8 * t, 8), :], rw.at[pl.ds(aligned((2 * m + t) * D, D), D)], sems.at[2 + m])
                        for t in range(2)]
            return [cp(h, rw.at[pl.ds(aligned(m * D * H, D * H), D * H)], sems.at[2 + m])]

        rw2 = rw.reshape(6 * D * 8, E) if st8 else None
        NWO = 8
        RO = H * E // NWO

        def c_o(j):
            start = j * RO if isinstance(j, int) else pl.multiple_of(j * RO, RO)
            return [cp(wo_h.at[pl.ds(start, RO), pl.ds(128 * n, 128)], ro.at[pl.ds(n * H * E + start, RO)], osem.at[j])
                    for n in range(4)]

        c_x = cp(bx_h.at[pl.ds(XA, S - XA)], bx.at[pl.ds(XA, S - XA)], sems.at[5])
        late = sum((c_o(j) for j in range(NWO)), []) + [c_x]
        for c in c_const + c_ax + c_w + c_qkv(wq_h, 0) + c_qkv(wk_h, 1) + c_qkv(wv_h, 2) + ([] if defer else late):
            c.start()
        on[...] = jnp.zeros(on.shape, f32)

        mark('wait_c')
        for c in c_const:
            c.wait()
        mat = lambda a, b: pltpu.bitcast(cm[a:b], bf16)
        fr, fi = fm[0:128, :], fm[128:256, :]
        for s in range(16):
            tr, ti = twv[s:s + 1, :], twv[16 + s:17 + s, :]
            gr, gi = fr * tr - fi * ti, fr * ti + fi * tr
            for c, v in enumerate((gr, gi, gr + gi, gi - gr)):
                gm[s, c] = v.astype(bf16)
        g_mat = lambda s, c: pltpu.bitcast(gm.bitcast(u32)[s, c], bf16)
        mark('wait_ax')
        for c in c_ax:
            c.wait()
        mark('fft12')
        fa, fb = mat(0, 64), mat(64, 128)
        fcd = jnp.concatenate([mat(128, 256), mat(256, 384)], axis=1)
        row = lax.broadcasted_iota(jnp.int32, (8, 128), 0)
        ax_u = ax.bitcast(u32)

        def rfft_rows(s1):
            un = (_lo, _hi)[s1 % 2]
            x0, x1, x2, x3 = (un(ax_u[pl.ds(j * (S // 2) + s1 // 2, 128, stride=8), :]) for j in range(4))
            s02, s13 = x0 + x2, x1 + x3
            xa = _dot(fa, (s02 + s13).astype(bf16), NT)
            xb = _dot(fb, (s02 - s13).astype(bf16), NT)
            xc = _dot(fcd, jnp.concatenate([x0 - x2, x1 - x3], axis=1).astype(bf16), NT)
            nyq = xa[64:72]
            re = jnp.concatenate([xa[:64], xb[:64], xc[:64], xc[128:192], nyq], axis=0)
            im = jnp.concatenate([jnp.where(row == 0, 0.0, nyq), xa[72:], xb[64:], xc[64:128], xc[192:]], axis=0)
            return re, im

        def dft128(s1, re, im):
            if gauss:
                k1 = _dot(jnp.concatenate([re[:256] + im, re[256:]], axis=0), g_mat(s1, 0))
                xs[s1, 0, 0:256, :] = k1[:256] - _dot(im, g_mat(s1, 2))
                xs[s1, 0, 256:264, :] = k1[256:]
                xs[s1, 1] = k1 + _dot(re, g_mat(s1, 3))
                return
            g = jnp.concatenate([g_mat(s1, 0), g_mat(s1, 1)], axis=1)
            p, q = _dot(re, g), _dot(im, g)
            xs[s1, 0, 0:256, :] = p[:256, :128] - q[:, 128:]
            xs[s1, 1, 0:256, :] = p[:256, 128:] + q[:, :128]
            xs[s1, 0, 256:264, :] = p[256:, :128]
            xs[s1, 1, 256:264, :] = p[256:, 128:]

        if not bonly:
            pend = rfft_rows(0)
            for s1 in range(16):
                nxt = rfft_rows(s1 + 1) if s1 < 15 else None
                dft128(s1, *pend)
                pend = nxt

        mark('wait_w')
        for c in c_w:
            c.wait()
        if defer:
            for c in late:
                c.start()
        mark('fft3')
        wr_u, wi_u = wrv.bitcast(u32), wiv.bitcast(u32)

        def spectral_filter(r0, w):
            y = _fft16([(xs[s, 0, pl.ds(r0, 8), :], xs[s, 1, pl.ds(r0, 8), :]) for s in range(16)], -1)
            z = _fft16([(a * w[k][0] - b * w[k][1], a * w[k][1] + b * w[k][0]) for k, (a, b) in enumerate(y)], +1)
            for s in range(16):
                ts[s, 0, pl.ds(r0, 8), :] = z[s][0]
                ts[s, 1, pl.ds(r0, 8), :] = z[s][1]

        if not bonly:
            nr, ni = wnr[...].astype(f32), wni[...].astype(f32)
            spectral_filter(256, [(jnp.broadcast_to(nr[:, 128 * k:128 * (k + 1)], (8, 128)),
                                   jnp.broadcast_to(ni[:, 128 * k:128 * (k + 1)], (8, 128))) for k in range(16)])

            for p, gs in ((0, (0, 1)), (1, (0, 1))) if f3u == 1 else ((0, (0,)), (0, (1,)), (1, (0,)), (1, (1,))):
                @pl.loop(0, 8)
                def _(i):
                    w0 = [pl.multiple_of(128 * k + 16 * i, 16) for k in range(16)]
                    ur = [wr_u.at[pl.ds(v, 16)][pl.ds(p, 8, stride=2), :] for v in w0]
                    ui = [wi_u.at[pl.ds(v, 16)][pl.ds(p, 8, stride=2), :] for v in w0]
                    for g in gs:
                        un = (_lo, _hi)[g]
                        spectral_filter(pl.multiple_of((2 * g + p) * 64 + 8 * i, 8), [(un(a), un(b)) for a, b in zip(ur, ui)])

        mark('fft45')
        ia, ib = mat(384, 448), mat(448, 512)
        icd = jnp.concatenate([mat(512, 640), mat(640, 768)], axis=1)

        def idft128(s1):
            rhs = []
            for g in range(4):
                tr, ti = ts[s1, 0, 64 * g:64 * (g + 1), :], ts[s1, 1, 64 * g:64 * (g + 1), :]
                a, b = ti, -tr
                if g == 0:
                    a = jnp.concatenate([jnp.where(row == 0, ts[s1, 0, 256:264, :], a[:8]), a[8:]], axis=0)
                    b = jnp.concatenate([jnp.where(row == 0, ts[s1, 1, 256:264, :], b[:8]), b[8:]], axis=0)
                rhs += [jnp.concatenate([tr, ti], axis=1), jnp.concatenate([a, b], axis=1)]
            return _dot(jnp.concatenate([g_mat(s1, 0), g_mat(s1, 1)], axis=1),
                        jnp.concatenate(rhs, axis=0).astype(bf16), NT)

        def irfft_rows(u):
            e0, e1, dd = _dot(u[:, 0:128], ia), _dot(u[:, 128:256], ib), _dot(u[:, 256:512], icd)
            p, q = e0 + e1, e0 - e1
            return [p + dd[:, :128], q + dd[:, 128:], p - dd[:, :128], q - dd[:, 128:]]

        if not bonly:
            pend = idft128(0)
            for s1 in range(16):
                nxt = idft128(s1 + 1) if s1 < 15 else None
                y = [pltpu.bitcast(v.astype(bf16).astype(f32), u32) for v in irfft_rows(pend)]
                if s1 % 2:
                    for j in range(4):
                        ya.bitcast(u32)[pl.ds(j * (S // 2) + s1 // 2, 128, stride=8), :] = (even[j] >> 16) | y[j]
                pend, even = nxt, y

        slot = lambda g, m, r: (m * NGq + g) * len(pq) + iq[r]
        wq = lambda g, m, r: pltpu.bitcast(tq.bitcast(u32)[slot(g, m, r)], bf16)

        def wo(g, r):
            return jnp.concatenate([pltpu.bitcast(to.bitcast(u32)[(g * len(po) + io[r]) * (NO // 128) + n], bf16)
                                    for n in range(NO // 128)], axis=1)

        def transform_qkv(m, i):
            for g in range(NGq):
                words = {}
                for k in range(Gq):
                    for j in range(g * Gq // 2, (g * Gq + Gq + 1) // 2):
                        if st8:
                            base = ((2 * m + j // 8) * D + k * KQ + 16 * i) * 8
                            words[(k, j)] = rw2.at[pl.ds(aligned(base, 128), 128)][pl.ds(j % 8, 16, stride=8), :]
                        else:
                            base = (m * D + k * KQ + 16 * i) * 16
                            words[(k, j)] = rw.bitcast(u32).at[pl.ds(aligned(base, 256), 256)][pl.ds(j, 16, stride=16), :]
                blocks = {(k, n): (_lo, _hi)[(g * Gq + n) % 2](words[(k, (g * Gq + n) // 2)])
                          for k in range(Gq) for n in range(Gq)}
                for r, v in _pre(blocks, lq, SV, pq).items():
                    tq[slot(g, m, r), pl.ds(aligned(16 * i, 16), 16), :] = v.astype(bf16)

        def transform_o(g, pieces):
            ru = ro.bitcast(u32)
            for e0 in (8 * p for p in pieces):
                for c in range(NO // 128):
                    blocks = {(k, n): pltpu.bitcast(ru[pl.ds(aligned(
                        ((n * (NO // 128) + c) * H + g * Go + k) * (E // 2) + e0, 8), 8), :], bf16).astype(f32)
                              for k in range(Go) for n in range(Go)}
                    for r, v in _pre(blocks, lo, SV, po).items():
                        to[(g * len(po) + io[r]) * (NO // 128) + c, 2 * e0:2 * e0 + 16, :] = v.astype(bf16)

        def x_lhs(c):
            start = c * (Gq * SEG)
            if not isinstance(c, int):
                start = pl.multiple_of(start, Gq * SEG)
            xv = bx[pl.ds(start, Gq * SEG), :].astype(f32)
            return _pre({(i, k): xv[i * SEG:(i + 1) * SEG, k * KQ:(k + 1) * KQ] for i in range(Gq) for k in range(Gq)},
                        lq, SU, pq)

        def first_rows(m, g):
            prods = {r: _dot(lq_ref[iq[r]], wq(g, m, r)) for r in pq}
            for (i, n), v in _post(prods, lq).items():
                if i == Gq - 1:
                    part[m, g * Gq + n] = v
                else:
                    qx[m, g * Gq + n, i * SEG:(i + 1) * SEG, :] = v

        mark('tr_qkv')
        for r, v in x_lhs(0).items():
            lq_ref[iq[r]] = v

        @pl.loop(0, 3)
        def _(m):
            for c in c_qkv(wq_h, m):
                c.wait()
            if not bonly:
                pl.loop(0, KQ // 16)(lambda i: transform_qkv(m, i))
                pl.loop(0, NGq, unroll=pun)(lambda g: first_rows(m, g))

        mark('tr_o')

        @pl.loop(0, NWO)
        def _(j):
            for c in c_o(j):
                c.wait()
            if not bonly:
                transform_o(j, range(8))

        c_ya = [cp(ya.at[pl.ds(j * S, S)], out_h.at[:, pl.ds(128 * j, 128)], sems.at[6]) for j in range(4)]
        for c in c_ya:
            c.start()

        R = nh * L
        NP = H // nh
        ri = lax.broadcasted_iota(jnp.int32, (R, R), 0)
        ci = lax.broadcasted_iota(jnp.int32, (R, R), 1)
        rh = sum(((ri >= L * j).astype(jnp.int32) for j in range(1, nh)), jnp.zeros_like(ri))
        ch = sum(((ci >= L * j).astype(jnp.int32) for j in range(1, nh)), jnp.zeros_like(ci))
        rr, cc = ri - rh * L, ci - ch * L
        same = rh == ch
        allowed = same & ((rr < M) | (rr >= cc))
        log2e = np.float32(np.log2(np.e))
        fill = jnp.where(same, np.float32(-1e9) * log2e, np.float32(-np.inf))

        held = {}

        def step(cyc, ph, mem, lx, zero):
            p_q, p_o = ph % Gq, ph % Go
            z1, z2, z3, z4 = ((zero if dz & b else 0) for b in (1, 2, 4, 8))
            lm = _pre({(p_q, k): mem[:, k * KQ:(k + 1) * KQ] for k in range(Gq)}, lq, SU, [e[0] for e in aq[p_q]])
            staged, lcache = [], {}

            def lhs(r, a, b, direct):
                if r not in lcache:
                    v = jnp.concatenate([lm[r], lx[r][a:b]], axis=0)
                    if lbf & 1 and v.shape[0] % 16 == 0:
                        v = v.astype(bf16)
                    elif dz:
                        return v
                    lcache[r] = v
                return lcache[r]

            rows_q = {r: (a, b) for (r, a, b) in aq[p_q]}
            qkv, res_q, acc, lmo = {}, {}, {}, {}
            sc, om = [None] * NP, [None] * H

            def finish_qkv(g, m):
                i = (p_q - 1) % Gq
                rows = lambda i, rb: slice(i * SEG + rb * 8, i * SEG + rb * 8 + 8)
                for n in range(Gq):
                    for rb in range(SEG // 8):
                        if cq[(i, n, rb)][-1] == i:
                            h = g * Gq + n
                            qx[m, h, rows(i, rb), :] = held.pop((m, h, i, rb)) if p_q else part[m, h, rows(0, rb), :]
                res = {r: res_q.pop((g, m, r)) for (r, a, b) in aq[p_q]}
                cmem = _post({r: v[:M] for r, v in res.items()}, lq, [p_q])
                for n in range(Gq):
                    qkv[(m, g * Gq + n)] = cmem[(p_q, n)]
                for rb in range(SEG // 8):
                    cx = _post({r: res[r][M + rb * 8 - a:M + rb * 8 + 8 - a]
                                for (r, a, b) in aq[p_q] if a <= rb * 8 < b}, lq)
                    for (i, n), v in cx.items():
                        h = g * Gq + n
                        phs = cq[(i, n, rb)]
                        assert phs[-1] >= i
                        if p_q != phs[0]:
                            v = v + held.pop((m, h, i, rb))
                        if p_q == phs[-1] and p_q != i:
                            qx[m, h, rows(i, rb), :] = v
                        elif p_q == Gq - 1:
                            part[m, h, rows(0, rb), :] = v
                        else:
                            held[(m, h, i, rb)] = v

            def cat(m, j):
                v = jnp.concatenate(sum(((qkv[(m, h)], qx[m, h, p_q * SEG:(p_q + 1) * SEG, :])
                                         for h in range(nh * j, nh * j + nh)), ()), axis=0)
                return v.astype(bf16) if (kvbf and m) else v

            def do_scores(j):
                s = jnp.where(allowed, _dot(cat(0, j).astype(bf16) if abf & 1 else cat(0, j), cat(1, j), NT) * (np.float32(scale) * log2e), fill)
                p = jnp.exp2(s - jnp.max(s, axis=-1, keepdims=True))
                l = jnp.sum(p, axis=-1, keepdims=True)
                if newton:
                    r0 = pl.reciprocal(l, approx=True)
                    sc[j] = p * (r0 * (2.0 - l * r0))
                else:
                    sc[j] = p * pl.reciprocal(l, approx=False)
                if abf & 2:
                    sc[j] = sc[j].astype(bf16)
                if pref:
                    pbuf[j] = sc[j]

            def do_pv(j):
                if p_o == 0:
                    for g in range((nh * j + Go - 1) // Go, (nh * j + nh + Go - 1) // Go):
                        prev = {(i, k): on[g * Go + k, i * SEG:(i + 1) * SEG, :] for i in range(Go) for k in range(Go)}
                        for r, v in _pre(prev, lo, SU, po).items():
                            lb[g * len(po) + io[r]] = v
                o = _dot(pbuf[j] if pref else sc[j], cat(2, j))
                for u in range(nh):
                    om[nh * j + u] = o[u * L:u * L + M]
                    on[nh * j + u, p_o * SEG:(p_o + 1) * SEG, :] = o[u * L + M:(u + 1) * L]

            def do_wo(gs, r, a, b):
                for g in gs:
                    if g not in lmo:
                        lmo[g] = _pre({(p_o, k): om[g * Go + k] for k in range(Go)}, lo, SU, [e[0] for e in ao[p_o]])
                l = jnp.concatenate([jnp.concatenate([lmo[g][r], lb[z3 + g * len(po) + io[r], a:b, :]], axis=0)
                                     for g in gs], axis=1)
                if lbf & 2 and l.shape[0] % 16 == 0:
                    l = l.astype(bf16)
                v = _dot(l, jnp.concatenate([wo(g, r) for g in gs], axis=0))
                if accref:
                    if gs[0] > 0:
                        v = v + wacc[io[r], 0:M + b - a, :]
                    if gs[-1] < NGo - 1:
                        wacc[io[r], 0:M + b - a, :] = v
                    acc[r] = v
                else:
                    acc[r] = v if r not in acc else acc[r] + v

            for pos, item in enumerate(schedule(ph)):
                if item[0] == 'q':
                    _, g, m, r = item
                    res_q[(g, m, r)] = _dot(lhs(r, *rows_q[r], pos < bnd), wq(g, m, r))
                    if all((g, m, e[0]) in res_q for e in aq[p_q]):
                        finish_qkv(g, m)
                elif item[0] == 's':
                    do_scores(item[1])
                elif item[0] == 'p':
                    do_pv(item[1])
                else:
                    do_wo(*item[1:])

            cmem = _post({r: v[:M] for r, v in acc.items()}, lo, [p_o])
            for rb in range(SEG // 8):
                cx = _post({r: acc[r][M + rb * 8 - a:M + rb * 8 + 8 - a]
                            for (r, a, b) in ao[p_o] if a <= rb * 8 < b}, lo)
                for (i, n), v in cx.items():
                    sl = (slice(i * SEG + rb * 8, i * SEG + rb * 8 + 8), slice(n * NO, (n + 1) * NO))
                    if p_o != co[(i, n, rb)][0]:
                        v = v + outp[sl]
                    outp[sl] = v
            if p_o == Go - 1:
                oc = jnp.maximum(cyc * (G // Go) + ph // Go - 1, 0)
                ob[pl.ds(pl.multiple_of(oc * (Go * SEG), Go * SEG), Go * SEG), :] = outp[...].astype(bf16)
            return jnp.concatenate([cmem[(p_o, n)] for n in range(Go)], axis=1)

        RB = G * SEG * unroll

        def out_copy(start, size):
            return cp(ob.at[pl.ds(start, size)], out_h.at[pl.ds(start, size), pl.ds(D, D)], sems.at[7])

        def iteration(it, mem):
            @pl.when(it == max(XA // RB - 1, 0))
            def _():
                c_x.wait()

            @pl.when(it >= 2)
            def _():
                out_copy(pl.multiple_of((it - 2) * RB, RB), RB).start()

            for u in range(unroll):
                cyc = it * unroll + u
                for ph in range(G):
                    if ph % Gq == 0:
                        lx = x_lhs(jnp.minimum(cyc * (G // Gq) + ph // Gq + 1, S // SEG // Gq - 1))
                    mem = step(cyc, ph, mem, lx, jnp.minimum(it, 0))
            return mem

        nit = ncyc // unroll
        mark('loop')
        lax.fori_loop(0, nit, iteration, memv[...].astype(f32))

        mark('epi')
        los = [_pre({(i, k): on[g * Go + k, i * SEG:(i + 1) * SEG, :] for i in range(Go) for k in range(Go)}, lo, SU, po)
               for g in range(NGo)]
        last = {r: _dot(jnp.concatenate([los[g][r] for g in range(NGo)], axis=1),
                        jnp.concatenate([wo(g, r) for g in range(NGo)], axis=0)) for r in po}
        for (i, n), v in _post(last, lo).items():
            ob[S - (Go - i) * SEG:S - (Go - i - 1) * SEG, n * NO:(n + 1) * NO] = v.astype(bf16)
        mark('tail')
        out_copy((nit - 2) * RB, 2 * RB).start()
        for c in c_ya:
            c.wait()
        out_copy(0, S).wait()
        mark(None)

    scratch = [
        pltpu.VMEM((4 * S, 128), bf16), pltpu.VMEM((16 * 256, 128), bf16), pltpu.VMEM((16 * 256, 128), bf16),
        pltpu.VMEM((1, S), bf16), pltpu.VMEM((1, S), bf16),
        pltpu.VMEM(_DFT_ROWS.shape, u32), pltpu.VMEM(_DFT_128.shape, f32), pltpu.VMEM(_DFT_TW.shape, f32),
        pltpu.VMEM((16, 4, 128, 128), bf16), pltpu.VMEM((16, 2, 264, 128), f32), pltpu.VMEM((16, 2, 264, 128), f32),
        pltpu.VMEM((4 * S, 128), bf16),
        pltpu.VMEM((S, D), bf16), pltpu.VMEM((M, D), bf16),
        pltpu.VMEM((6 * D, 8, E), u32) if st8 else pltpu.VMEM((3 * D * H, E), bf16),
        pltpu.VMEM((4 * H * E, 128), bf16),
        pltpu.VMEM((3 * NGq * len(pq), KQ, E), bf16),
        pltpu.VMEM((NGo * len(po) * (NO // 128), E, 128), bf16),
        pltpu.VMEM((3, H, Gq * SEG, E), f32), pltpu.VMEM((3, H, SEG, E), f32),
        pltpu.VMEM((len(pq), SEG, KQ), f32), pltpu.VMEM((len(pq), M, KQ), f32),
        pltpu.VMEM((H, Go * SEG, E), f32), pltpu.VMEM((NGo * len(po), SEG, E), f32),
        pltpu.VMEM((len(po), L, NO), f32), pltpu.VMEM((H // nh, nh * L, nh * L), bf16 if abf & 2 else f32),
        pltpu.VMEM((Go * SEG, D), f32), pltpu.VMEM((S, D), bf16),
        pltpu.SemaphoreType.DMA((9,)), pltpu.SemaphoreType.DMA((8,)),
    ]
    return kernel, scratch


def _run(A_x, A_w_r, A_w_i, B_x, B_mem0, B_Wq, B_Wk, B_Wv, B_Wo, flags=None, **cfg):
    kernel, scratch = _make_kernel(**cfg)
    hbm = pl.BlockSpec(memory_space=pl.ANY)
    out = pl.pallas_call(
        kernel,
        out_shape=jax.ShapeDtypeStruct((S, 2 * D), bf16),
        in_specs=[hbm] * 12,
        out_specs=hbm,
        scratch_shapes=scratch,
        compiler_params=pltpu.CompilerParams(vmem_limit_bytes=126 * 2 ** 20, flags=flags),
    )(A_x.reshape(S, D), A_w_r.T, A_w_i.T, B_x.reshape(S, D), B_mem0.reshape(M, D),
      *[w if cfg.get('st8', 0) else w.reshape(D * H, E) for w in (B_Wq, B_Wk, B_Wv)], B_Wo.reshape(H * E, D),
      _DFT_ROWS, _DFT_128, _DFT_TW)
    return out.reshape(1, S, 2 * D)


@jax.jit
def pallas_concat_heads__spectral_gfnet__memory_aug_recurrent_mem_tr__prompt_kernel(
    A_x: jax.Array,
    A_w_r: jax.Array,
    A_w_i: jax.Array,
    B_x: jax.Array,
    B_mem0: jax.Array,
    B_Wq: jax.Array,
    B_Wk: jax.Array,
    B_Wv: jax.Array,
    B_Wo: jax.Array,
    B_seg_len: jax.Array,
):
    del B_seg_len
    return _run(A_x, A_w_r, A_w_i, B_x, B_mem0, B_Wq, B_Wk, B_Wv, B_Wo, st8=1, pun=8)
```

```python
import jax
import jax.numpy as jnp
import ml_dtypes
import numpy as np
from jax import lax
import jax.experimental.pallas as pl
import jax.experimental.pallas.tpu as pltpu

S, D, H, E, M, SEG = 2048, 512, 32, 128, 8, 32
L = M + SEG
G = 4
NG = H // G
RB = G * SEG
NIT = S // RB
f32, bf16, u32 = jnp.float32, jnp.bfloat16, jnp.uint32
NN = (((1,), (0,)), ((), ()))
NT = (((1,), (1,)), ((), ()))


def _dot(a, b, dims=NN):
    return lax.dot_general(a, b, dims, preferred_element_type=f32)


def _lo(u):
    return pltpu.bitcast(u << 16, f32)


def _hi(u):
    return pltpu.bitcast(u & np.uint32(0xFFFF0000), f32)


SU = {1: (((0, 0), 1), ((1, 1), 1)), 2: (((1, 0), 1), ((1, 1), 1)), 3: (((0, 0), 1),), 4: (((1, 1), 1),),
      5: (((0, 0), 1), ((0, 1), 1)), 6: (((1, 0), 1), ((0, 0), -1)), 7: (((0, 1), 1), ((1, 1), -1))}
SV = {1: (((0, 0), 1), ((1, 1), 1)), 2: (((0, 0), 1),), 3: (((0, 1), 1), ((1, 1), -1)),
      4: (((1, 0), 1), ((0, 0), -1)), 5: (((1, 1), 1),), 6: (((0, 0), 1), ((0, 1), 1)),
      7: (((1, 0), 1), ((1, 1), 1))}
SW = {(0, 0): ((1, 1), (4, 1), (7, 1), (5, -1)), (0, 1): ((3, 1), (5, 1)), (1, 0): ((2, 1), (4, 1)),
      (1, 1): ((1, 1), (3, 1), (6, 1), (2, -1))}
OWN = ((3, 1, 5, 7), (4, 1, 2, 6))


def _lin(terms):
    terms = [(v, c) for v, c in terms if v is not None]
    if not terms:
        return None
    pos = [v for v, c in terms if c > 0]
    neg = [v for v, c in terms if c < 0]
    if pos:
        acc = pos[0]
        for v in pos[1:]:
            acc = acc + v
    else:
        acc, neg = -neg[0], neg[1:]
    for v in neg:
        acc = acc - v
    return acc


def _pre(blocks, table, want):
    if not want[0]:
        return {(): blocks.get((0, 0))}
    h = 2 ** (len(want[0]) - 1)
    out = {}
    for r in sorted({w[0] for w in want}):
        sub = {(i, k): _lin([(blocks.get((a * h + i, b * h + k)), c) for (a, b), c in table[r]])
               for i in range(h) for k in range(h)}
        for rest, v in _pre(sub, table, sorted(w[1:] for w in want if w[0] == r)).items():
            out[(r,) + rest] = v
    return out


def _post(prods, row=None):
    if () in prods:
        return {(0, 0): prods[()]}
    h = 2 ** (len(next(iter(prods))) - 1)
    inner = {r: _post({w[1:]: v for w, v in prods.items() if w[0] == r}, None if row is None else row % h)
             for r in sorted({w[0] for w in prods})}
    out = {}
    for (a, b), terms in SW.items():
        for i in range(h):
            if row is None or row == a * h + i:
                for n in range(h):
                    v = _lin([(inner.get(r, {}).get((i, n)), c) for r, c in terms])
                    if v is not None:
                        out[(a * h + i, b * h + n)] = v
    return out


PRODUCTS = [(a, b) for a in range(1, 8) for b in range(1, 8)]
NPR = len(PRODUCTS)
INDEX = {r: i for i, r in enumerate(PRODUCTS)}


def _token_rows():
    phases = [[(a, b) for a in OWN[p >> 1] for b in OWN[p & 1]] for p in range(G)]
    rows = []
    for p in range(G):
        rows.append({})
        for r in phases[p]:
            users = [q for q in range(G) if r in phases[q]]
            n = SEG // len(users)
            rows[p][r] = (users.index(p) * n, (users.index(p) + 1) * n)
    return rows


def _contributors(rows):
    out = {}
    for p in range(G):
        for r, (a, b) in rows[p].items():
            for rb in range(a // 8, b // 8):
                for key in _post({r: np.zeros(1)}):
                    if p not in out.setdefault(key + (rb,), []):
                        out[key + (rb,)].append(p)
    return out


ROWS = _token_rows()
ADDS = _contributors(ROWS)


def _schedule(p):
    size = {r: b - a for r, (a, b) in ROWS[p].items()}
    long_ = [r for r in size if size[r] == SEG]
    short = [r for r in size if size[r] == SEG // 2]
    tiny = [r for r in size if size[r] == SEG // 4]
    prev = (p - 1) % G
    early = [{(0, 1): (1, 3), (0, 0): (7,), (1, 1): (6,), (1, 0): (1, 4)}[(p >> s & 1, prev >> s & 1)] for s in (1, 0)]
    lead = ([r for r in long_ if r[0] in early[0] and r[1] in early[1]] + [long_[8]])[0]
    pool = [lead, short[4], tiny[0], short[5]]
    rest = [r for r in long_ if r != lead]
    groups = [(g, m) for g in range(NG) for m in (1, 0)] + [(g, 2) for g in range(NG)]
    shared = lambda i, r: [('project', g, m, r) for (g, m) in groups[i:i + 4]]
    own = lambda i, rs: [('project',) + groups[i] + (r,) for r in rs]
    rounds = []
    for i in range(len(groups)):
        a, b, c = own(i, rest[:4]), own(i, short[:4]), own(i, rest[4:])
        if i == 0:
            rounds += [shared(0, pool[0]), shared(0, pool[1]), a, shared(0, pool[2]), c, b, shared(0, pool[3])]
        else:
            rounds += [a, b, c]
        if i // 4 * 4 + 4 < len(groups):
            rounds.append(shared(i // 4 * 4 + 4, pool[i % 4]))
    done = {item[1:3]: t + 1 for t, rd in enumerate(rounds) for item in rd}
    rest, mixed = list(long_), []
    fill = [r for r in size if size[r] < SEG]
    while rest or fill:
        mixed += rest[:1]
        rest = rest[1:]
        if fill and len(fill) >= len(rest) - 1:
            mixed.append(fill.pop(0))
    for g0 in range(0, NG, 4):
        rounds += [[('output', tuple(range(g0, g0 + 4)), r)] for r in mixed]
    extra = {}

    def place(t, items):
        while any(abs(t - u) < 3 for u in extra):
            t += 1
        extra[t] = items
        return t

    scored = [place(max(done[(g, 0)], done[(g, 1)]) + 6, [('scores', G * g + n) for n in range(G)]) for g in range(NG)]
    for g in range(NG):
        place(max(done[(g, 2)] + 6, scored[g] + 5), [('values', G * g + n) for n in range(G)])
    return [item for t, rd in enumerate(rounds) for item in extra.get(t, []) + rd]


def _dft_constants():
    n = np.arange(128)[None, :]
    m = np.arange(64)[:, None]
    angle = lambda k: 2 * np.pi * ((k * n) % D) / D
    even0 = np.concatenate([np.cos(angle(4 * m)), -np.sin(angle(4 * m))])
    even0[64] = np.cos(np.pi * n[0])
    even2 = np.concatenate([np.cos(angle(4 * m + 2)), -np.sin(angle(4 * m + 2))])
    cr = np.concatenate([np.cos(angle(4 * m + 1)), np.cos(angle(4 * m + 3))])
    ci = np.concatenate([-np.sin(angle(4 * m + 1)), np.sin(angle(4 * m + 3))])
    fwd = np.concatenate([even0, even2, cr, cr + ci, ci - cr])
    gain = np.full((fwd.shape[0], 1), 2.0 / (S * D))
    gain[0] = gain[64] = 1.0 / (S * D)
    rows = np.concatenate([fwd, fwd * gain]).astype(np.float32).astype(ml_dtypes.bfloat16)
    rows = rows.view(np.uint16).astype(np.uint32)
    k = np.arange(128)
    ph = 2 * np.pi * ((k[:, None] * k[None, :]) % 128) / 128
    tw = 2 * np.pi * (np.arange(16)[:, None] * k[None, :]) / S
    return (rows[0::2] | (rows[1::2] << 16),
            np.concatenate([np.cos(ph), -np.sin(ph)]).astype(np.float32),
            np.concatenate([np.cos(tw), -np.sin(tw)]).astype(np.float32))


_DFT_ROWS, _DFT_128, _DFT_TWIDDLE = _dft_constants()


def _fft4(a, b, c, d, sign):
    t0 = (a[0] + c[0], a[1] + c[1])
    t1 = (a[0] - c[0], a[1] - c[1])
    t2 = (b[0] + d[0], b[1] + d[1])
    t3 = (b[0] - d[0], b[1] - d[1])
    y0 = (t0[0] + t2[0], t0[1] + t2[1])
    y2 = (t0[0] - t2[0], t0[1] - t2[1])
    p = (t1[0] + t3[1], t1[1] - t3[0])
    q = (t1[0] - t3[1], t1[1] + t3[0])
    return (y0, p, y2, q) if sign < 0 else (y0, q, y2, p)


def _rotate16(z, e, sign):
    if e == 0:
        return z
    r, i = z
    if e == 4:
        return (i, -r) if sign < 0 else (-i, r)
    h = np.float32(np.sqrt(0.5))
    if e == 2:
        return ((r + i) * h, (i - r) * h) if sign < 0 else ((r - i) * h, (r + i) * h)
    if e == 6:
        return ((i - r) * h, (r + i) * (-h)) if sign < 0 else ((r + i) * (-h), (r - i) * h)
    c = np.float32(np.cos(2 * np.pi * e / 16))
    s = np.float32(sign * np.sin(2 * np.pi * e / 16))
    return (r * c - i * s, r * s + i * c)


def _fft16(x, sign):
    col = [_fft4(x[n], x[4 + n], x[8 + n], x[12 + n], sign) for n in range(4)]
    y = [None] * 16
    for k1 in range(4):
        r = _fft4(*[_rotate16(col[n][k1], n * k1, sign) for n in range(4)], sign)
        for k2 in range(4):
            y[k1 + 4 * k2] = r[k2]
    return y


def _kernel(ax_h, wr_h, wi_h, bx_h, mem_h, wq_h, wk_h, wv_h, wo_h, rows_h, f128_h, tw_h, out_h,
            ax, wr, wi, nyq_r, nyq_i, rows_v, f128, tw, gmat, xs, ts, ya,
            bx, mem0, raw_qkv, raw_o, t_qkv, t_o, lhs0, tok, tok_late, att, att_lhs, probs, acc_o, acc_last,
            part_o, yb, sems, row_sems, filt_sems, wo_sems):
    copy = pltpu.make_async_copy

    def start(copies):
        for c in copies:
            c.start()

    def wait(copies):
        for c in copies:
            c.wait()

    half = _DFT_ROWS.shape[0] // 2
    c_const = [copy(f128_h, f128, sems.at[0]), copy(tw_h, tw, sems.at[0]),
               copy(rows_h.at[pl.ds(0, half)], rows_v.at[pl.ds(0, half)], sems.at[0])]
    c_ax = [copy(ax_h.bitcast(u32).at[:, j, :], ax.at[j], row_sems.at[j]) for j in range(8)]
    c_filt = [[copy(src.at[pl.ds(128 * b, 128), pl.ds(128 * k, 128)], dst.at[pl.ds(256 * k + 128 * b, 128)], filt_sems.at[b])
               for k in range(16) for src, dst in ((wr_h, wr), (wi_h, wi))] for b in range(2)]
    c_filt[0] += [copy(src.at[pl.ds(256, 1)], dst, filt_sems.at[0]) for src, dst in ((wr_h, nyq_r), (wi_h, nyq_i))]
    c_small = [copy(rows_h.at[pl.ds(half, half)], rows_v.at[pl.ds(half, half)], sems.at[1]),
               copy(bx_h.at[pl.ds(0, 2 * RB)], bx.at[pl.ds(0, 2 * RB)], sems.at[1]), copy(mem_h, mem0, sems.at[1])]
    c_qkv = [[copy(src.bitcast(u32).at[:, j, :], raw_qkv.at[m * (H // 2) + j], sems.at[2 + m]) for j in range(H // 2)]
             for m, src in enumerate((wq_h, wk_h, wv_h))]
    c_bx = copy(bx_h.at[pl.ds(2 * RB, S - 2 * RB)], bx.at[pl.ds(2 * RB, S - 2 * RB)], sems.at[5])
    c_ya = [copy(ya.at[j], out_h.bitcast(u32).at[:, j, pl.ds(0, D)], sems.at[6]) for j in range(8)]

    def c_wo(g):
        r0 = g * (G * E) if isinstance(g, int) else pl.multiple_of(g * (G * E), G * E)
        return [copy(wo_h.at[pl.ds(r0, G * E), pl.ds(128 * n, 128)], raw_o.at[pl.ds(n * H * E + r0, G * E)], wo_sems.at[g])
                for n in range(G)]

    def c_yb(row, size):
        rows = pl.ds(row // 16, size // 16)
        return copy(yb.at[rows], out_h.at[rows, :, pl.ds(D, D)], sems.at[7])

    start(c_const + c_ax + c_filt[0])
    for ref in (att, acc_last, part_o):
        ref[...] = jnp.zeros(ref.shape, f32)

    wait(c_const)
    fr, fi = f128[0:128, :], f128[128:256, :]
    for s in range(16):
        tr, ti = tw[s:s + 1, :], tw[16 + s:17 + s, :]
        gr, gi = fr * tr - fi * ti, fr * ti + fi * tr
        for c, v in enumerate((gr, gi, gr + gi, gi - gr)):
            gmat[s, c] = v.astype(bf16)
    g_mat = lambda s, c: pltpu.bitcast(gmat.bitcast(u32)[s, c], bf16)
    row_mat = lambda i: pltpu.bitcast(rows_v[64 * i:64 * (i + 1)], bf16)
    first = lax.broadcasted_iota(jnp.int32, (8, 128), 0) == 0

    def rfft_rows(s):
        unpack = (_lo, _hi)[s % 2]
        x0, x1, x2, x3 = (unpack(ax[s // 2, :, 128 * j:128 * (j + 1)]) for j in range(4))
        s02, s13 = x0 + x2, x1 + x3
        xa = _dot(row_mat(0), (s02 + s13).astype(bf16), NT)
        xb = _dot(row_mat(1), (s02 - s13).astype(bf16), NT)
        d0, d1 = x0 - x2, x3 - x1
        k1 = _dot(row_mat(2), (d0 + d1).astype(bf16), NT)
        er = k1 - _dot(row_mat(3), d1.astype(bf16), NT)
        ei = k1 + _dot(row_mat(4), d0.astype(bf16), NT)
        nyq = xa[64:72]
        return (jnp.concatenate([xa[:64], xb[:64], er, nyq], axis=0),
                jnp.concatenate([jnp.where(first, 0.0, nyq), xa[72:], xb[64:], ei[:64], -ei[64:]], axis=0))

    def dft128(s, re, im):
        k1 = _dot(jnp.concatenate([re[:256] + im, re[256:]], axis=0), g_mat(s, 0))
        xs[s, 0, 0:256, :] = k1[:256] - _dot(im, g_mat(s, 2))
        xs[s, 0, 256:264, :] = k1[256:]
        xs[s, 1] = k1 + _dot(re, g_mat(s, 3))

    wait(c_ax[:2])
    pending = rfft_rows(0)
    for s in range(16):
        if s == 3:
            wait(c_ax[2:4])
            start(c_filt[1] + c_small)
        if s == 7:
            wait(c_ax[4:])
            start(c_qkv[0])
        ahead = rfft_rows(s + 1) if s < 15 else None
        dft128(s, *pending)
        pending = ahead

    wait(c_filt[0])
    start(c_qkv[1])

    def spectral_filter(r0, w):
        y = _fft16([(xs[s, 0, r0:r0 + 8, :], xs[s, 1, r0:r0 + 8, :]) for s in range(16)], -1)
        z = _fft16([(a * w[k][0] - b * w[k][1], a * w[k][1] + b * w[k][0]) for k, (a, b) in enumerate(y)], +1)
        for s in range(16):
            ts[s, 0, r0:r0 + 8, :] = z[s][0]
            ts[s, 1, r0:r0 + 8, :] = z[s][1]

    nr, ni = nyq_r[...].astype(f32), nyq_i[...].astype(f32)
    spectral_filter(256, [(jnp.broadcast_to(nr[:, 128 * k:128 * (k + 1)], (8, 128)),
                           jnp.broadcast_to(ni[:, 128 * k:128 * (k + 1)], (8, 128))) for k in range(16)])
    for i in range(8):
        if i == 4:
            wait(c_filt[1])
        for p in range(2):
            words = [[ref.bitcast(u32).at[pl.ds(128 * k + 16 * i, 16)][pl.ds(p, 8, stride=2), :] for ref in (wr, wi)]
                     for k in range(16)]
            for g, unpack in enumerate((_lo, _hi)):
                spectral_filter((2 * g + p) * 64 + 8 * i, [(unpack(a), unpack(b)) for a, b in words])

    start(c_qkv[2])
    wait(c_small)

    def idft128(s):
        real, imag = [], []
        for g in range(4):
            tr, ti = ts[s, 0, 64 * g:64 * (g + 1), :], ts[s, 1, 64 * g:64 * (g + 1), :]
            a, b = (-ti, tr) if g == 3 else (ti, -tr)
            if g == 0:
                a = jnp.concatenate([jnp.where(first, ts[s, 0, 256:264, :], a[:8]), a[8:]], axis=0)
                b = jnp.concatenate([jnp.where(first, ts[s, 1, 256:264, :], b[:8]), b[8:]], axis=0)
            real.append(jnp.concatenate([tr, ti], axis=1))
            imag.append(jnp.concatenate([a, b], axis=1))
        rhs = jnp.concatenate([real[0], imag[0], real[1], imag[1], real[2], real[3], imag[2], imag[3]], axis=0)
        return _dot(jnp.concatenate([g_mat(s, 0), g_mat(s, 1)], axis=1), rhs.astype(bf16), NT)

    def irfft_rows(u):
        e0, e1 = _dot(u[:, 0:128], row_mat(5)), _dot(u[:, 128:256], row_mat(6))
        ur, ui = u[:, 256:384], u[:, 384:512]
        k1 = _dot(ur + ui, row_mat(7))
        d0, d1 = k1 + _dot(ui, row_mat(9)), k1 - _dot(ur, row_mat(8))
        p, q = e0 + e1, e0 - e1
        return [p + d0, q - d1, p - d0, q + d1]

    pending = idft128(0)
    for s in range(16):
        ahead = idft128(s + 1) if s < 15 else None
        y = [pltpu.bitcast(v.astype(bf16).astype(f32), u32) for v in irfft_rows(pending)]
        if s % 2:
            for j in range(4):
                ya[s // 2, :, 128 * j:128 * (j + 1)] = (even[j] >> 16) | y[j]
        pending, even = ahead, y

    def w_qkv(g, m, r):
        return pltpu.bitcast(t_qkv.bitcast(u32)[(m * NG + g) * NPR + INDEX[r]], bf16)

    def w_o(g, r):
        return pltpu.bitcast(t_o.bitcast(u32)[g * NPR + INDEX[r]], bf16)

    def token_operands(it):
        x = bx[pl.ds(it * RB if isinstance(it, int) else pl.multiple_of(it * RB, RB), RB), :].astype(f32)
        return _pre({(i, k): x[i * SEG:(i + 1) * SEG, k * 128:(k + 1) * 128] for i in range(G) for k in range(G)},
                    SU, PRODUCTS)

    for r, v in token_operands(0).items():
        lhs0[INDEX[r]] = v
    for m in range(3):
        wait(c_qkv[m])
        if m == 0:
            start(sum((c_wo(g) for g in range(NG)), []) + [c_bx])

        @pl.loop(0, NG)
        def _(g):
            for d0 in range(0, 128, 16):
                words = {(k, j): raw_qkv[m * (H // 2) + 2 * g + j, k * 128 + d0:k * 128 + d0 + 16, :]
                         for k in range(G) for j in range(2)}
                blocks = {(k, n): (_lo, _hi)[n % 2](words[(k, n // 2)]) for k in range(G) for n in range(G)}
                for r, v in _pre(blocks, SV, PRODUCTS).items():
                    t_qkv[(m * NG + g) * NPR + INDEX[r], d0:d0 + 16, :] = v.astype(bf16)

        for g in range(NG):
            for (i, n), v in _post({r: _dot(lhs0[INDEX[r]], w_qkv(g, m, r)) for r in PRODUCTS}).items():
                if i == G - 1:
                    tok_late[m, G * g + n] = v
                else:
                    tok[m, G * g + n, i * SEG:(i + 1) * SEG, :] = v

    @pl.loop(0, NG)
    def _(g):
        wait(c_wo(g))
        for e0 in range(0, E, 16):
            blocks = {(k, n): pltpu.bitcast(raw_o.bitcast(u32)[pl.ds(pl.multiple_of(
                (n * H + G * g + k) * (E // 2) + e0 // 2, 8), 8), :], bf16).astype(f32) for k in range(G) for n in range(G)}
            for r, v in _pre(blocks, SV, PRODUCTS).items():
                t_o[g * NPR + INDEX[r], e0:e0 + 16, :] = v.astype(bf16)

    start(c_ya)

    ri = lax.broadcasted_iota(jnp.int32, (L, L), 0)
    ci = lax.broadcasted_iota(jnp.int32, (L, L), 1)
    allowed = (ri < M) | (ri >= ci)
    log2e = np.float32(np.log2(np.e))
    slab = lambda i, rb: slice(i * SEG + rb * 8, i * SEG + rb * 8 + 8)

    def combine(p, prods):
        for rb in range(SEG // 8):
            here = {r: prods[r][rb * 8 - a:rb * 8 + 8 - a] for r, (a, b) in ROWS[p].items() if a <= rb * 8 < b}
            for (i, n), v in _post(here).items():
                yield i, n, rb, v

    def emit(p, prods, it):
        for i, n, rb, v in combine(p, prods):
            where = (slab(i, rb), slice(128 * n, 128 * (n + 1)))
            part_o[where] = v if p == ADDS[(i, n, rb)][0] else v + part_o[where]
        if p == G - 1:
            yb[pl.ds(jnp.maximum(it, 0) * (RB // 16), RB // 16)] = part_o[...].astype(bf16).reshape(RB // 16, 16, D)

    def emit_last(it):
        emit(G - 1, {r: acc_last[INDEX[r], 0:b - a, :] for r, (a, b) in ROWS[G - 1].items()}, it)

    def segment(p, mem, ahead, held):
        prods = list(ROWS[p])
        mem_in = _pre({(p, k): mem[:, 128 * k:128 * (k + 1)] for k in range(G)}, SU, prods)
        operand = {r: jnp.concatenate([ahead[r][a:b], mem_in[r]], axis=0) for r, (a, b) in ROWS[p].items()}
        result, mem_qkv, mem_att, mem_out, acc = {}, {}, {}, {}, {}

        def project(g, m, r):
            result[(g, m, r)] = _dot(operand[r], w_qkv(g, m, r))
            if any((g, m, q) not in result for q in prods):
                return
            i = (p - 1) % G
            for n in range(G):
                for rb in range(SEG // 8):
                    if ADDS[(i, n, rb)][-1] == i:
                        h = G * g + n
                        tok[m, h, slab(i, rb), :] = held.pop((m, h, i, rb)) if p else tok_late[m, h, slab(0, rb), :]
            res = {q: result.pop((g, m, q)) for q in prods}
            for (_, n), v in _post({q: v[-M:] for q, v in res.items()}, p).items():
                mem_qkv[(m, G * g + n)] = v
            for i, n, rb, v in combine(p, res):
                h, adds = G * g + n, ADDS[(i, n, rb)]
                assert adds[-1] >= i
                if p != adds[0]:
                    v = v + held.pop((m, h, i, rb))
                if p == adds[-1] and p != i:
                    tok[m, h, slab(i, rb), :] = v
                elif p == G - 1:
                    tok_late[m, h, slab(0, rb), :] = v
                else:
                    held[(m, h, i, rb)] = v

        def rows_of(m, h):
            return jnp.concatenate([mem_qkv[(m, h)], tok[m, h, p * SEG:(p + 1) * SEG, :]], axis=0)

        def scores(h):
            s = _dot(rows_of(0, h), rows_of(1, h).astype(bf16), NT) * (np.float32(E ** -0.5) * log2e)
            s = jnp.where(allowed, s, np.float32(-1e9) * log2e)
            e = jnp.exp2(s - jnp.max(s, axis=-1, keepdims=True))
            total = jnp.sum(e, axis=-1, keepdims=True)
            r = pl.reciprocal(total, approx=True)
            probs[h] = e * (r * (2.0 - total * r))

        def values(h):
            if p == 0 and h % G == 0:
                before = {(i, k): att[h + k, i * SEG:(i + 1) * SEG, :] for i in range(G) for k in range(G)}
                for r, v in _pre(before, SU, PRODUCTS).items():
                    att_lhs[h // G * NPR + INDEX[r]] = v
            o = _dot(probs[h], rows_of(2, h).astype(bf16))
            mem_att[h] = o[:M]
            att[h, p * SEG:(p + 1) * SEG, :] = o[M:]

        def output(gs, r):
            a, b = ROWS[p][r]
            for g in gs:
                if g not in mem_out:
                    mem_out[g] = _pre({(p, k): mem_att[G * g + k] for k in range(G)}, SU, prods)
            v = _dot(jnp.concatenate([jnp.concatenate([mem_out[g][r], att_lhs[g * NPR + INDEX[r], a:b, :]], axis=0)
                                      for g in gs], axis=1),
                     jnp.concatenate([w_o(g, r) for g in gs], axis=0))
            if gs[0] > 0:
                v = v + acc_o[INDEX[r], 0:M + b - a, :]
            if gs[-1] < NG - 1:
                acc_o[INDEX[r], 0:M + b - a, :] = v
            acc[r] = v

        run = {'project': project, 'scores': scores, 'values': values, 'output': output}
        for item in _schedule(p):
            run[item[0]](*item[1:])
        if p < G - 1:
            emit(p, {r: v[M:] for r, v in acc.items()}, None)
        else:
            for r, (a, b) in ROWS[p].items():
                acc_last[INDEX[r], 0:b - a, :] = acc[r][M:]
        new = _post({r: v[:M] for r, v in acc.items()}, p)
        return jnp.concatenate([new[(p, n)] for n in range(G)], axis=1)

    def iteration(it, mem):
        @pl.when((it == 1) | ((it % 4 == 2) & (it > 2)))
        def _():
            pl.when(it == 1)(c_bx.wait)
            pl.when(it > 1)(lambda: c_yb((it - 6) * RB, 4 * RB).start())

        emit_last(it - 2)
        ahead, held = token_operands(jnp.minimum(it + 1, NIT - 1)), {}
        for p in range(G):
            mem = segment(p, mem, ahead, held)
        return mem

    lax.fori_loop(0, NIT, iteration, mem0[...].astype(f32))
    emit_last(NIT - 2)
    c_yb((NIT - 4) * RB, 3 * RB).start()

    last = [_pre({(i, k): att[G * g + k, i * SEG:(i + 1) * SEG, :] for i in range(G) for k in range(G)}, SU, PRODUCTS)
            for g in range(NG)]
    prods = {r: _dot(jnp.concatenate([last[g][r] for g in range(NG)], axis=1),
                     jnp.concatenate([w_o(g, r) for g in range(NG)], axis=0)) for r in PRODUCTS}
    for (i, n), v in _post(prods).items():
        r0 = (S - RB + i * SEG) // 16
        yb[r0:r0 + SEG // 16, :, 128 * n:128 * (n + 1)] = v.astype(bf16).reshape(SEG // 16, 16, 128)
    c_yb(S - RB, RB).start()
    wait(c_ya)
    c_yb(0, S).wait()


def _scratch():
    vmem = pltpu.VMEM
    return [
        vmem((8, 128, D), u32), vmem((16 * 256, 128), bf16), vmem((16 * 256, 128), bf16),
        vmem((1, S), bf16), vmem((1, S), bf16),
        vmem(_DFT_ROWS.shape, u32), vmem(_DFT_128.shape, f32), vmem(_DFT_TWIDDLE.shape, f32),
        vmem((16, 4, 128, 128), bf16),
        vmem((16, 2, 264, 128), f32), vmem((16, 2, 264, 128), f32), vmem((8, 128, D), u32),
        vmem((S, D), bf16), vmem((M, D), bf16),
        vmem((3 * H // 2, D, E), u32), vmem((G * H * E, 128), bf16),
        vmem((3 * NG * NPR, 128, E), bf16), vmem((NG * NPR, E, 128), bf16),
        vmem((NPR, SEG, 128), f32), vmem((3, H, RB, E), f32), vmem((3, H, SEG, E), f32),
        vmem((H, RB, E), f32), vmem((NG * NPR, SEG, E), f32), vmem((H, L, L), f32),
        vmem((NPR, L, 128), f32), vmem((NPR, SEG, 128), f32),
        vmem((RB, D), f32), vmem((S // 16, 16, D), bf16),
        pltpu.SemaphoreType.DMA((8,)), pltpu.SemaphoreType.DMA((8,)),
        pltpu.SemaphoreType.DMA((2,)), pltpu.SemaphoreType.DMA((NG,)),
    ]


@jax.jit
def pallas_concat_heads__spectral_gfnet__memory_aug_recurrent_mem_tr__prompt_kernel(
    A_x: jax.Array,
    A_w_r: jax.Array,
    A_w_i: jax.Array,
    B_x: jax.Array,
    B_mem0: jax.Array,
    B_Wq: jax.Array,
    B_Wk: jax.Array,
    B_Wv: jax.Array,
    B_Wo: jax.Array,
    B_seg_len: jax.Array,
):
    del B_seg_len
    hbm = pl.BlockSpec(memory_space=pl.ANY)
    out = pl.pallas_call(
        _kernel,
        out_shape=jax.ShapeDtypeStruct((S // 16, 16, 2 * D), bf16),
        in_specs=[hbm] * 12,
        out_specs=hbm,
        scratch_shapes=_scratch(),
        compiler_params=pltpu.CompilerParams(vmem_limit_bytes=120 * 2 ** 20),
    )(A_x.reshape(S // 16, 16, D), A_w_r.T, A_w_i.T, B_x.reshape(S, D), B_mem0.reshape(M, D),
      B_Wq, B_Wk, B_Wv, B_Wo.reshape(H * E, D), _DFT_ROWS, _DFT_128, _DFT_TWIDDLE)
    return out.reshape(1, S, 2 * D)
```

```python
import jax
import jax.numpy as jnp
import ml_dtypes
import numpy as np
from jax import lax
import jax.experimental.pallas as pl
import jax.experimental.pallas.tpu as pltpu

S, D, H, E, M, SEG = 2048, 512, 32, 128, 8, 32
L = M + SEG
G = 4
NG = H // G
RB = G * SEG
NIT = S // RB
SHIFT = (0, 3, 1)
f32, bf16, u32 = jnp.float32, jnp.bfloat16, jnp.uint32
NN = (((1,), (0,)), ((), ()))
NT = (((1,), (1,)), ((), ()))


def _dot(a, b, dims=NN):
    return lax.dot_general(a, b, dims, preferred_element_type=f32)


def _lo(u):
    return pltpu.bitcast(u << 16, f32)


def _hi(u):
    return pltpu.bitcast(u & np.uint32(0xFFFF0000), f32)


SU = {1: (((0, 0), 1), ((1, 1), 1)), 2: (((1, 0), 1), ((1, 1), 1)), 3: (((0, 0), 1),), 4: (((1, 1), 1),),
      5: (((0, 0), 1), ((0, 1), 1)), 6: (((1, 0), 1), ((0, 0), -1)), 7: (((0, 1), 1), ((1, 1), -1))}
SV = {1: (((0, 0), 1), ((1, 1), 1)), 2: (((0, 0), 1),), 3: (((0, 1), 1), ((1, 1), -1)),
      4: (((1, 0), 1), ((0, 0), -1)), 5: (((1, 1), 1),), 6: (((0, 0), 1), ((0, 1), 1)),
      7: (((1, 0), 1), ((1, 1), 1))}
SW = {(0, 0): ((1, 1), (4, 1), (7, 1), (5, -1)), (0, 1): ((3, 1), (5, 1)), (1, 0): ((2, 1), (4, 1)),
      (1, 1): ((1, 1), (3, 1), (6, 1), (2, -1))}
OWN = ((3, 1, 5, 7), (4, 1, 2, 6))


def _lin(terms):
    terms = [(v, c) for v, c in terms if v is not None]
    if not terms:
        return None
    pos = [v for v, c in terms if c > 0]
    neg = [v for v, c in terms if c < 0]
    if pos:
        acc = pos[0]
        for v in pos[1:]:
            acc = acc + v
    else:
        acc, neg = -neg[0], neg[1:]
    for v in neg:
        acc = acc - v
    return acc


def _pre(blocks, table, want):
    if not want[0]:
        return {(): blocks.get((0, 0))}
    h = 2 ** (len(want[0]) - 1)
    out = {}
    for r in sorted({w[0] for w in want}):
        sub = {(i, k): _lin([(blocks.get((a * h + i, b * h + k)), c) for (a, b), c in table[r]])
               for i in range(h) for k in range(h)}
        for rest, v in _pre(sub, table, sorted(w[1:] for w in want if w[0] == r)).items():
            out[(r,) + rest] = v
    return out


def _post(prods, row=None):
    if () in prods:
        return {(0, 0): prods[()]}
    h = 2 ** (len(next(iter(prods))) - 1)
    inner = {r: _post({w[1:]: v for w, v in prods.items() if w[0] == r}, None if row is None else row % h)
             for r in sorted({w[0] for w in prods})}
    out = {}
    for (a, b), terms in SW.items():
        for i in range(h):
            if row is None or row == a * h + i:
                for n in range(h):
                    v = _lin([(inner.get(r, {}).get((i, n)), c) for r, c in terms])
                    if v is not None:
                        out[(a * h + i, b * h + n)] = v
    return out


PRODUCTS = [(a, b) for a in range(1, 8) for b in range(1, 8)]
NPR = len(PRODUCTS)
INDEX = {r: i for i, r in enumerate(PRODUCTS)}


def _token_rows():
    phases = [[(a, b) for a in OWN[p >> 1] for b in OWN[p & 1]] for p in range(G)]
    rows = []
    for p in range(G):
        rows.append({})
        for r in phases[p]:
            users = [q for q in range(G) if r in phases[q]]
            n = SEG // len(users)
            rows[p][r] = (users.index(p) * n, (users.index(p) + 1) * n)
    return rows


def _contributors(rows):
    out = {}
    for p in range(G):
        for r, (a, b) in rows[p].items():
            for rb in range(a // 8, b // 8):
                for key in _post({r: np.zeros(1)}):
                    if p not in out.setdefault(key + (rb,), []):
                        out[key + (rb,)].append(p)
    return out


ROWS = _token_rows()
ADDS = _contributors(ROWS)


def _schedule(p, ahead):
    final = not ahead and p == G - 1
    size = {r: b - a for r, (a, b) in ROWS[p].items()}
    long_ = [r for r in size if size[r] == SEG]
    short = [r for r in size if size[r] == SEG // 2]
    tiny = [r for r in size if size[r] == SEG // 4]
    prev = (p - 1) % G
    early = [{(0, 1): (1, 3), (0, 0): (7,), (1, 1): (6,), (1, 0): (1, 4)}[(p >> s & 1, prev >> s & 1)] for s in (1, 0)]
    lead = ([r for r in long_ if r[0] in early[0] and r[1] in early[1]] + [long_[8]])[0]
    pool = [lead, short[4], tiny[0], short[5]]
    rest = [r for r in long_ if r != lead]
    groups = [(g, m) for g in range(NG) for m in ((1,) if final else (0, 1))] + [(g, 2) for g in range(NG)]
    shared = lambda i, r: [('project', g, m, r) for (g, m) in groups[i:i + 4]]
    own = lambda i, rs: [('project',) + groups[i] + (r,) for r in rs]
    rounds = []
    for i in range(len(groups)):
        a, b, c = own(i, rest[:4]), own(i, short[:4]), own(i, rest[4:])
        if i == 0:
            rounds += [shared(0, pool[0]), shared(0, pool[1]), a, shared(0, pool[2]), c, b, shared(0, pool[3])]
        else:
            rounds += [a, b, c]
        if i // 4 * 4 + 4 < len(groups):
            rounds.append(shared(i // 4 * 4 + 4, pool[i % 4]))
    if not ahead:
        items = [('project', g, m, r) for (g, m) in groups for r in size]
        head = [it for it in items if it[3][0] in early[0] and it[3][1] in early[1]][:16]
        items = head + [it for it in items if it not in head]
        rounds = [items[i:i + 4] for i in range(0, len(items), 4)]
    done = {item[1:3]: t + 1 for t, rd in enumerate(rounds) for item in rd}
    rest, mixed = list(long_), []
    fill = [r for r in size if size[r] < SEG]
    while rest or fill:
        mixed += rest[:1]
        rest = rest[1:]
        if fill and len(fill) >= len(rest) - 1:
            mixed.append(fill.pop(0))
    if not ahead:
        soon = [((3, 5), (2, 4))[p >> s & 1] for s in (1, 0)]
        mixed = sorted(mixed, key=lambda r: not (r[0] in soon[0] and r[1] in soon[1]))
    for g0 in range(0, 0 if final else NG, 4):
        rounds += [[('output', tuple(range(g0, g0 + 4)), r)] for r in mixed]
    extra = {}

    def place(t, items):
        while any(abs(t - u) < 3 for u in extra):
            t += 1
        extra[t] = items
        return t

    scored = [place(done[(g, 1)] + (6 + g % 2 if ahead else 7), [('scores', G * g + n) for n in range(G)]) for g in range(NG)]
    for g in range(NG):
        place(max(done[(g, 2)] + 6, scored[g] + 5), [('values', G * g + n) for n in range(G)])
    if final:
        rounds += [[('output', tuple(range(g0, g0 + 4)), r)] for g0 in range(0, NG, 4)
                   for r in sorted(PRODUCTS, key=lambda r: tuple((3, 5, 1, 7, 4, 2, 6).index(x) for x in r))]
    return [item for t, rd in enumerate(rounds) for item in extra.get(t, []) + rd]


def _dft_constants():
    n = np.arange(128)[None, :]
    m = np.arange(64)[:, None]
    angle = lambda k: 2 * np.pi * ((k * n) % D) / D
    even0 = np.concatenate([np.cos(angle(4 * m)), -np.sin(angle(4 * m))])
    even0[64] = np.cos(np.pi * n[0])
    even2 = np.concatenate([np.cos(angle(4 * m + 2)), -np.sin(angle(4 * m + 2))])
    cr = np.concatenate([np.cos(angle(4 * m + 1)), np.cos(angle(4 * m + 3))])
    ci = np.concatenate([-np.sin(angle(4 * m + 1)), np.sin(angle(4 * m + 3))])
    rows = np.concatenate([even0, even2, cr, cr + ci, ci - cr]).astype(np.float32).astype(ml_dtypes.bfloat16)
    rows = rows.view(np.uint16).astype(np.uint32)
    offsets = np.concatenate([128 * np.arange(16), 16 * np.arange(8), np.arange(16)])
    turn = 2 * np.pi * ((offsets[:, None] * n) % S) / S
    return rows[0::2] | (rows[1::2] << 16), np.concatenate([np.cos(turn), -np.sin(turn)]).astype(np.float32)


_DFT_ROWS, _DFT_TURNS = _dft_constants()


def _fft4(a, b, c, d, sign):
    t0 = (a[0] + c[0], a[1] + c[1])
    t1 = (a[0] - c[0], a[1] - c[1])
    t2 = (b[0] + d[0], b[1] + d[1])
    t3 = (b[0] - d[0], b[1] - d[1])
    y0 = (t0[0] + t2[0], t0[1] + t2[1])
    y2 = (t0[0] - t2[0], t0[1] - t2[1])
    p = (t1[0] + t3[1], t1[1] - t3[0])
    q = (t1[0] - t3[1], t1[1] + t3[0])
    return (y0, p, y2, q) if sign < 0 else (y0, q, y2, p)


def _rotate16(z, e, sign):
    if e == 0:
        return z
    r, i = z
    if e == 4:
        return (i, -r) if sign < 0 else (-i, r)
    h = np.float32(np.sqrt(0.5))
    if e == 2:
        return ((r + i) * h, (i - r) * h) if sign < 0 else ((r - i) * h, (r + i) * h)
    if e == 6:
        return ((i - r) * h, (r + i) * (-h)) if sign < 0 else ((r + i) * (-h), (r - i) * h)
    c = np.float32(np.cos(2 * np.pi * e / 16))
    s = np.float32(sign * np.sin(2 * np.pi * e / 16))
    return (r * c - i * s, r * s + i * c)


def _fft16(x, sign):
    col = [_fft4(x[n], x[4 + n], x[8 + n], x[12 + n], sign) for n in range(4)]
    y = [None] * 16
    for k1 in range(4):
        r = _fft4(*[_rotate16(col[n][k1], n * k1, sign) for n in range(4)], sign)
        for k2 in range(4):
            y[k1 + 4 * k2] = r[k2]
    return y


def _kernel(ax_h, wr_h, wi_h, bx_h, mem_h, wq_h, wk_h, wv_h, wo_h, rows_h, turns_h, out_h,
            ax, wr, wi, nyq_r, nyq_i, rows_v, turns, rows_inv, gmat, xs, ts, ya,
            bx, mem0, raw_qkv, raw_o, t_qkv, t_o, tok_lhs, tok, tok_late, att, att_lhs, probs, acc_o, acc_last,
            part_o, yb, sems, row_sems, filt_sems, qkv_sems, wo_sems):
    copy = pltpu.make_async_copy

    def start(copies):
        for c in copies:
            c.start()

    def wait(copies):
        for c in copies:
            c.wait()

    c_turns, c_rows = copy(turns_h, turns, sems.at[0]), copy(rows_h, rows_v, sems.at[2])
    c_ax = [copy(ax_h.bitcast(u32).at[:, j, :], ax.at[j], row_sems.at[j]) for j in range(8)]
    c_filt = [[copy(src.at[pl.ds(128 * b, 128), pl.ds(128 * k, 128)], dst.at[pl.ds(256 * k + 128 * b, 128)], filt_sems.at[b])
               for k in range(16) for src, dst in ((wr_h, wr), (wi_h, wi))] for b in range(2)]
    c_filt[0] += [copy(src.at[pl.ds(256, 1)], dst, filt_sems.at[0]) for src, dst in ((wr_h, nyq_r), (wi_h, nyq_i))]
    c_small = [copy(bx_h.at[pl.ds(0, 3 * RB)], bx.at[pl.ds(0, 3 * RB)], sems.at[1]), copy(mem_h, mem0, sems.at[1])]
    def c_qkv(m, g):
        return [copy((wq_h, wk_h, wv_h)[m].bitcast(u32).at[:, 2 * g + j, :], raw_qkv.at[m * (H // 2) + 2 * g + j],
                     qkv_sems.at[m * NG + g]) for j in range(2)]

    c_bx = copy(bx_h.at[pl.ds(3 * RB, S - 3 * RB)], bx.at[pl.ds(3 * RB, S - 3 * RB)], sems.at[5])
    c_ya = [copy(ya.at[j], out_h.bitcast(u32).at[:, j, pl.ds(0, D)], sems.at[6]) for j in range(8)]

    def c_wo(g):
        r0 = g * (G * E) if isinstance(g, int) else pl.multiple_of(g * (G * E), G * E)
        return [copy(wo_h.at[pl.ds(r0, G * E), pl.ds(128 * n, 128)], raw_o.at[pl.ds(n * H * E + r0, G * E)], wo_sems.at[g])
                for n in range(G)]

    def c_yb(row, size):
        rows = pl.ds(row // 16, size // 16)
        return copy(yb.at[rows], out_h.at[rows, :, pl.ds(D, D)], sems.at[7])

    start([c_turns, c_rows] + c_ax + c_filt[0])
    for ref in (att, acc_last, part_o):
        ref[...] = jnp.zeros(ref.shape, f32)

    c_turns.wait()
    br, bi = turns[16:24, :], turns[56:64, :]
    for s in range(16):
        cr, ci = turns[24 + s:25 + s, :], turns[64 + s:65 + s, :]
        ar, ai = br * cr - bi * ci, br * ci + bi * cr
        gr = jnp.concatenate([ar * turns[a:a + 1, :] - ai * turns[40 + a:41 + a, :] for a in range(16)], axis=0)
        gi = jnp.concatenate([ar * turns[40 + a:41 + a, :] + ai * turns[a:a + 1, :] for a in range(16)], axis=0)
        for c, v in enumerate((gr, gi, gr + gi, gi - gr)):
            gmat[s, c] = v.astype(bf16)
    g_mat = lambda s, c: pltpu.bitcast(gmat.bitcast(u32)[s, c], bf16)
    row_mat = lambda i: pltpu.bitcast(rows_v[64 * i:64 * (i + 1)], bf16)
    inv_mat = lambda i: pltpu.bitcast(rows_inv.bitcast(u32)[64 * i:64 * (i + 1)], bf16)
    c_rows.wait()
    edge = lax.broadcasted_iota(jnp.int32, (128, 128), 0) % 64 == 0
    for i in range(5):
        gain = np.float32(2.0 / (S * D))
        rows_inv[128 * i:128 * (i + 1), :] = (row_mat(i).astype(f32) * (gain if i else jnp.where(edge, gain / 2, gain))).astype(bf16)
    first = lax.broadcasted_iota(jnp.int32, (8, 128), 0) == 0

    def rfft_rows(s):
        unpack = (_lo, _hi)[s % 2]
        x0, x1, x2, x3 = (unpack(ax[s // 2, :, 128 * j:128 * (j + 1)]) for j in range(4))
        s02, s13 = x0 + x2, x1 + x3
        xa = _dot(row_mat(0), (s02 + s13).astype(bf16), NT)
        xb = _dot(row_mat(1), (s02 - s13).astype(bf16), NT)
        d0, d1 = x0 - x2, x3 - x1
        k1 = _dot(row_mat(2), (d0 + d1).astype(bf16), NT)
        er = k1 - _dot(row_mat(3), d1.astype(bf16), NT)
        ei = k1 + _dot(row_mat(4), d0.astype(bf16), NT)
        nyq = xa[64:72]
        return (jnp.concatenate([xa[:64], xb[:64], er, nyq], axis=0),
                jnp.concatenate([jnp.where(first, 0.0, nyq), xa[72:], xb[64:], ei[:64], -ei[64:]], axis=0))

    def dft128(s, re, im):
        k1 = _dot(jnp.concatenate([re[:256] + im, re[256:]], axis=0), g_mat(s, 0))
        xs[s, 0, 0:256, :] = k1[:256] - _dot(im, g_mat(s, 2))
        xs[s, 0, 256:264, :] = k1[256:]
        xs[s, 1] = k1 + _dot(re, g_mat(s, 3))

    wait(c_ax[:2])
    pending = rfft_rows(0)
    for s in range(16):
        if s == 3:
            wait(c_ax[2:4])
            start(c_filt[1] + c_small)
        if s == 7:
            wait(c_ax[4:])
            start(sum((c_qkv(0, g) for g in range(NG)), []))
        ahead = rfft_rows(s + 1) if s < 15 else None
        dft128(s, *pending)
        pending = ahead

    wait(c_filt[0])
    start(sum((c_qkv(1, g) for g in range(NG)), []))

    def spectral_filter(r0, w):
        y = _fft16([(xs[s, 0, pl.ds(r0, 8), :], xs[s, 1, pl.ds(r0, 8), :]) for s in range(16)], -1)
        z = _fft16([(a * w[k][0] - b * w[k][1], a * w[k][1] + b * w[k][0]) for k, (a, b) in enumerate(y)], +1)
        for s in range(16):
            ts[s, 0, pl.ds(r0, 8), :] = z[s][0]
            ts[s, 1, pl.ds(r0, 8), :] = z[s][1]

    nr, ni = nyq_r[...].astype(f32), nyq_i[...].astype(f32)
    spectral_filter(256, [(jnp.broadcast_to(nr[:, 128 * k:128 * (k + 1)], (8, 128)),
                           jnp.broadcast_to(ni[:, 128 * k:128 * (k + 1)], (8, 128))) for k in range(16)])
    def filter_rows(i):
        for p in range(2):
            words = [[ref.bitcast(u32).at[pl.ds(pl.multiple_of(128 * k + 16 * i, 16), 16)][pl.ds(p, 8, stride=2), :]
                      for ref in (wr, wi)] for k in range(16)]
            for g, unpack in enumerate((_lo, _hi)):
                spectral_filter(pl.multiple_of((2 * g + p) * 64 + 8 * i, 8), [(unpack(a), unpack(b)) for a, b in words])

    @pl.loop(0, 2)
    def _(half):
        pl.when(half == 1)(lambda: wait(c_filt[1]))
        for i in range(4):
            filter_rows(4 * half + i)

    start(sum((c_qkv(2, g) for g in range(NG)), []))
    wait(c_small)

    def idft128(s):
        real, imag = [], []
        for g in range(4):
            tr, ti = ts[s, 0, 64 * g:64 * (g + 1), :], ts[s, 1, 64 * g:64 * (g + 1), :]
            a, b = (-ti, tr) if g == 3 else (ti, -tr)
            if g == 0:
                a = jnp.concatenate([jnp.where(first, ts[s, 0, 256:264, :], a[:8]), a[8:]], axis=0)
                b = jnp.concatenate([jnp.where(first, ts[s, 1, 256:264, :], b[:8]), b[8:]], axis=0)
            real.append(jnp.concatenate([tr, ti], axis=1))
            imag.append(jnp.concatenate([a, b], axis=1))
        rhs = jnp.concatenate([real[0], imag[0], real[1], imag[1], real[2], real[3], imag[2], imag[3]], axis=0)
        return _dot(jnp.concatenate([g_mat(s, 0), g_mat(s, 1)], axis=1), rhs.astype(bf16), NT)

    def irfft_rows(u):
        e0, e1 = _dot(u[:, 0:128], inv_mat(0)), _dot(u[:, 128:256], inv_mat(1))
        ur, ui = u[:, 256:384], u[:, 384:512]
        k1 = _dot(ur + ui, inv_mat(2))
        d0, d1 = k1 + _dot(ui, inv_mat(4)), k1 - _dot(ur, inv_mat(3))
        p, q = e0 + e1, e0 - e1
        return [p + d0, q - d1, p - d0, q + d1]

    pending = idft128(0)
    for s in range(16):
        ahead = idft128(s + 1) if s < 15 else None
        y = [pltpu.bitcast(v.astype(bf16).astype(f32), u32) for v in irfft_rows(pending)]
        if s % 2:
            for j in range(4):
                ya[s // 2, :, 128 * j:128 * (j + 1)] = (even[j] >> 16) | y[j]
        pending, even = ahead, y

    def w_qkv(g, m, r):
        return pltpu.bitcast(t_qkv.bitcast(u32)[(m * NG + g) * NPR + INDEX[r]], bf16)

    def w_o(g, r):
        return pltpu.bitcast(t_o.bitcast(u32)[g * NPR + INDEX[r]], bf16)

    def stage_tokens(it):
        x = bx[pl.ds(it * RB if isinstance(it, int) else pl.multiple_of(it * RB, RB), RB), :].astype(f32)
        blocks = {(i, k): x[i * SEG:(i + 1) * SEG, k * 128:(k + 1) * 128] for i in range(G) for k in range(G)}
        for r, v in _pre(blocks, SU, PRODUCTS).items():
            tok_lhs[INDEX[r]] = v

    stage_tokens(0)
    start(sum((c_wo(g) for g in range(NG)), []) + [c_bx])

    def prepare(m):
        shift = SHIFT[m] if isinstance(m, int) else jnp.where(m == 0, SHIFT[0], SHIFT[1])
        for g in range(NG):
            for (i, n), v in _post({r: _dot(tok_lhs[INDEX[r]], w_qkv(g, m, r)) for r in PRODUCTS}).items():
                if i == G - 1:
                    tok_late[m, G * g + (n ^ shift)] = v
                else:
                    tok[m, G * g + (n ^ shift), i * SEG:(i + 1) * SEG, :] = v

    for m in range(3):

        @pl.loop(0, NG)
        def _(g):
            wait(c_qkv(m, g))
            for d0 in (0, 16, 48, 32, 64, 80, 112, 96):
                words = {(k, j): raw_qkv[m * (H // 2) + 2 * g + j, k * 128 + d0:k * 128 + d0 + 16, :]
                         for k in range(G) for j in range(2)}
                blocks = {(k, j ^ SHIFT[m]): (_lo, _hi)[j % 2](words[(k, j // 2)]) for k in range(G) for j in range(G)}
                for r, v in _pre(blocks, SV, PRODUCTS).items():
                    t_qkv[(m * NG + g) * NPR + INDEX[r], d0:d0 + 16, :] = v.astype(bf16)

        if m == 1:
            pl.loop(0, 2)(prepare)
        elif m == 2:
            prepare(2)

    stage_tokens(1)

    @pl.loop(0, NG)
    def _(g):
        wait(c_wo(g))
        for e0 in range(0, E, 16):
            blocks = {(k, n): pltpu.bitcast(raw_o.bitcast(u32)[pl.ds(pl.multiple_of(
                (n * H + G * g + k) * (E // 2) + e0 // 2, 8), 8), :], bf16).astype(f32) for k in range(G) for n in range(G)}
            for r, v in _pre(blocks, SV, PRODUCTS).items():
                t_o[g * NPR + INDEX[r], e0:e0 + 16, :] = v.astype(bf16)

    start(c_ya)

    ri = lax.broadcasted_iota(jnp.int32, (L, L), 0)
    ci = lax.broadcasted_iota(jnp.int32, (L, L), 1)
    allowed = (ri < M) | (ri >= ci)
    log2e = np.float32(np.log2(np.e))
    slab = lambda i, rb: slice(i * SEG + rb * 8, i * SEG + rb * 8 + 8)

    def combine(p, prods):
        for rb in range(SEG // 8):
            here = {r: prods[r][rb * 8 - a:rb * 8 + 8 - a] for r, (a, b) in ROWS[p].items() if a <= rb * 8 < b}
            for (i, n), v in _post(here).items():
                yield i, n, rb, v

    def emit(p, prods, it):
        for i, n, rb, v in combine(p, prods):
            where = (slab(i, rb), slice(128 * n, 128 * (n + 1)))
            part_o[where] = v if p == ADDS[(i, n, rb)][0] else v + part_o[where]
        if p == G - 1:
            yb[pl.ds(jnp.maximum(it, 0) * (RB // 16), RB // 16)] = part_o[...].astype(bf16).reshape(RB // 16, 16, D)

    def emit_last(it):
        emit(G - 1, {r: acc_last[INDEX[r], 0:b - a, :] for r, (a, b) in ROWS[G - 1].items()}, it)

    def segment(p, mem, held, ahead=True):
        final = not ahead and p == G - 1
        prods = list(ROWS[p])
        mem_in = _pre({(p, k): mem[:, 128 * k:128 * (k + 1)] for k in range(G)}, SU, prods)
        result, mem_qkv, mem_att, mem_out, acc = {}, {}, {}, {}, {}

        def project(g, m, r):
            a, b = ROWS[p][r]
            lhs = jnp.concatenate([tok_lhs[INDEX[r], a:b, :], mem_in[r]], axis=0) if ahead else mem_in[r]
            result[(g, m, r)] = _dot(lhs, w_qkv(g, m, r))
            if any((g, m, q) not in result for q in prods):
                return
            for n in range(G):
                for rb in range(SEG // 8):
                    if ahead and p and ADDS[(p - 1, n, rb)][-1] == p - 1:
                        h = G * g + (n ^ SHIFT[m])
                        tok[m, h, slab(p - 1, rb), :] = held.pop((m, h, p - 1, rb))
            if p == G - 2:
                for h in range(G * g, G * g + G):
                    tok[m, h, (G - 1) * SEG:G * SEG, :] = tok_late[m, h]
            res = {q: result.pop((g, m, q)) for q in prods}
            for (_, n), v in _post({q: v[-M:] for q, v in res.items()}, p).items():
                mem_qkv[(m, G * g + (n ^ SHIFT[m]))] = v
            for i, n, rb, v in combine(p, res) if ahead else ():
                h, adds = G * g + (n ^ SHIFT[m]), ADDS[(i, n, rb)]
                assert adds[-1] >= i
                if p != adds[0]:
                    v = v + held.pop((m, h, i, rb))
                if p == adds[-1] and p != i:
                    tok[m, h, slab(i, rb), :] = v
                elif p == G - 1:
                    tok_late[m, h, slab(0, rb), :] = v
                else:
                    held[(m, h, i, rb)] = v

        def rows_of(m, h):
            tokens = tok[m, h, p * SEG:(p + 1) * SEG, :]
            return tokens if final and m == 0 else jnp.concatenate([mem_qkv[(m, h)], tokens], axis=0)

        skip = M if final else 0
        earlier = lambda g, r, a, b: att_lhs[g * NPR + INDEX[r], a:b, :] if ahead else held[(g, r)][a:b]

        def scores(h):
            s = _dot(rows_of(0, h), rows_of(1, h).astype(bf16), NT) * (np.float32(E ** -0.5) * log2e)
            s = jnp.where(allowed[skip:], s, np.float32(-1e9) * log2e)
            e = jnp.exp2(s - jnp.max(s, axis=-1, keepdims=True))
            total = jnp.sum(e, axis=-1, keepdims=True)
            r = pl.reciprocal(total, approx=True)
            probs[h, skip:, :] = e * (r * (2.0 - total * r))

        def values(h):
            if p == 0 and h % G == 0:
                before = {(i, k): att[h + k, i * SEG:(i + 1) * SEG, :] for i in range(G) for k in range(G)}
                for r, v in _pre(before, SU, PRODUCTS).items():
                    if ahead:
                        att_lhs[h // G * NPR + INDEX[r]] = v
                    else:
                        held[(h // G, r)] = v
            o = _dot(probs[h, skip:, :], rows_of(2, h).astype(bf16))
            mem_att[h] = o[:M]
            if ahead:
                att[h, p * SEG:(p + 1) * SEG, :] = o[M:]
            else:
                held[('att', h, p)] = o[M - skip:]

        def output(gs, r):
            a, b = ROWS[p][r]
            for g in gs:
                if g not in mem_out:
                    mem_out[g] = _pre({(p, k): mem_att[G * g + k] for k in range(G)}, SU, prods)
            v = _dot(jnp.concatenate([jnp.concatenate([mem_out[g][r], earlier(g, r, a, b)], axis=0)
                                      for g in gs], axis=1),
                     jnp.concatenate([w_o(g, r) for g in gs], axis=0))
            if gs[0] > 0:
                v = v + acc_o[INDEX[r], 0:M + b - a, :]
            if gs[-1] < NG - 1:
                acc_o[INDEX[r], 0:M + b - a, :] = v
            acc[r] = v

        def final_output(gs, r):
            for g in gs:
                if g not in mem_out:
                    mem_out[g] = _pre({(i, k): held[('att', G * g + k, i)] for i in range(G) for k in range(G)}, SU, PRODUCTS)
            a, b = ROWS[p].get(r, (0, 0))
            rows = [jnp.concatenate([mem_out[g][r], earlier(g, r, a, b)], axis=0) if b else mem_out[g][r]
                    for g in gs]
            v = _dot(jnp.concatenate(rows, axis=1), jnp.concatenate([w_o(g, r) for g in gs], axis=0))
            acc[r] = acc[r] + v if gs[0] else v

        run = {'project': project, 'scores': scores, 'values': values, 'output': final_output if final else output}
        for item in _schedule(p, ahead):
            run[item[0]](*item[1:])
        if final:
            return acc
        if p < G - 1:
            emit(p, {r: v[M:] for r, v in acc.items()}, None)
        else:
            for r, (a, b) in ROWS[p].items():
                acc_last[INDEX[r], 0:b - a, :] = acc[r][M:]
        new = _post({r: v[:M] for r, v in acc.items()}, p)
        return jnp.concatenate([new[(p, n)] for n in range(G)], axis=1)

    def iteration(it, mem):
        @pl.when((it == 1) | ((it % 4 == 2) & (it > 2)))
        def _():
            pl.when(it == 1)(c_bx.wait)
            pl.when(it > 1)(lambda: c_yb((it - 6) * RB, 4 * RB).start())

        emit_last(it - 2)
        held = {}
        for p in range(G):
            mem = segment(p, mem, held)
        stage_tokens(jnp.minimum(it + 2, NIT - 1))
        return mem

    mem = lax.fori_loop(0, NIT - 1, iteration, mem0[...].astype(f32))

    emit_last(NIT - 3)
    c_yb((NIT - 4) * RB, 2 * RB).start()
    held = {}
    for p in range(G):
        mem = segment(p, mem, held, ahead=False)
    emit(G - 1, {r: mem[r][SEG:] for r in ROWS[G - 1]}, NIT - 2)
    for (i, n), v in _post({r: v[:SEG] for r, v in mem.items()}).items():
        r0 = (S - RB + i * SEG) // 16
        yb[r0:r0 + SEG // 16, :, 128 * n:128 * (n + 1)] = v.astype(bf16).reshape(SEG // 16, 16, 128)
    c_yb(S - 2 * RB, 2 * RB).start()
    wait(c_ya)
    c_yb(0, S).wait()


def _scratch():
    vmem = pltpu.VMEM
    return [
        vmem((8, 128, D), u32), vmem((16 * 256, 128), bf16), vmem((16 * 256, 128), bf16),
        vmem((1, S), bf16), vmem((1, S), bf16),
        vmem(_DFT_ROWS.shape, u32), vmem(_DFT_TURNS.shape, f32), vmem((5 * 128, 128), bf16),
        vmem((16, 4, 128, 128), bf16),
        vmem((16, 2, 264, 128), f32), vmem((16, 2, 264, 128), f32), vmem((8, 128, D), u32),
        vmem((S, D), bf16), vmem((M, D), bf16),
        vmem((3 * H // 2, D, E), u32), vmem((G * H * E, 128), bf16),
        vmem((3 * NG * NPR, 128, E), bf16), vmem((NG * NPR, E, 128), bf16),
        vmem((NPR, SEG, 128), f32), vmem((3, H, RB, E), f32), vmem((3, H, SEG, E), f32),
        vmem((H, RB, E), f32), vmem((NG * NPR, SEG, E), f32), vmem((H, L, L), f32),
        vmem((NPR, L, 128), f32), vmem((NPR, SEG, 128), f32),
        vmem((RB, D), f32), vmem((S // 16, 16, D), bf16),
        pltpu.SemaphoreType.DMA((8,)), pltpu.SemaphoreType.DMA((8,)),
        pltpu.SemaphoreType.DMA((2,)), pltpu.SemaphoreType.DMA((3 * NG,)),
        pltpu.SemaphoreType.DMA((NG,)),
    ]


@jax.jit
def pallas_concat_heads__spectral_gfnet__memory_aug_recurrent_mem_tr__prompt_kernel(
    A_x: jax.Array,
    A_w_r: jax.Array,
    A_w_i: jax.Array,
    B_x: jax.Array,
    B_mem0: jax.Array,
    B_Wq: jax.Array,
    B_Wk: jax.Array,
    B_Wv: jax.Array,
    B_Wo: jax.Array,
    B_seg_len: jax.Array,
):
    del B_seg_len
    hbm = pl.BlockSpec(memory_space=pl.ANY)
    out = pl.pallas_call(
        _kernel,
        out_shape=jax.ShapeDtypeStruct((S // 16, 16, 2 * D), bf16),
        in_specs=[hbm] * 11,
        out_specs=hbm,
        scratch_shapes=_scratch(),
        compiler_params=pltpu.CompilerParams(vmem_limit_bytes=120 * 2 ** 20),
    )(A_x.reshape(S // 16, 16, D), A_w_r.T, A_w_i.T, B_x.reshape(S, D), B_mem0.reshape(M, D),
      B_Wq, B_Wk, B_Wv, B_Wo.reshape(H * E, D), _DFT_ROWS, _DFT_TURNS)
    return out.reshape(1, S, 2 * D)
```

```python
import jax
import jax.numpy as jnp
import ml_dtypes
import numpy as np
from jax import lax
import jax.experimental.pallas as pl
import jax.experimental.pallas.tpu as pltpu

S, D, H, E, M, SEG = 2048, 512, 32, 128, 8, 32
L = M + SEG
G = 4
NG = H // G
RB = G * SEG
NIT = S // RB
SHIFT = (0, 3, 1)
f32, bf16, u32 = jnp.float32, jnp.bfloat16, jnp.uint32
NN = (((1,), (0,)), ((), ()))
NT = (((1,), (1,)), ((), ()))


def _dot(a, b, dims=NN):
    return lax.dot_general(a, b, dims, preferred_element_type=f32)


def _lo(u):
    return pltpu.bitcast(u << 16, f32)


def _hi(u):
    return pltpu.bitcast(u & np.uint32(0xFFFF0000), f32)


SU = {1: (((0, 0), 1), ((1, 1), 1)), 2: (((1, 0), 1), ((1, 1), 1)), 3: (((0, 0), 1),), 4: (((1, 1), 1),),
      5: (((0, 0), 1), ((0, 1), 1)), 6: (((1, 0), 1), ((0, 0), -1)), 7: (((0, 1), 1), ((1, 1), -1))}
SV = {1: (((0, 0), 1), ((1, 1), 1)), 2: (((0, 0), 1),), 3: (((0, 1), 1), ((1, 1), -1)),
      4: (((1, 0), 1), ((0, 0), -1)), 5: (((1, 1), 1),), 6: (((0, 0), 1), ((0, 1), 1)),
      7: (((1, 0), 1), ((1, 1), 1))}
SW = {(0, 0): ((1, 1), (4, 1), (7, 1), (5, -1)), (0, 1): ((3, 1), (5, 1)), (1, 0): ((2, 1), (4, 1)),
      (1, 1): ((1, 1), (3, 1), (6, 1), (2, -1))}
OWN = ((3, 1, 5, 7), (4, 1, 2, 6))


def _lin(terms):
    terms = [(v, c) for v, c in terms if v is not None]
    if not terms:
        return None
    pos = [v for v, c in terms if c > 0]
    neg = [v for v, c in terms if c < 0]
    if pos:
        acc = pos[0]
        for v in pos[1:]:
            acc = acc + v
    else:
        acc, neg = -neg[0], neg[1:]
    for v in neg:
        acc = acc - v
    return acc


def _pre(blocks, table, want):
    if not want[0]:
        return {(): blocks.get((0, 0))}
    h = 2 ** (len(want[0]) - 1)
    out = {}
    for r in sorted({w[0] for w in want}):
        sub = {(i, k): _lin([(blocks.get((a * h + i, b * h + k)), c) for (a, b), c in table[r]])
               for i in range(h) for k in range(h)}
        for rest, v in _pre(sub, table, sorted(w[1:] for w in want if w[0] == r)).items():
            out[(r,) + rest] = v
    return out


def _post(prods, row=None):
    if () in prods:
        return {(0, 0): prods[()]}
    h = 2 ** (len(next(iter(prods))) - 1)
    inner = {r: _post({w[1:]: v for w, v in prods.items() if w[0] == r}, None if row is None else row % h)
             for r in sorted({w[0] for w in prods})}
    out = {}
    for (a, b), terms in SW.items():
        for i in range(h):
            if row is None or row == a * h + i:
                for n in range(h):
                    v = _lin([(inner.get(r, {}).get((i, n)), c) for r, c in terms])
                    if v is not None:
                        out[(a * h + i, b * h + n)] = v
    return out


PRODUCTS = [(a, b) for a in range(1, 8) for b in range(1, 8)]
NPR = len(PRODUCTS)
INDEX = {r: i for i, r in enumerate(PRODUCTS)}


def _token_rows():
    phases = [[(a, b) for a in OWN[p >> 1] for b in OWN[p & 1]] for p in range(G)]
    rows = []
    for p in range(G):
        rows.append({})
        for r in phases[p]:
            users = [q for q in range(G) if r in phases[q]]
            n = SEG // len(users)
            rows[p][r] = (users.index(p) * n, (users.index(p) + 1) * n)
    return rows


def _contributors(rows):
    out = {}
    for p in range(G):
        for r, (a, b) in rows[p].items():
            for rb in range(a // 8, b // 8):
                for key in _post({r: np.zeros(1)}):
                    if p not in out.setdefault(key + (rb,), []):
                        out[key + (rb,)].append(p)
    return out


ROWS = _token_rows()
ADDS = _contributors(ROWS)


def _schedule(p, ahead):
    final = not ahead and p == G - 1
    size = {r: b - a for r, (a, b) in ROWS[p].items()}
    long_ = [r for r in size if size[r] == SEG]
    short = [r for r in size if size[r] == SEG // 2]
    tiny = [r for r in size if size[r] == SEG // 4]
    prev = (p - 1) % G
    early = [{(0, 1): (1, 3), (0, 0): (7,), (1, 1): (6,), (1, 0): (1, 4)}[(p >> s & 1, prev >> s & 1)] for s in (1, 0)]
    lead = ([r for r in long_ if r[0] in early[0] and r[1] in early[1]] + [long_[8]])[0]
    pool = [lead, short[4], tiny[0], short[5]]
    rest = [r for r in long_ if r != lead]
    groups = [(g, m) for g in range(NG) for m in ((1,) if final else (0, 1))] + [(g, 2) for g in range(NG)]
    shared = lambda i, r: [('project', g, m, r) for (g, m) in groups[i:i + 4]]
    own = lambda i, rs: [('project',) + groups[i] + (r,) for r in rs]
    rounds = []
    for i in range(len(groups)):
        a, b, c = own(i, rest[:4]), own(i, short[:4]), own(i, rest[4:])
        if i == 0:
            rounds += [shared(0, pool[0]), shared(0, pool[1]), a, shared(0, pool[2]), c, b, shared(0, pool[3])]
        else:
            rounds += [a, b, c]
        if i // 4 * 4 + 4 < len(groups):
            rounds.append(shared(i // 4 * 4 + 4, pool[i % 4]))
    if not ahead:
        items = [('project', g, m, r) for (g, m) in groups for r in size]
        head = [it for it in items if it[3][0] in early[0] and it[3][1] in early[1]][:16]
        items = head + [it for it in items if it not in head]
        rounds = [items[i:i + 4] for i in range(0, len(items), 4)]
    done = {item[1:3]: t + 1 for t, rd in enumerate(rounds) for item in rd}
    rest, mixed = list(long_), []
    fill = [r for r in size if size[r] < SEG]
    while rest or fill:
        mixed += rest[:1]
        rest = rest[1:]
        if fill and len(fill) >= len(rest) - 1:
            mixed.append(fill.pop(0))
    if not ahead:
        soon = [((3, 5), (2, 4))[p >> s & 1] for s in (1, 0)]
        mixed = sorted(mixed, key=lambda r: not (r[0] in soon[0] and r[1] in soon[1]))
    for g0 in range(0, 0 if final else NG, 4):
        rounds += [[('output', tuple(range(g0, g0 + 4)), r)] for r in mixed]
    extra = {}

    def place(t, items):
        while any(abs(t - u) < 3 for u in extra):
            t += 1
        extra[t] = items
        return t

    scored = [place(done[(g, 1)] + (6 + g % 2 if ahead else 7), [('scores', G * g + n) for n in range(G)]) for g in range(NG)]
    for g in range(NG):
        place(max(done[(g, 2)] + 6, scored[g] + 5), [('values', G * g + n) for n in range(G)])
    if final:
        order = sorted(PRODUCTS, key=lambda r: tuple((3, 5, 1, 7, 4, 2, 6).index(x) for x in r))
        rounds += [[('output', (0, 1, 2, 3), r)] for r in order]
        order = sorted(order, key=lambda r: r not in size)
        rounds += [[('output', (4, 5, 6, 7), r)] for r in order]
    return [item for t, rd in enumerate(rounds) for item in extra.get(t, []) + rd]


def _dft_constants():
    n = np.arange(128)[None, :]
    m = np.arange(64)[:, None]
    angle = lambda k: 2 * np.pi * ((k * n) % D) / D
    even0 = np.concatenate([np.cos(angle(4 * m)), -np.sin(angle(4 * m))])
    even0[64] = np.cos(np.pi * n[0])
    even2 = np.concatenate([np.cos(angle(4 * m + 2)), -np.sin(angle(4 * m + 2))])
    cr = np.concatenate([np.cos(angle(4 * m + 1)), np.cos(angle(4 * m + 3))])
    ci = np.concatenate([-np.sin(angle(4 * m + 1)), np.sin(angle(4 * m + 3))])
    rows = np.concatenate([even0, even2, cr, cr + ci, ci - cr]).astype(np.float32).astype(ml_dtypes.bfloat16)
    rows = rows.view(np.uint16).astype(np.uint32)
    offsets = np.concatenate([128 * np.arange(16), 16 * np.arange(8), np.arange(16)])
    turn = 2 * np.pi * ((offsets[:, None] * n) % S) / S
    return rows[0::2] | (rows[1::2] << 16), np.concatenate([np.cos(turn), -np.sin(turn)]).astype(np.float32)


_DFT_ROWS, _DFT_TURNS = _dft_constants()


def _fft4(a, b, c, d, sign):
    t0 = (a[0] + c[0], a[1] + c[1])
    t1 = (a[0] - c[0], a[1] - c[1])
    t2 = (b[0] + d[0], b[1] + d[1])
    t3 = (b[0] - d[0], b[1] - d[1])
    y0 = (t0[0] + t2[0], t0[1] + t2[1])
    y2 = (t0[0] - t2[0], t0[1] - t2[1])
    p = (t1[0] + t3[1], t1[1] - t3[0])
    q = (t1[0] - t3[1], t1[1] + t3[0])
    return (y0, p, y2, q) if sign < 0 else (y0, q, y2, p)


def _rotate16(z, e, sign):
    if e == 0:
        return z
    r, i = z
    if e == 4:
        return (i, -r) if sign < 0 else (-i, r)
    h = np.float32(np.sqrt(0.5))
    if e == 2:
        return ((r + i) * h, (i - r) * h) if sign < 0 else ((r - i) * h, (r + i) * h)
    if e == 6:
        return ((i - r) * h, (r + i) * (-h)) if sign < 0 else ((r + i) * (-h), (r - i) * h)
    c = np.float32(np.cos(2 * np.pi * e / 16))
    s = np.float32(sign * np.sin(2 * np.pi * e / 16))
    return (r * c - i * s, r * s + i * c)


def _fft16(x, sign):
    col = [_fft4(x[n], x[4 + n], x[8 + n], x[12 + n], sign) for n in range(4)]
    y = [None] * 16
    for k1 in range(4):
        r = _fft4(*[_rotate16(col[n][k1], n * k1, sign) for n in range(4)], sign)
        for k2 in range(4):
            y[k1 + 4 * k2] = r[k2]
    return y


def _kernel(ax_h, wr_h, wi_h, bx_h, mem_h, wq_h, wk_h, wv_h, wo_h, rows_h, turns_h, out_h,
            ax, wr, wi, nyq_r, nyq_i, rows_v, turns, rows_inv, gmat, xs, ts, ya,
            bx, mem0, raw_qkv, raw_o, t_qkv, t_o, tok_lhs, tok, tok_late, att, att_lhs, probs, acc_o, acc_last,
            part_o, yb, sems, row_sems, filt_sems, qkv_sems, wo_sems):
    copy = pltpu.make_async_copy

    def start(copies):
        for c in copies:
            c.start()

    def wait(copies):
        for c in copies:
            c.wait()

    c_turns, c_rows = copy(turns_h, turns, sems.at[0]), copy(rows_h, rows_v, sems.at[2])
    c_ax = [copy(ax_h.bitcast(u32).at[:, j, :], ax.at[j], row_sems.at[j]) for j in range(8)]
    c_filt = [[copy(src.at[pl.ds(128 * b, 128), pl.ds(128 * k, 128)], dst.at[pl.ds(256 * k + 128 * b, 128)], filt_sems.at[b])
               for k in range(16) for src, dst in ((wr_h, wr), (wi_h, wi))] for b in range(2)]
    c_filt[0] += [copy(src.at[pl.ds(256, 1)], dst, filt_sems.at[0]) for src, dst in ((wr_h, nyq_r), (wi_h, nyq_i))]
    c_small = [copy(bx_h.at[pl.ds(0, 3 * RB)], bx.at[pl.ds(0, 3 * RB)], sems.at[1]), copy(mem_h, mem0, sems.at[1])]
    def c_qkv(m, g):
        return [copy((wq_h, wk_h, wv_h)[m].bitcast(u32).at[:, 2 * g + j, :], raw_qkv.at[m * (H // 2) + 2 * g + j],
                     qkv_sems.at[m * NG + g]) for j in range(2)]

    c_bx = copy(bx_h.at[pl.ds(3 * RB, S - 3 * RB)], bx.at[pl.ds(3 * RB, S - 3 * RB)], sems.at[3])
    c_ya = [copy(ya.at[j], out_h.bitcast(u32).at[:, j, pl.ds(0, D)], sems.at[4]) for j in range(8)]

    def c_wo(g):
        r0 = g * (G * E) if isinstance(g, int) else pl.multiple_of(g * (G * E), G * E)
        return [copy(wo_h.at[pl.ds(r0, G * E), pl.ds(128 * n, 128)], raw_o.at[pl.ds(n * H * E + r0, G * E)], wo_sems.at[g])
                for n in range(G)]

    def c_yb(row, size):
        rows = pl.ds(row // 16, size // 16)
        return copy(yb.at[rows], out_h.at[rows, :, pl.ds(D, D)], sems.at[5])

    start([c_turns, c_rows] + c_ax + c_filt[0])
    for ref in (att, acc_last, part_o):
        ref[...] = jnp.zeros(ref.shape, f32)

    c_turns.wait()
    br, bi = turns[16:24, :], turns[56:64, :]
    for s in range(16):
        cr, ci = turns[24 + s:25 + s, :], turns[64 + s:65 + s, :]
        ar, ai = br * cr - bi * ci, br * ci + bi * cr
        gr = jnp.concatenate([ar * turns[a:a + 1, :] - ai * turns[40 + a:41 + a, :] for a in range(16)], axis=0)
        gi = jnp.concatenate([ar * turns[40 + a:41 + a, :] + ai * turns[a:a + 1, :] for a in range(16)], axis=0)
        for c, v in enumerate((gr, gi, gr + gi, gi - gr)):
            gmat[s, c] = v.astype(bf16)
    g_mat = lambda s, c: pltpu.bitcast(gmat.bitcast(u32)[s, c], bf16)
    row_mat = lambda i: pltpu.bitcast(rows_v[64 * i:64 * (i + 1)], bf16)
    inv_mat = lambda i: pltpu.bitcast(rows_inv.bitcast(u32)[64 * i:64 * (i + 1)], bf16)
    c_rows.wait()
    edge = lax.broadcasted_iota(jnp.int32, (128, 128), 0) % 64 == 0
    for i in range(5):
        gain = np.float32(2.0 / (S * D))
        rows_inv[128 * i:128 * (i + 1), :] = (row_mat(i).astype(f32) * (gain if i else jnp.where(edge, gain / 2, gain))).astype(bf16)
    first = lax.broadcasted_iota(jnp.int32, (8, 128), 0) == 0

    def rfft_rows(s):
        unpack = (_lo, _hi)[s % 2]
        x0, x1, x2, x3 = (unpack(ax[s // 2, :, 128 * j:128 * (j + 1)]) for j in range(4))
        s02, s13 = x0 + x2, x1 + x3
        xa = _dot(row_mat(0), (s02 + s13).astype(bf16), NT)
        xb = _dot(row_mat(1), (s02 - s13).astype(bf16), NT)
        d0, d1 = x0 - x2, x3 - x1
        k1 = _dot(row_mat(2), (d0 + d1).astype(bf16), NT)
        er = k1 - _dot(row_mat(3), d1.astype(bf16), NT)
        ei = k1 + _dot(row_mat(4), d0.astype(bf16), NT)
        nyq = xa[64:72]
        return (jnp.concatenate([xa[:64], xb[:64], er, nyq], axis=0),
                jnp.concatenate([jnp.where(first, 0.0, nyq), xa[72:], xb[64:], ei[:64], -ei[64:]], axis=0))

    def dft128(s, re, im):
        k1 = _dot(jnp.concatenate([re[:256] + im, re[256:]], axis=0), g_mat(s, 0))
        xs[s, 0, 0:256, :] = k1[:256] - _dot(im, g_mat(s, 2))
        xs[s, 0, 256:264, :] = k1[256:]
        xs[s, 1] = k1 + _dot(re, g_mat(s, 3))

    wait(c_ax[:2])
    pending = rfft_rows(0)
    for s in range(16):
        if s == 3:
            wait(c_ax[2:4])
            start(c_filt[1] + c_small)
        if s == 7:
            wait(c_ax[4:])
            start(sum((c_qkv(0, g) for g in range(NG)), []))
        ahead = rfft_rows(s + 1) if s < 15 else None
        dft128(s, *pending)
        pending = ahead

    wait(c_filt[0])
    start(sum((c_qkv(1, g) for g in range(NG)), []))

    def spectral_filter(r0, w):
        y = _fft16([(xs[s, 0, pl.ds(r0, 8), :], xs[s, 1, pl.ds(r0, 8), :]) for s in range(16)], -1)
        z = _fft16([(a * w[k][0] - b * w[k][1], a * w[k][1] + b * w[k][0]) for k, (a, b) in enumerate(y)], +1)
        for s in range(16):
            ts[s, 0, pl.ds(r0, 8), :] = z[s][0]
            ts[s, 1, pl.ds(r0, 8), :] = z[s][1]

    nr, ni = nyq_r[...].astype(f32), nyq_i[...].astype(f32)
    spectral_filter(256, [(jnp.broadcast_to(nr[:, 128 * k:128 * (k + 1)], (8, 128)),
                           jnp.broadcast_to(ni[:, 128 * k:128 * (k + 1)], (8, 128))) for k in range(16)])
    def filter_rows(i):
        for p in range(2):
            words = [[ref.bitcast(u32).at[pl.ds(pl.multiple_of(128 * k + 16 * i, 16), 16)][pl.ds(p, 8, stride=2), :]
                      for ref in (wr, wi)] for k in range(16)]
            for g, unpack in enumerate((_lo, _hi)):
                spectral_filter(pl.multiple_of((2 * g + p) * 64 + 8 * i, 8), [(unpack(a), unpack(b)) for a, b in words])

    @pl.loop(0, 2)
    def _(half):
        pl.when(half == 1)(lambda: wait(c_filt[1]))
        for i in range(4):
            filter_rows(4 * half + i)

    start(sum((c_qkv(2, g) for g in range(NG)), []))
    wait(c_small)

    def idft128(s):
        real, imag = [], []
        for g in range(4):
            tr, ti = ts[s, 0, 64 * g:64 * (g + 1), :], ts[s, 1, 64 * g:64 * (g + 1), :]
            a, b = (-ti, tr) if g == 3 else (ti, -tr)
            if g == 0:
                a = jnp.concatenate([jnp.where(first, ts[s, 0, 256:264, :], a[:8]), a[8:]], axis=0)
                b = jnp.concatenate([jnp.where(first, ts[s, 1, 256:264, :], b[:8]), b[8:]], axis=0)
            real.append(jnp.concatenate([tr, ti], axis=1))
            imag.append(jnp.concatenate([a, b], axis=1))
        rhs = jnp.concatenate([real[0], imag[0], real[1], imag[1], real[2], real[3], imag[2], imag[3]], axis=0)
        return _dot(jnp.concatenate([g_mat(s, 0), g_mat(s, 1)], axis=1), rhs.astype(bf16), NT)

    def irfft_rows(u):
        e0, e1 = _dot(u[:, 0:128], inv_mat(0)), _dot(u[:, 128:256], inv_mat(1))
        ur, ui = u[:, 256:384], u[:, 384:512]
        k1 = _dot(ur + ui, inv_mat(2))
        d0, d1 = k1 + _dot(ui, inv_mat(4)), k1 - _dot(ur, inv_mat(3))
        p, q = e0 + e1, e0 - e1
        return [p + d0, q - d1, p - d0, q + d1]

    pending = idft128(0)
    for s in range(16):
        ahead = idft128(s + 1) if s < 15 else None
        y = [pltpu.bitcast(v.astype(bf16).astype(f32), u32) for v in irfft_rows(pending)]
        if s % 2:
            for j in range(4):
                ya[s // 2, :, 128 * j:128 * (j + 1)] = (even[j] >> 16) | y[j]
        pending, even = ahead, y

    def w_qkv(g, m, r):
        return pltpu.bitcast(t_qkv.bitcast(u32)[(m * NG + g) * NPR + INDEX[r]], bf16)

    def w_o(g, r):
        return pltpu.bitcast(t_o.bitcast(u32)[g * NPR + INDEX[r]], bf16)

    def stage_tokens(it):
        x = bx[pl.ds(it * RB if isinstance(it, int) else pl.multiple_of(it * RB, RB), RB), :].astype(f32)
        blocks = {(i, k): x[i * SEG:(i + 1) * SEG, k * 128:(k + 1) * 128] for i in range(G) for k in range(G)}
        for r, v in _pre(blocks, SU, PRODUCTS).items():
            tok_lhs[INDEX[r]] = v

    stage_tokens(0)
    start(sum((c_wo(g) for g in range(NG)), []) + [c_bx])

    def prepare(m):
        shift = SHIFT[m] if isinstance(m, int) else jnp.where(m == 0, SHIFT[0], SHIFT[1])
        for g in range(NG):
            for (i, n), v in _post({r: _dot(tok_lhs[INDEX[r]], w_qkv(g, m, r)) for r in PRODUCTS}).items():
                if i == G - 1:
                    tok_late[m, G * g + (n ^ shift)] = v
                else:
                    tok[m, G * g + (n ^ shift), i * SEG:(i + 1) * SEG, :] = v

    for m in range(3):

        @pl.loop(0, NG)
        def _(g):
            wait(c_qkv(m, g))
            for d0 in (0, 16, 48, 32, 64, 80, 112, 96):
                words = {(k, j): raw_qkv[m * (H // 2) + 2 * g + j, k * 128 + d0:k * 128 + d0 + 16, :]
                         for k in range(G) for j in range(2)}
                blocks = {(k, j ^ SHIFT[m]): (_lo, _hi)[j % 2](words[(k, j // 2)]) for k in range(G) for j in range(G)}
                for r, v in _pre(blocks, SV, PRODUCTS).items():
                    t_qkv[(m * NG + g) * NPR + INDEX[r], d0:d0 + 16, :] = v.astype(bf16)

        if m == 1:
            pl.loop(0, 2)(prepare)
        elif m == 2:
            prepare(2)

    stage_tokens(1)

    @pl.loop(0, NG)
    def _(g):
        wait(c_wo(g))
        for e0 in range(0, E, 16):
            blocks = {(k, n): pltpu.bitcast(raw_o.bitcast(u32)[pl.ds(pl.multiple_of(
                (n * H + G * g + k) * (E // 2) + e0 // 2, 8), 8), :], bf16).astype(f32) for k in range(G) for n in range(G)}
            for r, v in _pre(blocks, SV, PRODUCTS).items():
                t_o[g * NPR + INDEX[r], e0:e0 + 16, :] = v.astype(bf16)

    start(c_ya)

    ri = lax.broadcasted_iota(jnp.int32, (L, L), 0)
    ci = lax.broadcasted_iota(jnp.int32, (L, L), 1)
    allowed = (ri < M) | (ri >= ci)
    log2e = np.float32(np.log2(np.e))
    slab = lambda i, rb: slice(i * SEG + rb * 8, i * SEG + rb * 8 + 8)

    def combine(p, prods):
        for rb in range(SEG // 8):
            here = {r: prods[r][rb * 8 - a:rb * 8 + 8 - a] for r, (a, b) in ROWS[p].items() if a <= rb * 8 < b}
            for (i, n), v in _post(here).items():
                yield i, n, rb, v

    def emit(p, prods, it):
        for i, n, rb, v in combine(p, prods):
            where = (slab(i, rb), slice(128 * n, 128 * (n + 1)))
            part_o[where] = v if p == ADDS[(i, n, rb)][0] else v + part_o[where]
        if p == G - 1:
            yb[pl.ds(jnp.maximum(it, 0) * (RB // 16), RB // 16)] = part_o[...].astype(bf16).reshape(RB // 16, 16, D)

    def emit_last(it):
        emit(G - 1, {r: acc_last[INDEX[r], 0:b - a, :] for r, (a, b) in ROWS[G - 1].items()}, it)

    def segment(p, mem, held, ahead=True):
        final = not ahead and p == G - 1
        prods = list(ROWS[p])
        mem_in = _pre({(p, k): mem[:, 128 * k:128 * (k + 1)] for k in range(G)}, SU, prods)
        result, mem_qkv, mem_att, mem_out, acc = {}, {}, {}, {}, {}

        def project(g, m, r):
            a, b = ROWS[p][r]
            lhs = jnp.concatenate([tok_lhs[INDEX[r], a:b, :], mem_in[r]], axis=0) if ahead else mem_in[r]
            result[(g, m, r)] = _dot(lhs, w_qkv(g, m, r))
            if any((g, m, q) not in result for q in prods):
                return
            for n in range(G):
                for rb in range(SEG // 8):
                    if ahead and p and ADDS[(p - 1, n, rb)][-1] == p - 1:
                        h = G * g + (n ^ SHIFT[m])
                        tok[m, h, slab(p - 1, rb), :] = held.pop((m, h, p - 1, rb))
            if p == G - 2:
                for h in range(G * g, G * g + G):
                    tok[m, h, (G - 1) * SEG:G * SEG, :] = tok_late[m, h]
            res = {q: result.pop((g, m, q)) for q in prods}
            for (_, n), v in _post({q: v[-M:] for q, v in res.items()}, p).items():
                mem_qkv[(m, G * g + (n ^ SHIFT[m]))] = v
            for i, n, rb, v in combine(p, res) if ahead else ():
                h, adds = G * g + (n ^ SHIFT[m]), ADDS[(i, n, rb)]
                assert adds[-1] >= i
                if p != adds[0]:
                    v = v + held.pop((m, h, i, rb))
                if p == adds[-1] and p != i:
                    tok[m, h, slab(i, rb), :] = v
                elif p == G - 1:
                    tok_late[m, h, slab(0, rb), :] = v
                else:
                    held[(m, h, i, rb)] = v

        def rows_of(m, h):
            tokens = tok[m, h, p * SEG:(p + 1) * SEG, :]
            return tokens if final and m == 0 else jnp.concatenate([mem_qkv[(m, h)], tokens], axis=0)

        skip = M if final else 0
        earlier = lambda g, r, a, b: att_lhs[g * NPR + INDEX[r], a:b, :] if ahead else held[(g, r)][a:b]

        def scores(h):
            s = _dot(rows_of(0, h), rows_of(1, h).astype(bf16), NT) * (np.float32(E ** -0.5) * log2e)
            s = jnp.where(allowed[skip:], s, np.float32(-1e9) * log2e)
            e = jnp.exp2(s - jnp.max(s, axis=-1, keepdims=True))
            total = jnp.sum(e, axis=-1, keepdims=True)
            r = pl.reciprocal(total, approx=True)
            probs[h, skip:, :] = e * (r * (2.0 - total * r))

        def values(h):
            if p == 0 and h % G == 0:
                before = {(i, k): att[h + k, i * SEG:(i + 1) * SEG, :] for i in range(G) for k in range(G)}
                for r, v in _pre(before, SU, PRODUCTS).items():
                    if ahead:
                        att_lhs[h // G * NPR + INDEX[r]] = v
                    else:
                        held[(h // G, r)] = v
            o = _dot(probs[h, skip:, :], rows_of(2, h).astype(bf16))
            mem_att[h] = o[:M]
            if ahead:
                att[h, p * SEG:(p + 1) * SEG, :] = o[M:]
            else:
                held[('att', h, p)] = o[M - skip:]

        def output(gs, r):
            a, b = ROWS[p][r]
            for g in gs:
                if g not in mem_out:
                    mem_out[g] = _pre({(p, k): mem_att[G * g + k] for k in range(G)}, SU, prods)
            v = _dot(jnp.concatenate([jnp.concatenate([mem_out[g][r], earlier(g, r, a, b)], axis=0)
                                      for g in gs], axis=1),
                     jnp.concatenate([w_o(g, r) for g in gs], axis=0))
            if gs[0] > 0:
                v = v + acc_o[INDEX[r], 0:M + b - a, :]
            if gs[-1] < NG - 1:
                acc_o[INDEX[r], 0:M + b - a, :] = v
            acc[r] = v

        def final_output(gs, r):
            for g in gs:
                if g not in mem_out:
                    mem_out[g] = _pre({(i, k): held[('att', G * g + k, i)] for i in range(G) for k in range(G)}, SU, PRODUCTS)
            a, b = ROWS[p].get(r, (0, 0))
            rows = [jnp.concatenate([mem_out[g][r], earlier(g, r, a, b)], axis=0) if b else mem_out[g][r]
                    for g in gs]
            v = _dot(jnp.concatenate(rows, axis=1), jnp.concatenate([w_o(g, r) for g in gs], axis=0))
            acc[r] = acc[r] + v if gs[0] else v
            if gs[0] and b:
                result[r] = acc[r][SEG:]
                if all(q in result for q in prods):
                    emit(p, result, NIT - 2)
                    c_yb(S - 2 * RB, RB).start()

        run = {'project': project, 'scores': scores, 'values': values, 'output': final_output if final else output}
        for item in _schedule(p, ahead):
            run[item[0]](*item[1:])
        if final:
            return acc
        if p < G - 1:
            emit(p, {r: v[M:] for r, v in acc.items()}, None)
        else:
            for r, (a, b) in ROWS[p].items():
                acc_last[INDEX[r], 0:b - a, :] = acc[r][M:]
        new = _post({r: v[:M] for r, v in acc.items()}, p)
        return jnp.concatenate([new[(p, n)] for n in range(G)], axis=1)

    def iteration(it, mem):
        @pl.when((it == 1) | ((it % 4 == 2) & (it > 2)))
        def _():
            pl.when(it == 1)(c_bx.wait)
            pl.when(it > 1)(lambda: c_yb((it - 6) * RB, 4 * RB).start())

        emit_last(it - 2)
        held = {}
        for p in range(G):
            mem = segment(p, mem, held)
        stage_tokens(jnp.minimum(it + 2, NIT - 1))
        return mem

    mem = lax.fori_loop(0, NIT - 1, iteration, mem0[...].astype(f32))

    emit_last(NIT - 3)
    c_yb((NIT - 4) * RB, 2 * RB).start()
    held = {}
    for p in range(G - 1):
        mem = segment(p, mem, held, ahead=False)
    for (i, n), v in _post({r: v[:SEG] for r, v in segment(G - 1, mem, held, ahead=False).items()}).items():
        r0 = (S - RB + i * SEG) // 16
        yb[r0:r0 + SEG // 16, :, 128 * n:128 * (n + 1)] = v.astype(bf16).reshape(SEG // 16, 16, 128)
    c_yb(S - RB, RB).start()
    wait(c_ya)
    c_yb(0, S).wait()


def _scratch():
    vmem = pltpu.VMEM
    return [
        vmem((8, 128, D), u32), vmem((16 * 256, 128), bf16), vmem((16 * 256, 128), bf16),
        vmem((1, S), bf16), vmem((1, S), bf16),
        vmem(_DFT_ROWS.shape, u32), vmem(_DFT_TURNS.shape, f32), vmem((5 * 128, 128), bf16),
        vmem((16, 4, 128, 128), bf16),
        vmem((16, 2, 264, 128), f32), vmem((16, 2, 264, 128), f32), vmem((8, 128, D), u32),
        vmem((S, D), bf16), vmem((M, D), bf16),
        vmem((3 * H // 2, D, E), u32), vmem((G * H * E, 128), bf16),
        vmem((3 * NG * NPR, 128, E), bf16), vmem((NG * NPR, E, 128), bf16),
        vmem((NPR, SEG, 128), f32), vmem((3, H, RB, E), f32), vmem((3, H, SEG, E), f32),
        vmem((H, RB, E), f32), vmem((NG * NPR, SEG, E), f32), vmem((H, L, L), f32),
        vmem((NPR, L, 128), f32), vmem((NPR, SEG, 128), f32),
        vmem((RB, D), f32), vmem((S // 16, 16, D), bf16),
        pltpu.SemaphoreType.DMA((6,)), pltpu.SemaphoreType.DMA((8,)),
        pltpu.SemaphoreType.DMA((2,)), pltpu.SemaphoreType.DMA((3 * NG,)),
        pltpu.SemaphoreType.DMA((NG,)),
    ]


@jax.jit
def pallas_concat_heads__spectral_gfnet__memory_aug_recurrent_mem_tr__prompt_kernel(
    A_x: jax.Array,
    A_w_r: jax.Array,
    A_w_i: jax.Array,
    B_x: jax.Array,
    B_mem0: jax.Array,
    B_Wq: jax.Array,
    B_Wk: jax.Array,
    B_Wv: jax.Array,
    B_Wo: jax.Array,
    B_seg_len: jax.Array,
):
    del B_seg_len
    hbm = pl.BlockSpec(memory_space=pl.ANY)
    out = pl.pallas_call(
        _kernel,
        out_shape=jax.ShapeDtypeStruct((S // 16, 16, 2 * D), bf16),
        in_specs=[hbm] * 11,
        out_specs=hbm,
        scratch_shapes=_scratch(),
        compiler_params=pltpu.CompilerParams(vmem_limit_bytes=120 * 2 ** 20),
    )(A_x.reshape(S // 16, 16, D), A_w_r.T, A_w_i.T, B_x.reshape(S, D), B_mem0.reshape(M, D),
      B_Wq, B_Wk, B_Wv, B_Wo.reshape(H * E, D), _DFT_ROWS, _DFT_TURNS)
    return out.reshape(1, S, 2 * D)
```

```python
import jax
import jax.numpy as jnp
import ml_dtypes
import numpy as np
from jax import lax
import jax.experimental.pallas as pl
import jax.experimental.pallas.tpu as pltpu

S, D, H, E, M, SEG = 2048, 512, 32, 128, 8, 32
L = M + SEG
G = 4
NG = H // G
RB = G * SEG
NIT = S // RB
SHIFT = (0, 3, 1)
f32, bf16, u32 = jnp.float32, jnp.bfloat16, jnp.uint32
NN = (((1,), (0,)), ((), ()))
NT = (((1,), (1,)), ((), ()))


def _dot(a, b, dims=NN):
    return lax.dot_general(a, b, dims, preferred_element_type=f32)


def _lo(u):
    return pltpu.bitcast(u << 16, f32)


def _hi(u):
    return pltpu.bitcast(u & np.uint32(0xFFFF0000), f32)


SU = {1: (((0, 0), 1), ((1, 1), 1)), 2: (((1, 0), 1), ((1, 1), 1)), 3: (((0, 0), 1),), 4: (((1, 1), 1),),
      5: (((0, 0), 1), ((0, 1), 1)), 6: (((1, 0), 1), ((0, 0), -1)), 7: (((0, 1), 1), ((1, 1), -1))}
SV = {1: (((0, 0), 1), ((1, 1), 1)), 2: (((0, 0), 1),), 3: (((0, 1), 1), ((1, 1), -1)),
      4: (((1, 0), 1), ((0, 0), -1)), 5: (((1, 1), 1),), 6: (((0, 0), 1), ((0, 1), 1)),
      7: (((1, 0), 1), ((1, 1), 1))}
SW = {(0, 0): ((1, 1), (4, 1), (7, 1), (5, -1)), (0, 1): ((3, 1), (5, 1)), (1, 0): ((2, 1), (4, 1)),
      (1, 1): ((1, 1), (3, 1), (6, 1), (2, -1))}
OWN = ((3, 1, 5, 7), (4, 1, 2, 6))


def _lin(terms):
    terms = [(v, c) for v, c in terms if v is not None]
    if not terms:
        return None
    pos = [v for v, c in terms if c > 0]
    neg = [v for v, c in terms if c < 0]
    if pos:
        acc = pos[0]
        for v in pos[1:]:
            acc = acc + v
    else:
        acc, neg = -neg[0], neg[1:]
    for v in neg:
        acc = acc - v
    return acc


def _pre(blocks, table, want):
    if not want[0]:
        return {(): blocks.get((0, 0))}
    h = 2 ** (len(want[0]) - 1)
    out = {}
    for r in sorted({w[0] for w in want}):
        sub = {(i, k): _lin([(blocks.get((a * h + i, b * h + k)), c) for (a, b), c in table[r]])
               for i in range(h) for k in range(h)}
        for rest, v in _pre(sub, table, sorted(w[1:] for w in want if w[0] == r)).items():
            out[(r,) + rest] = v
    return out


def _post(prods, row=None):
    if () in prods:
        return {(0, 0): prods[()]}
    h = 2 ** (len(next(iter(prods))) - 1)
    inner = {r: _post({w[1:]: v for w, v in prods.items() if w[0] == r}, None if row is None else row % h)
             for r in sorted({w[0] for w in prods})}
    out = {}
    for (a, b), terms in SW.items():
        for i in range(h):
            if row is None or row == a * h + i:
                for n in range(h):
                    v = _lin([(inner.get(r, {}).get((i, n)), c) for r, c in terms])
                    if v is not None:
                        out[(a * h + i, b * h + n)] = v
    return out


PRODUCTS = [(a, b) for a in range(1, 8) for b in range(1, 8)]
NPR = len(PRODUCTS)
INDEX = {r: i for i, r in enumerate(PRODUCTS)}


def _token_rows():
    phases = [[(a, b) for a in OWN[p >> 1] for b in OWN[p & 1]] for p in range(G)]
    rows = []
    for p in range(G):
        rows.append({})
        for r in phases[p]:
            users = [q for q in range(G) if r in phases[q]]
            n = SEG // len(users)
            rows[p][r] = (users.index(p) * n, (users.index(p) + 1) * n)
    return rows


def _contributors(rows):
    out = {}
    for p in range(G):
        for r, (a, b) in rows[p].items():
            for rb in range(a // 8, b // 8):
                for key in _post({r: np.zeros(1)}):
                    if p not in out.setdefault(key + (rb,), []):
                        out[key + (rb,)].append(p)
    return out


ROWS = _token_rows()
ADDS = _contributors(ROWS)


def _schedule(p, ahead):
    final = not ahead and p == G - 1
    size = {r: b - a for r, (a, b) in ROWS[p].items()}
    long_ = [r for r in size if size[r] == SEG]
    short = [r for r in size if size[r] == SEG // 2]
    tiny = [r for r in size if size[r] == SEG // 4]
    prev = (p - 1) % G
    early = [{(0, 1): (1, 3), (0, 0): (7,), (1, 1): (6,), (1, 0): (1, 4)}[(p >> s & 1, prev >> s & 1)] for s in (1, 0)]
    lead = ([r for r in long_ if r[0] in early[0] and r[1] in early[1]] + [long_[8]])[0]
    pool = [lead, short[4], tiny[0], short[5]]
    rest = [r for r in long_ if r != lead]
    groups = [(g, m) for g in range(NG) for m in ((1,) if final else (0, 1))] + [(g, 2) for g in range(NG)]
    shared = lambda i, r: [('project', g, m, r) for (g, m) in groups[i:i + 4]]
    own = lambda i, rs: [('project',) + groups[i] + (r,) for r in rs]
    rounds = []
    for i in range(len(groups)):
        a, b, c = own(i, rest[:4]), own(i, short[:4]), own(i, rest[4:])
        if i == 0:
            rounds += [shared(0, pool[0]), shared(0, pool[1]), a, shared(0, pool[2]), c, b, shared(0, pool[3])]
        else:
            rounds += [a, b, c]
        if i // 4 * 4 + 4 < len(groups):
            rounds.append(shared(i // 4 * 4 + 4, pool[i % 4]))
    if not ahead:
        items = [('project', g, m, r) for (g, m) in groups for r in size]
        head = [it for it in items if it[3][0] in early[0] and it[3][1] in early[1]][:16]
        items = head + [it for it in items if it not in head]
        rounds = [items[i:i + 4] for i in range(0, len(items), 4)]
    done = {item[1:3]: t + 1 for t, rd in enumerate(rounds) for item in rd}
    rest, mixed = list(long_), []
    fill = [r for r in size if size[r] < SEG]
    while rest or fill:
        mixed += rest[:1]
        rest = rest[1:]
        if fill and len(fill) >= len(rest) - 1:
            mixed.append(fill.pop(0))
    if not ahead:
        soon = [((3, 5), (2, 4))[p >> s & 1] for s in (1, 0)]
        mixed = sorted(mixed, key=lambda r: not (r[0] in soon[0] and r[1] in soon[1]))
    for g0 in range(0, 0 if final else NG, 4):
        rounds += [[('output', tuple(range(g0, g0 + 4)), r)] for r in mixed]
    extra = {}

    def place(t, items):
        while any(abs(t - u) < 3 for u in extra):
            t += 1
        extra[t] = items
        return t

    scored = [place(done[(g, 1)] + (6 + g % 2 if ahead else 7), [('scores', G * g + n) for n in range(G)]) for g in range(NG)]
    for g in range(NG):
        place(max(done[(g, 2)] + 6, scored[g] + 5), [('values', G * g + n) for n in range(G)])
    if final:
        order = sorted(PRODUCTS, key=lambda r: tuple((3, 5, 1, 7, 4, 2, 6).index(x) for x in r))
        rounds += [[('output', (0, 1, 2, 3), r)] for r in order]
        order = sorted(order, key=lambda r: r not in size)
        rounds += [[('output', (4, 5, 6, 7), r)] for r in order]
    return [item for t, rd in enumerate(rounds) for item in extra.get(t, []) + rd]


def _dft_constants():
    n = np.arange(128)[None, :]
    m = np.arange(64)[:, None]
    angle = lambda k: 2 * np.pi * ((k * n) % D) / D
    even0 = np.concatenate([np.cos(angle(4 * m)), -np.sin(angle(4 * m))])
    even0[64] = np.cos(np.pi * n[0])
    even2 = np.concatenate([np.cos(angle(4 * m + 2)), -np.sin(angle(4 * m + 2))])
    cr = np.concatenate([np.cos(angle(4 * m + 1)), np.cos(angle(4 * m + 3))])
    ci = np.concatenate([-np.sin(angle(4 * m + 1)), np.sin(angle(4 * m + 3))])
    rows = np.concatenate([even0, even2, cr, cr + ci, ci - cr]).astype(np.float32).astype(ml_dtypes.bfloat16)
    rows = rows.view(np.uint16).astype(np.uint32)
    offsets = np.concatenate([128 * np.arange(16), 16 * np.arange(8), np.arange(16)])
    turn = 2 * np.pi * ((offsets[:, None] * n) % S) / S
    return rows[0::2] | (rows[1::2] << 16), np.concatenate([np.cos(turn), -np.sin(turn)]).astype(np.float32)


_DFT_ROWS, _DFT_TURNS = _dft_constants()


def _fft4(a, b, c, d, sign):
    t0 = (a[0] + c[0], a[1] + c[1])
    t1 = (a[0] - c[0], a[1] - c[1])
    t2 = (b[0] + d[0], b[1] + d[1])
    t3 = (b[0] - d[0], b[1] - d[1])
    y0 = (t0[0] + t2[0], t0[1] + t2[1])
    y2 = (t0[0] - t2[0], t0[1] - t2[1])
    p = (t1[0] + t3[1], t1[1] - t3[0])
    q = (t1[0] - t3[1], t1[1] + t3[0])
    return (y0, p, y2, q) if sign < 0 else (y0, q, y2, p)


def _rotate16(z, e, sign):
    if e == 0:
        return z
    r, i = z
    if e == 4:
        return (i, -r) if sign < 0 else (-i, r)
    h = np.float32(np.sqrt(0.5))
    if e == 2:
        return ((r + i) * h, (i - r) * h) if sign < 0 else ((r - i) * h, (r + i) * h)
    if e == 6:
        return ((i - r) * h, (r + i) * (-h)) if sign < 0 else ((r + i) * (-h), (r - i) * h)
    c = np.float32(np.cos(2 * np.pi * e / 16))
    s = np.float32(sign * np.sin(2 * np.pi * e / 16))
    return (r * c - i * s, r * s + i * c)


def _fft16(x, sign):
    col = [_fft4(x[n], x[4 + n], x[8 + n], x[12 + n], sign) for n in range(4)]
    y = [None] * 16
    for k1 in range(4):
        r = _fft4(*[_rotate16(col[n][k1], n * k1, sign) for n in range(4)], sign)
        for k2 in range(4):
            y[k1 + 4 * k2] = r[k2]
    return y


def _kernel(ax_h, wr_h, wi_h, bx_h, mem_h, wq_h, wk_h, wv_h, wo_h, rows_h, turns_h, out_h,
            ax, wr, wi, nyq_r, nyq_i, rows_v, turns, rows_inv, gmat, xs, ts, ya,
            bx, mem0, raw_qkv, raw_o, t_qkv, t_o, tok_lhs, tok, tok_late, att, att_lhs, probs, acc_o, acc_last,
            part_o, yb, sems, row_sems, filt_sems, qkv_sems, wo_sems):
    copy = pltpu.make_async_copy

    def start(copies):
        for c in copies:
            c.start()

    def wait(copies):
        for c in copies:
            c.wait()

    c_turns, c_rows = copy(turns_h, turns, sems.at[0]), copy(rows_h, rows_v, sems.at[2])
    c_ax = [copy(ax_h.bitcast(u32).at[:, j, :], ax.at[j], row_sems.at[j]) for j in range(8)]
    c_filt = [[copy(src.at[pl.ds(128 * b, 128), pl.ds(128 * k, 128)], dst.at[pl.ds(256 * k + 128 * b, 128)], filt_sems.at[b])
               for k in range(16) for src, dst in ((wr_h, wr), (wi_h, wi))] for b in range(2)]
    c_filt[0] += [copy(src.at[pl.ds(256, 1)], dst, filt_sems.at[0]) for src, dst in ((wr_h, nyq_r), (wi_h, nyq_i))]
    c_small = [copy(bx_h.at[pl.ds(0, 3 * RB)], bx.at[pl.ds(0, 3 * RB)], sems.at[1]), copy(mem_h, mem0, sems.at[1])]
    def c_qkv(m, g):
        return [copy((wq_h, wk_h, wv_h)[m].bitcast(u32).at[:, 2 * g + j, :], raw_qkv.at[m * (H // 2) + 2 * g + j],
                     qkv_sems.at[m * NG + g]) for j in range(2)]

    c_bx = copy(bx_h.at[pl.ds(3 * RB, S - 3 * RB)], bx.at[pl.ds(3 * RB, S - 3 * RB)], sems.at[3])
    c_ya = [copy(ya.at[j], out_h.bitcast(u32).at[:, j, pl.ds(0, D)], sems.at[4]) for j in range(8)]

    wo_cuts = (0, 5, NG - 1, NG)
    c_wo = [[copy(wo_h.at[pl.ds(a * G * E, (b - a) * G * E), pl.ds(128 * c, 128)],
                  raw_o.at[pl.ds((c * H + a * G) * E, (b - a) * G * E)], wo_sems.at[i]) for c in range(G)]
            for i, (a, b) in enumerate(zip(wo_cuts, wo_cuts[1:]))]

    def c_yb(tile, size):
        rows = pl.ds(tile, size // 16)
        return copy(yb.at[rows], out_h.at[rows, :, pl.ds(D, D)], sems.at[5])

    start([c_turns, c_rows] + c_ax + c_filt[0])
    for ref in (att, acc_last, part_o):
        ref[...] = jnp.zeros(ref.shape, f32)

    c_turns.wait()
    br, bi = turns[16:24, :], turns[56:64, :]
    for s in range(16):
        cr, ci = turns[24 + s:25 + s, :], turns[64 + s:65 + s, :]
        ar, ai = br * cr - bi * ci, br * ci + bi * cr
        gr = jnp.concatenate([ar * turns[a:a + 1, :] - ai * turns[40 + a:41 + a, :] for a in range(16)], axis=0)
        gi = jnp.concatenate([ar * turns[40 + a:41 + a, :] + ai * turns[a:a + 1, :] for a in range(16)], axis=0)
        for c, v in enumerate((gr, gi, gr + gi, gi - gr)):
            gmat[s, c] = v.astype(bf16)
    g_mat = lambda s, c: pltpu.bitcast(gmat.bitcast(u32)[s, c], bf16)
    row_mat = lambda i: pltpu.bitcast(rows_v[64 * i:64 * (i + 1)], bf16)
    inv_mat = lambda i: pltpu.bitcast(rows_inv.bitcast(u32)[64 * i:64 * (i + 1)], bf16)
    c_rows.wait()
    edge = lax.broadcasted_iota(jnp.int32, (128, 128), 0) % 64 == 0
    for i in range(5):
        gain = np.float32(2.0 / (S * D))
        rows_inv[128 * i:128 * (i + 1), :] = (row_mat(i).astype(f32) * (gain if i else jnp.where(edge, gain / 2, gain))).astype(bf16)
    first = lax.broadcasted_iota(jnp.int32, (8, 128), 0) == 0

    def rfft_rows(s):
        unpack = (_lo, _hi)[s % 2]
        x0, x1, x2, x3 = (unpack(ax[s // 2, :, 128 * j:128 * (j + 1)]) for j in range(4))
        s02, s13 = x0 + x2, x1 + x3
        xa = _dot(row_mat(0), (s02 + s13).astype(bf16), NT)
        xb = _dot(row_mat(1), (s02 - s13).astype(bf16), NT)
        d0, d1 = x0 - x2, x3 - x1
        k1 = _dot(row_mat(2), (d0 + d1).astype(bf16), NT)
        er = k1 - _dot(row_mat(3), d1.astype(bf16), NT)
        ei = k1 + _dot(row_mat(4), d0.astype(bf16), NT)
        nyq = xa[64:72]
        return (jnp.concatenate([xa[:64], xb[:64], er, nyq], axis=0),
                jnp.concatenate([jnp.where(first, 0.0, nyq), xa[72:], xb[64:], ei[:64], -ei[64:]], axis=0))

    def dft128(s, re, im):
        k1 = _dot(jnp.concatenate([re[:256] + im, re[256:]], axis=0), g_mat(s, 0))
        xs[s, 0, 0:256, :] = k1[:256] - _dot(im, g_mat(s, 2))
        xs[s, 0, 256:264, :] = k1[256:]
        xs[s, 1] = k1 + _dot(re, g_mat(s, 3))

    wait(c_ax[:2])
    pending = rfft_rows(0)
    for s in range(16):
        if s == 3:
            wait(c_ax[2:4])
            start(c_filt[1] + c_small)
        if s == 7:
            wait(c_ax[4:])
            start(sum((c_qkv(0, g) for g in range(NG)), []))
        ahead = rfft_rows(s + 1) if s < 15 else None
        dft128(s, *pending)
        pending = ahead

    wait(c_filt[0])
    start(sum((c_qkv(1, g) for g in range(NG)), []))

    def spectral_filter(r0, w):
        y = _fft16([(xs[s, 0, pl.ds(r0, 8), :], xs[s, 1, pl.ds(r0, 8), :]) for s in range(16)], -1)
        z = _fft16([(a * w[k][0] - b * w[k][1], a * w[k][1] + b * w[k][0]) for k, (a, b) in enumerate(y)], +1)
        for s in range(16):
            ts[s, 0, pl.ds(r0, 8), :] = z[s][0]
            ts[s, 1, pl.ds(r0, 8), :] = z[s][1]

    nr, ni = nyq_r[...].astype(f32), nyq_i[...].astype(f32)
    spectral_filter(256, [(jnp.broadcast_to(nr[:, 128 * k:128 * (k + 1)], (8, 128)),
                           jnp.broadcast_to(ni[:, 128 * k:128 * (k + 1)], (8, 128))) for k in range(16)])
    def filter_rows(i):
        for p in range(2):
            words = [[ref.bitcast(u32).at[pl.ds(pl.multiple_of(128 * k + 16 * i, 16), 16)][pl.ds(p, 8, stride=2), :]
                      for ref in (wr, wi)] for k in range(16)]
            for g, unpack in enumerate((_lo, _hi)):
                spectral_filter(pl.multiple_of((2 * g + p) * 64 + 8 * i, 8), [(unpack(a), unpack(b)) for a, b in words])

    @pl.loop(0, 2)
    def _(half):
        pl.when(half == 1)(lambda: wait(c_filt[1]))
        for i in range(4):
            filter_rows(4 * half + i)

    start(sum((c_qkv(2, g) for g in range(NG)), []))
    wait(c_small)

    def idft128(s):
        real, imag = [], []
        for g in range(4):
            tr, ti = ts[s, 0, 64 * g:64 * (g + 1), :], ts[s, 1, 64 * g:64 * (g + 1), :]
            a, b = (-ti, tr) if g == 3 else (ti, -tr)
            if g == 0:
                a = jnp.concatenate([jnp.where(first, ts[s, 0, 256:264, :], a[:8]), a[8:]], axis=0)
                b = jnp.concatenate([jnp.where(first, ts[s, 1, 256:264, :], b[:8]), b[8:]], axis=0)
            real.append(jnp.concatenate([tr, ti], axis=1))
            imag.append(jnp.concatenate([a, b], axis=1))
        rhs = jnp.concatenate([real[0], imag[0], real[1], imag[1], real[2], real[3], imag[2], imag[3]], axis=0)
        return _dot(jnp.concatenate([g_mat(s, 0), g_mat(s, 1)], axis=1), rhs.astype(bf16), NT)

    def irfft_rows(u):
        e0, e1 = _dot(u[:, 0:128], inv_mat(0)), _dot(u[:, 128:256], inv_mat(1))
        ur, ui = u[:, 256:384], u[:, 384:512]
        k1 = _dot(ur + ui, inv_mat(2))
        d0, d1 = k1 + _dot(ui, inv_mat(4)), k1 - _dot(ur, inv_mat(3))
        p, q = e0 + e1, e0 - e1
        return [p + d0, q - d1, p - d0, q + d1]

    pending = idft128(0)
    for s in range(16):
        ahead = idft128(s + 1) if s < 15 else None
        y = [pltpu.bitcast(v.astype(bf16).astype(f32), u32) for v in irfft_rows(pending)]
        if s % 2:
            for j in range(4):
                ya[s // 2, :, 128 * j:128 * (j + 1)] = (even[j] >> 16) | y[j]
        pending, even = ahead, y

    def w_qkv(g, m, r):
        return pltpu.bitcast(t_qkv.bitcast(u32)[(m * NG + g) * NPR + INDEX[r]], bf16)

    def w_o(g, r):
        return pltpu.bitcast(t_o.bitcast(u32)[g * NPR + INDEX[r]], bf16)

    def stage_tokens(it):
        x = bx[pl.ds(it * RB if isinstance(it, int) else pl.multiple_of(it * RB, RB), RB), :].astype(f32)
        blocks = {(i, k): x[i * SEG:(i + 1) * SEG, k * 128:(k + 1) * 128] for i in range(G) for k in range(G)}
        for r, v in _pre(blocks, SU, PRODUCTS).items():
            tok_lhs[INDEX[r]] = v

    stage_tokens(0)
    start(sum(c_wo, []) + [c_bx])

    def prepare(m):
        shift = SHIFT[m] if isinstance(m, int) else jnp.where(m == 0, SHIFT[0], SHIFT[1])
        for g in range(NG):
            for (i, n), v in _post({r: _dot(tok_lhs[INDEX[r]], w_qkv(g, m, r)) for r in PRODUCTS}).items():
                if i == G - 1:
                    tok_late[m, G * g + (n ^ shift)] = v
                else:
                    tok[m, G * g + (n ^ shift), i * SEG:(i + 1) * SEG, :] = v

    for m in range(3):

        @pl.loop(0, NG)
        def _(g):
            wait(c_qkv(m, g))
            for d0 in (0, 16, 48, 32, 64, 80, 112, 96):
                words = {(k, j): raw_qkv[m * (H // 2) + 2 * g + j, k * 128 + d0:k * 128 + d0 + 16, :]
                         for k in range(G) for j in range(2)}
                blocks = {(k, j ^ SHIFT[m]): (_lo, _hi)[j % 2](words[(k, j // 2)]) for k in range(G) for j in range(G)}
                for r, v in _pre(blocks, SV, PRODUCTS).items():
                    t_qkv[(m * NG + g) * NPR + INDEX[r], d0:d0 + 16, :] = v.astype(bf16)

        if m == 1:
            pl.loop(0, 2)(prepare)
        elif m == 2:
            prepare(2)

    stage_tokens(1)

    @pl.loop(0, NG)
    def _(g):
        for at, copies in zip(wo_cuts, c_wo):
            pl.when(g == at)(lambda copies=copies: wait(copies))
        for e0 in range(0, E, 16):
            blocks = {(k, n): pltpu.bitcast(raw_o.bitcast(u32)[pl.ds(pl.multiple_of(
                (n * H + G * g + k) * (E // 2) + e0 // 2, 8), 8), :], bf16).astype(f32) for k in range(G) for n in range(G)}
            for r, v in _pre(blocks, SV, PRODUCTS).items():
                t_o[g * NPR + INDEX[r], e0:e0 + 16, :] = v.astype(bf16)

    start(c_ya)

    ri = lax.broadcasted_iota(jnp.int32, (L, L), 0)
    ci = lax.broadcasted_iota(jnp.int32, (L, L), 1)
    allowed = (ri < M) | (ri >= ci)
    log2e = np.float32(np.log2(np.e))
    slab = lambda i, rb: slice(i * SEG + rb * 8, i * SEG + rb * 8 + 8)

    def combine(p, prods):
        for rb in range(SEG // 8):
            here = {r: prods[r][rb * 8 - a:rb * 8 + 8 - a] for r, (a, b) in ROWS[p].items() if a <= rb * 8 < b}
            for (i, n), v in _post(here).items():
                yield i, n, rb, v

    def emit(p, prods, it):
        for i, n, rb, v in combine(p, prods):
            where = (slab(i, rb), slice(128 * n, 128 * (n + 1)))
            part_o[where] = v if p == ADDS[(i, n, rb)][0] else v + part_o[where]
        if p == G - 1:
            yb[pl.ds(jnp.maximum(it, 0) * (RB // 16), RB // 16)] = part_o[...].astype(bf16).reshape(RB // 16, 16, D)

    def emit_last(it):
        emit(G - 1, {r: acc_last[INDEX[r], 0:b - a, :] for r, (a, b) in ROWS[G - 1].items()}, it)

    def segment(p, mem, held, ahead=True):
        final = not ahead and p == G - 1
        prods = list(ROWS[p])
        mem_in = _pre({(p, k): mem[:, 128 * k:128 * (k + 1)] for k in range(G)}, SU, prods)
        result, mem_qkv, mem_att, mem_out, acc = {}, {}, {}, {}, {}

        def project(g, m, r):
            a, b = ROWS[p][r]
            lhs = jnp.concatenate([tok_lhs[INDEX[r], a:b, :], mem_in[r]], axis=0) if ahead else mem_in[r]
            result[(g, m, r)] = _dot(lhs, w_qkv(g, m, r))
            if any((g, m, q) not in result for q in prods):
                return
            for n in range(G):
                for rb in range(SEG // 8):
                    if ahead and p and ADDS[(p - 1, n, rb)][-1] == p - 1:
                        h = G * g + (n ^ SHIFT[m])
                        tok[m, h, slab(p - 1, rb), :] = held.pop((m, h, p - 1, rb))
            if p == G - 2:
                for h in range(G * g, G * g + G):
                    tok[m, h, (G - 1) * SEG:G * SEG, :] = tok_late[m, h]
            res = {q: result.pop((g, m, q)) for q in prods}
            for (_, n), v in _post({q: v[-M:] for q, v in res.items()}, p).items():
                mem_qkv[(m, G * g + (n ^ SHIFT[m]))] = v
            for i, n, rb, v in combine(p, res) if ahead else ():
                h, adds = G * g + (n ^ SHIFT[m]), ADDS[(i, n, rb)]
                assert adds[-1] >= i
                if p != adds[0]:
                    v = v + held.pop((m, h, i, rb))
                if p == adds[-1] and p != i:
                    tok[m, h, slab(i, rb), :] = v
                elif p == G - 1:
                    tok_late[m, h, slab(0, rb), :] = v
                else:
                    held[(m, h, i, rb)] = v

        def rows_of(m, h):
            tokens = tok[m, h, p * SEG:(p + 1) * SEG, :]
            return tokens if final and m == 0 else jnp.concatenate([mem_qkv[(m, h)], tokens], axis=0)

        skip = M if final else 0
        earlier = lambda g, r, a, b: att_lhs[g * NPR + INDEX[r], a:b, :] if ahead else held[(g, r)][a:b]

        def scores(h):
            s = _dot(rows_of(0, h), rows_of(1, h).astype(bf16), NT) * (np.float32(E ** -0.5) * log2e)
            s = jnp.where(allowed[skip:], s, np.float32(-1e9) * log2e)
            e = jnp.exp2(s - jnp.max(s, axis=-1, keepdims=True))
            total = jnp.sum(e, axis=-1, keepdims=True)
            r = pl.reciprocal(total, approx=True)
            probs[h, skip:, :] = e * (r * (2.0 - total * r))

        def values(h):
            if p == 0 and h % G == 0:
                before = {(i, k): att[h + k, i * SEG:(i + 1) * SEG, :] for i in range(G) for k in range(G)}
                for r, v in _pre(before, SU, PRODUCTS).items():
                    if ahead:
                        att_lhs[h // G * NPR + INDEX[r]] = v
                    else:
                        held[(h // G, r)] = v
            o = _dot(probs[h, skip:, :], rows_of(2, h).astype(bf16))
            mem_att[h] = o[:M]
            if ahead:
                att[h, p * SEG:(p + 1) * SEG, :] = o[M:]
            else:
                held[('att', h, p)] = o[M - skip:]

        def output(gs, r):
            a, b = ROWS[p][r]
            for g in gs:
                if g not in mem_out:
                    mem_out[g] = _pre({(p, k): mem_att[G * g + k] for k in range(G)}, SU, prods)
            v = _dot(jnp.concatenate([jnp.concatenate([mem_out[g][r], earlier(g, r, a, b)], axis=0)
                                      for g in gs], axis=1),
                     jnp.concatenate([w_o(g, r) for g in gs], axis=0))
            if gs[0] > 0:
                v = v + acc_o[INDEX[r], 0:M + b - a, :]
            if gs[-1] < NG - 1:
                acc_o[INDEX[r], 0:M + b - a, :] = v
            acc[r] = v

        def final_output(gs, r):
            for g in gs:
                if g not in mem_out:
                    mem_out[g] = _pre({(i, k): held[('att', G * g + k, i)] for i in range(G) for k in range(G)}, SU, PRODUCTS)
            a, b = ROWS[p].get(r, (0, 0))
            rows = [jnp.concatenate([mem_out[g][r], earlier(g, r, a, b)], axis=0) if b else mem_out[g][r]
                    for g in gs]
            v = _dot(jnp.concatenate(rows, axis=1), jnp.concatenate([w_o(g, r) for g in gs], axis=0))
            acc[r] = acc[r] + v if gs[0] else v
            if gs[0] and b:
                result[r] = acc[r][SEG:]
                if all(q in result for q in prods):
                    emit(p, result, NIT - 2)
                    c_yb((S - 2 * RB) // 16, RB).start()

        run = {'project': project, 'scores': scores, 'values': values, 'output': final_output if final else output}
        for item in _schedule(p, ahead):
            run[item[0]](*item[1:])
        if final:
            return acc
        if p < G - 1:
            emit(p, {r: v[M:] for r, v in acc.items()}, None)
        else:
            for r, (a, b) in ROWS[p].items():
                acc_last[INDEX[r], 0:b - a, :] = acc[r][M:]
        new = _post({r: v[:M] for r, v in acc.items()}, p)
        return jnp.concatenate([new[(p, n)] for n in range(G)], axis=1)

    def iteration(it, mem):
        pl.when(it == 1)(c_bx.wait)
        pl.when(((it & 3) == 2) & (it > 2))(lambda: c_yb((it - 6) * (RB // 16), 4 * RB).start())
        emit_last(it - 2)
        held = {}
        for p in range(G):
            mem = segment(p, mem, held)
        stage_tokens(jnp.minimum(it + 2, NIT - 1))
        return mem

    mem = lax.fori_loop(0, NIT - 1, iteration, mem0[...].astype(f32))

    emit_last(NIT - 3)
    c_yb((S - 4 * RB) // 16, 2 * RB).start()
    held = {}
    for p in range(G - 1):
        mem = segment(p, mem, held, ahead=False)
    for (i, n), v in _post({r: v[:SEG] for r, v in segment(G - 1, mem, held, ahead=False).items()}).items():
        r0 = (S - RB + i * SEG) // 16
        yb[r0:r0 + SEG // 16, :, 128 * n:128 * (n + 1)] = v.astype(bf16).reshape(SEG // 16, 16, 128)
    c_yb((S - RB) // 16, RB).start()
    wait(c_ya)
    c_yb(0, S).wait()


def _scratch():
    vmem = pltpu.VMEM
    return [
        vmem((8, 128, D), u32), vmem((16 * 256, 128), bf16), vmem((16 * 256, 128), bf16),
        vmem((1, S), bf16), vmem((1, S), bf16),
        vmem(_DFT_ROWS.shape, u32), vmem(_DFT_TURNS.shape, f32), vmem((5 * 128, 128), bf16),
        vmem((16, 4, 128, 128), bf16),
        vmem((16, 2, 264, 128), f32), vmem((16, 2, 264, 128), f32), vmem((8, 128, D), u32),
        vmem((S, D), bf16), vmem((M, D), bf16),
        vmem((3 * H // 2, D, E), u32), vmem((G * H * E, 128), bf16),
        vmem((3 * NG * NPR, 128, E), bf16), vmem((NG * NPR, E, 128), bf16),
        vmem((NPR, SEG, 128), f32), vmem((3, H, RB, E), f32), vmem((3, H, SEG, E), f32),
        vmem((H, RB, E), f32), vmem((NG * NPR, SEG, E), f32), vmem((H, L, L), f32),
        vmem((NPR, L, 128), f32), vmem((NPR, SEG, 128), f32),
        vmem((RB, D), f32), vmem((S // 16, 16, D), bf16),
        pltpu.SemaphoreType.DMA((6,)), pltpu.SemaphoreType.DMA((8,)),
        pltpu.SemaphoreType.DMA((2,)), pltpu.SemaphoreType.DMA((3 * NG,)),
        pltpu.SemaphoreType.DMA((3,)),
    ]


@jax.jit
def pallas_concat_heads__spectral_gfnet__memory_aug_recurrent_mem_tr__prompt_kernel(
    A_x: jax.Array,
    A_w_r: jax.Array,
    A_w_i: jax.Array,
    B_x: jax.Array,
    B_mem0: jax.Array,
    B_Wq: jax.Array,
    B_Wk: jax.Array,
    B_Wv: jax.Array,
    B_Wo: jax.Array,
    B_seg_len: jax.Array,
):
    del B_seg_len
    hbm = pl.BlockSpec(memory_space=pl.ANY)
    out = pl.pallas_call(
        _kernel,
        out_shape=jax.ShapeDtypeStruct((S // 16, 16, 2 * D), bf16),
        in_specs=[hbm] * 11,
        out_specs=hbm,
        scratch_shapes=_scratch(),
        compiler_params=pltpu.CompilerParams(vmem_limit_bytes=120 * 2 ** 20),
    )(A_x.reshape(S // 16, 16, D), A_w_r.T, A_w_i.T, B_x.reshape(S, D), B_mem0.reshape(M, D),
      B_Wq, B_Wk, B_Wv, B_Wo.reshape(H * E, D), _DFT_ROWS, _DFT_TURNS)
    return out.reshape(1, S, 2 * D)
```

```python
import jax
import jax.numpy as jnp
import ml_dtypes
import numpy as np
from jax import lax
import jax.experimental.pallas as pl
import jax.experimental.pallas.tpu as pltpu

S, D, H, E, M, SEG = 2048, 512, 32, 128, 8, 32
L = M + SEG
G = 4
NG = H // G
RB = G * SEG
NIT = S // RB
SHIFT = (0, 2, 0)
f32, bf16, u32 = jnp.float32, jnp.bfloat16, jnp.uint32
NN = (((1,), (0,)), ((), ()))
NT = (((1,), (1,)), ((), ()))


def _dot(a, b, dims=NN):
    return lax.dot_general(a, b, dims, preferred_element_type=f32)


def _lo(u):
    return pltpu.bitcast(u << 16, f32)


def _hi(u):
    return pltpu.bitcast(u & np.uint32(0xFFFF0000), f32)


SU = {1: (((0, 0), 1), ((1, 1), 1)), 2: (((1, 0), 1), ((1, 1), 1)), 3: (((0, 0), 1),), 4: (((1, 1), 1),),
      5: (((0, 0), 1), ((0, 1), 1)), 6: (((1, 0), 1), ((0, 0), -1)), 7: (((0, 1), 1), ((1, 1), -1))}
SV = {1: (((0, 0), 1), ((1, 1), 1)), 2: (((0, 0), 1),), 3: (((0, 1), 1), ((1, 1), -1)),
      4: (((1, 0), 1), ((0, 0), -1)), 5: (((1, 1), 1),), 6: (((0, 0), 1), ((0, 1), 1)),
      7: (((1, 0), 1), ((1, 1), 1))}
SW = {(0, 0): ((1, 1), (4, 1), (7, 1), (5, -1)), (0, 1): ((3, 1), (5, 1)), (1, 0): ((2, 1), (4, 1)),
      (1, 1): ((1, 1), (3, 1), (6, 1), (2, -1))}
OWN = ((3, 1, 5, 7), (4, 1, 2, 6))


def _lin(terms):
    terms = [(v, c) for v, c in terms if v is not None]
    if not terms:
        return None
    pos = [v for v, c in terms if c > 0]
    neg = [v for v, c in terms if c < 0]
    if pos:
        acc = pos[0]
        for v in pos[1:]:
            acc = acc + v
    else:
        acc, neg = -neg[0], neg[1:]
    for v in neg:
        acc = acc - v
    return acc


def _pre(blocks, table, want):
    if not want[0]:
        return {(): blocks.get((0, 0))}
    h = 2 ** (len(want[0]) - 1)
    out = {}
    for r in sorted({w[0] for w in want}):
        sub = {(i, k): _lin([(blocks.get((a * h + i, b * h + k)), c) for (a, b), c in table[r]])
               for i in range(h) for k in range(h)}
        for rest, v in _pre(sub, table, sorted(w[1:] for w in want if w[0] == r)).items():
            out[(r,) + rest] = v
    return out


def _post(prods, row=None):
    if () in prods:
        return {(0, 0): prods[()]}
    h = 2 ** (len(next(iter(prods))) - 1)
    inner = {r: _post({w[1:]: v for w, v in prods.items() if w[0] == r}, None if row is None else row % h)
             for r in sorted({w[0] for w in prods})}
    out = {}
    for (a, b), terms in SW.items():
        for i in range(h):
            if row is None or row == a * h + i:
                for n in range(h):
                    v = _lin([(inner.get(r, {}).get((i, n)), c) for r, c in terms])
                    if v is not None:
                        out[(a * h + i, b * h + n)] = v
    return out


PRODUCTS = [(a, b) for a in range(1, 8) for b in range(1, 8)]
NPR = len(PRODUCTS)
INDEX = {r: i for i, r in enumerate(PRODUCTS)}


def _token_rows():
    phases = [[(a, b) for a in OWN[p >> 1] for b in OWN[p & 1]] for p in range(G)]
    rows = []
    for p in range(G):
        rows.append({})
        for r in phases[p]:
            users = [q for q in range(G) if r in phases[q]]
            n = SEG // len(users)
            rows[p][r] = (users.index(p) * n, (users.index(p) + 1) * n)
    return rows


def _contributors(rows):
    out = {}
    for p in range(G):
        for r, (a, b) in rows[p].items():
            for rb in range(a // 8, b // 8):
                for key in _post({r: np.zeros(1)}):
                    if p not in out.setdefault(key + (rb,), []):
                        out[key + (rb,)].append(p)
    return out


ROWS = _token_rows()
ADDS = _contributors(ROWS)


def _schedule(p, ahead):
    final = not ahead and p == G - 1
    size = {r: b - a for r, (a, b) in ROWS[p].items()}
    long_ = [r for r in size if size[r] == SEG]
    short = [r for r in size if size[r] == SEG // 2]
    tiny = [r for r in size if size[r] == SEG // 4]
    prev = (p - 1) % G
    early = [{(0, 1): (1, 3), (0, 0): (7,), (1, 1): (6,), (1, 0): (1, 4)}[(p >> s & 1, prev >> s & 1)] for s in (1, 0)]
    lead = ([r for r in long_ if r[0] in early[0] and r[1] in early[1]] + [long_[8]])[0]
    pool = [lead, short[4], tiny[0], short[5]]
    rest = [r for r in long_ if r != lead]
    groups = [(g, m) for g in range(NG) for m in ((1,) if final else (0, 1))] + [(g, 2) for g in range(NG)]
    shared = lambda i, r: [('project', g, m, r) for (g, m) in groups[i:i + 4]]
    own = lambda i, rs: [('project',) + groups[i] + (r,) for r in rs]
    rounds = []
    for i in range(len(groups)):
        a, b, c = own(i, rest[:4]), own(i, short[:4]), own(i, rest[4:])
        if i == 0:
            rounds += [shared(0, pool[0]), shared(0, pool[1]), a, shared(0, pool[2]), c, b, shared(0, pool[3])]
        else:
            rounds += [a, b, c]
        if i // 4 * 4 + 4 < len(groups):
            rounds.append(shared(i // 4 * 4 + 4, pool[i % 4]))
    if not ahead:
        items = [('project', g, m, r) for (g, m) in groups for r in size]
        head = [it for it in items if it[3][0] in early[0] and it[3][1] in early[1]][:16]
        items = head + [it for it in items if it not in head]
        rounds = [items[i:i + 4] for i in range(0, len(items), 4)]
    done = {item[1:3]: t + 1 for t, rd in enumerate(rounds) for item in rd}
    rest, mixed = list(long_), []
    fill = [r for r in size if size[r] < SEG]
    while rest or fill:
        mixed += rest[:1]
        rest = rest[1:]
        if fill and len(fill) >= len(rest) - 1:
            mixed.append(fill.pop(0))
    if not ahead:
        soon = [((3, 5), (2, 4))[p >> s & 1] for s in (1, 0)]
        mixed = sorted(mixed, key=lambda r: not (r[0] in soon[0] and r[1] in soon[1]))
    for g0 in range(0, 0 if final else NG, 4):
        rounds += [[('output', tuple(range(g0, g0 + 4)), r)] for r in mixed]
    extra = {}

    def place(t, items):
        while any(abs(t - u) < 3 for u in extra):
            t += 1
        extra[t] = items
        return t

    scored = [place(done[(g, 1)] + (6 + g % 2 if ahead else 7), [('scores', G * g + n) for n in range(G)]) for g in range(NG)]
    for g in range(NG):
        place(max(done[(g, 2)] + 6, scored[g] + 5), [('values', G * g + n) for n in range(G)])
    if final:
        order = sorted(PRODUCTS, key=lambda r: tuple((3, 5, 1, 7, 4, 2, 6).index(x) for x in r))
        rounds += [[('output', (0, 1, 2, 3), r)] for r in order]
        order = sorted(order, key=lambda r: r not in size)
        rounds += [[('output', (4, 5, 6, 7), r)] for r in order]
    return [item for t, rd in enumerate(rounds) for item in extra.get(t, []) + rd]


def _dft_constants():
    n = np.arange(128)[None, :]
    m = np.arange(64)[:, None]
    angle = lambda k: 2 * np.pi * ((k * n) % D) / D
    even0 = np.concatenate([np.cos(angle(4 * m)), -np.sin(angle(4 * m))])
    even0[64] = np.cos(np.pi * n[0])
    even2 = np.concatenate([np.cos(angle(4 * m + 2)), -np.sin(angle(4 * m + 2))])
    cr = np.concatenate([np.cos(angle(4 * m + 1)), np.cos(angle(4 * m + 3))])
    ci = np.concatenate([-np.sin(angle(4 * m + 1)), np.sin(angle(4 * m + 3))])
    rows = np.concatenate([even0, even2, cr, cr + ci, ci - cr]).astype(np.float32).astype(ml_dtypes.bfloat16)
    rows = rows.view(np.uint16).astype(np.uint32)
    offsets = np.concatenate([128 * np.arange(16), 16 * np.arange(8), np.arange(16)])
    turn = 2 * np.pi * ((offsets[:, None] * n) % S) / S
    return rows[0::2] | (rows[1::2] << 16), np.concatenate([np.cos(turn), -np.sin(turn)]).astype(np.float32)


_DFT_ROWS, _DFT_TURNS = _dft_constants()


def _fft4(a, b, c, d, sign):
    t0 = (a[0] + c[0], a[1] + c[1])
    t1 = (a[0] - c[0], a[1] - c[1])
    t2 = (b[0] + d[0], b[1] + d[1])
    t3 = (b[0] - d[0], b[1] - d[1])
    y0 = (t0[0] + t2[0], t0[1] + t2[1])
    y2 = (t0[0] - t2[0], t0[1] - t2[1])
    p = (t1[0] + t3[1], t1[1] - t3[0])
    q = (t1[0] - t3[1], t1[1] + t3[0])
    return (y0, p, y2, q) if sign < 0 else (y0, q, y2, p)


def _rotate16(z, e, sign):
    if e == 0:
        return z
    r, i = z
    if e == 4:
        return (i, -r) if sign < 0 else (-i, r)
    h = np.float32(np.sqrt(0.5))
    if e == 2:
        return ((r + i) * h, (i - r) * h) if sign < 0 else ((r - i) * h, (r + i) * h)
    if e == 6:
        return ((i - r) * h, (r + i) * (-h)) if sign < 0 else ((r + i) * (-h), (r - i) * h)
    c = np.float32(np.cos(2 * np.pi * e / 16))
    s = np.float32(sign * np.sin(2 * np.pi * e / 16))
    return (r * c - i * s, r * s + i * c)


def _fft16(x, sign):
    col = [_fft4(x[n], x[4 + n], x[8 + n], x[12 + n], sign) for n in range(4)]
    y = [None] * 16
    for k1 in range(4):
        r = _fft4(*[_rotate16(col[n][k1], n * k1, sign) for n in range(4)], sign)
        for k2 in range(4):
            y[k1 + 4 * k2] = r[k2]
    return y


def _kernel(ax_h, wr_h, wi_h, bx_h, mem_h, wq_h, wk_h, wv_h, wo_h, rows_h, turns_h, out_h,
            ax, wr, wi, nyq_r, nyq_i, rows_v, turns, rows_inv, gmat, xs, ts, ya,
            bx, mem0, raw_qkv, raw_o, t_qkv, t_o, tok_lhs, tok, tok_late, att, att_lhs, probs, acc_o, acc_last,
            part_o, yb, sems, row_sems, filt_sems, qkv_sems, wo_sems):
    copy = pltpu.make_async_copy

    def start(copies):
        for c in copies:
            c.start()

    def wait(copies):
        for c in copies:
            c.wait()

    c_turns, c_rows = copy(turns_h, turns, sems.at[0]), copy(rows_h, rows_v, sems.at[2])
    c_ax = [copy(ax_h.bitcast(u32).at[:, j, :], ax.at[j], row_sems.at[j]) for j in range(8)]
    c_filt = [[copy(src.at[pl.ds(128 * b, 128), pl.ds(128 * k, 128)], dst.at[pl.ds(256 * k + 128 * b, 128)], filt_sems.at[b])
               for k in range(16) for src, dst in ((wr_h, wr), (wi_h, wi))] for b in range(2)]
    c_filt[0] += [copy(src.at[pl.ds(256, 1)], dst, filt_sems.at[0]) for src, dst in ((wr_h, nyq_r), (wi_h, nyq_i))]
    c_small = [copy(bx_h.at[pl.ds(0, 3 * RB)], bx.at[pl.ds(0, 3 * RB)], sems.at[1]), copy(mem_h, mem0, sems.at[1])]

    def c_qkv(src, m, g):
        return [copy(src.bitcast(u32).at[:, 2 * g + j, :], raw_qkv.at[m * (H // 2) + 2 * g + j], qkv_sems.at[m * NG + g])
                for j in range(2)]

    c_bx = copy(bx_h.at[pl.ds(3 * RB, S - 3 * RB)], bx.at[pl.ds(3 * RB, S - 3 * RB)], sems.at[3])
    c_ya = [copy(ya.at[j], out_h.bitcast(u32).at[:, j, pl.ds(0, D)], sems.at[4]) for j in range(8)]

    wo_cuts = (0, 4, NG - 1, NG)
    c_wo = [[copy(wo_h.at[pl.ds(a * G * E, (b - a) * G * E), pl.ds(128 * c, 128)],
                  raw_o.at[pl.ds((c * H + a * G) * E, (b - a) * G * E)], wo_sems.at[i]) for c in range(G)]
            for i, (a, b) in enumerate(zip(wo_cuts, wo_cuts[1:]))]

    def c_yb(tile, size):
        rows = pl.ds(tile, size // 16)
        return copy(yb.at[rows], out_h.at[rows, :, pl.ds(D, D)], sems.at[5])

    start([c_turns, c_rows] + c_ax + c_filt[0])
    for ref in (att, acc_last, part_o):
        ref[...] = jnp.zeros(ref.shape, f32)

    c_turns.wait()
    br, bi = turns[16:24, :], turns[56:64, :]
    for s in range(16):
        cr, ci = turns[24 + s:25 + s, :], turns[64 + s:65 + s, :]
        ar, ai = br * cr - bi * ci, br * ci + bi * cr
        gr = jnp.concatenate([ar * turns[a:a + 1, :] - ai * turns[40 + a:41 + a, :] for a in range(16)], axis=0)
        gi = jnp.concatenate([ar * turns[40 + a:41 + a, :] + ai * turns[a:a + 1, :] for a in range(16)], axis=0)
        for c, v in enumerate((gr, gi, gr + gi, gi - gr)):
            gmat[s, c] = v.astype(bf16)
    g_mat = lambda s, c: pltpu.bitcast(gmat.bitcast(u32)[s, c], bf16)
    row_mat = lambda i: pltpu.bitcast(rows_v[64 * i:64 * (i + 1)], bf16)
    inv_mat = lambda i: pltpu.bitcast(rows_inv.bitcast(u32)[64 * i:64 * (i + 1)], bf16)
    c_rows.wait()
    edge = lax.broadcasted_iota(jnp.int32, (128, 128), 0) % 64 == 0
    for i in range(5):
        gain = np.float32(2.0 / (S * D))
        rows_inv[128 * i:128 * (i + 1), :] = (row_mat(i).astype(f32) * (gain if i else jnp.where(edge, gain / 2, gain))).astype(bf16)
    first = lax.broadcasted_iota(jnp.int32, (8, 128), 0) == 0

    def rfft_rows(s):
        unpack = (_lo, _hi)[s % 2]
        x0, x1, x2, x3 = (unpack(ax[s // 2, :, 128 * j:128 * (j + 1)]) for j in range(4))
        s02, s13 = x0 + x2, x1 + x3
        xa = _dot(row_mat(0), (s02 + s13).astype(bf16), NT)
        xb = _dot(row_mat(1), (s02 - s13).astype(bf16), NT)
        d0, d1 = x0 - x2, x3 - x1
        k1 = _dot(row_mat(2), (d0 + d1).astype(bf16), NT)
        er = k1 - _dot(row_mat(3), d1.astype(bf16), NT)
        ei = k1 + _dot(row_mat(4), d0.astype(bf16), NT)
        nyq = xa[64:72]
        return (jnp.concatenate([xa[:64], xb[:64], er, nyq], axis=0),
                jnp.concatenate([jnp.where(first, 0.0, nyq), xa[72:], xb[64:], ei[:64], -ei[64:]], axis=0))

    def dft128(s, re, im):
        k1 = _dot(jnp.concatenate([re[:256] + im, re[256:]], axis=0), g_mat(s, 0))
        xs[s, 0, 0:256, :] = k1[:256] - _dot(im, g_mat(s, 2))
        xs[s, 0, 256:264, :] = k1[256:]
        xs[s, 1] = k1 + _dot(re, g_mat(s, 3))

    wait(c_ax[:2])
    pending = rfft_rows(0)
    for s in range(16):
        if s == 3:
            wait(c_ax[2:4])
            start(c_filt[1] + c_small)
        if s == 7:
            wait(c_ax[4:])
            start(sum((c_qkv(wq_h, 0, g) for g in range(NG)), []))
        ahead = rfft_rows(s + 1) if s < 15 else None
        dft128(s, *pending)
        pending = ahead

    wait(c_filt[0])
    start(sum((c_qkv(wk_h, 1, g) for g in range(NG)), []))

    def spectral_filter(r0, w):
        y = _fft16([(xs[s, 0, pl.ds(r0, 8), :], xs[s, 1, pl.ds(r0, 8), :]) for s in range(16)], -1)
        z = _fft16([(a * w[k][0] - b * w[k][1], a * w[k][1] + b * w[k][0]) for k, (a, b) in enumerate(y)], +1)
        for s in range(16):
            ts[s, 0, pl.ds(r0, 8), :] = z[s][0]
            ts[s, 1, pl.ds(r0, 8), :] = z[s][1]

    nr, ni = nyq_r[...].astype(f32), nyq_i[...].astype(f32)
    spectral_filter(256, [(jnp.broadcast_to(nr[:, 128 * k:128 * (k + 1)], (8, 128)),
                           jnp.broadcast_to(ni[:, 128 * k:128 * (k + 1)], (8, 128))) for k in range(16)])

    def filter_rows(i):
        for p in range(2):
            words = [[ref.bitcast(u32).at[pl.ds(128 * k + 16 * i, 16)][pl.ds(p, 8, stride=2), :]
                      for ref in (wr, wi)] for k in range(16)]
            for g, unpack in enumerate((_lo, _hi)):
                spectral_filter((2 * g + p) * 64 + 8 * i, [(unpack(a), unpack(b)) for a, b in words])

    for i in range(8):
        if i == 4:
            wait(c_filt[1])
        filter_rows(i)

    start(sum((c_qkv(wv_h, 2, g) for g in range(NG)), []))
    wait(c_small)

    def idft128(s):
        real, imag = [], []
        for g in range(4):
            tr, ti = ts[s, 0, 64 * g:64 * (g + 1), :], ts[s, 1, 64 * g:64 * (g + 1), :]
            a, b = (-ti, tr) if g == 3 else (ti, -tr)
            if g == 0:
                a = jnp.concatenate([jnp.where(first, ts[s, 0, 256:264, :], a[:8]), a[8:]], axis=0)
                b = jnp.concatenate([jnp.where(first, ts[s, 1, 256:264, :], b[:8]), b[8:]], axis=0)
            real.append(jnp.concatenate([tr, ti], axis=1))
            imag.append(jnp.concatenate([a, b], axis=1))
        rhs = jnp.concatenate([real[0], imag[0], real[1], imag[1], real[2], real[3], imag[2], imag[3]], axis=0)
        return _dot(jnp.concatenate([g_mat(s, 0), g_mat(s, 1)], axis=1), rhs.astype(bf16), NT)

    def irfft_rows(u):
        e0, e1 = _dot(u[:, 0:128], inv_mat(0)), _dot(u[:, 128:256], inv_mat(1))
        ur, ui = u[:, 256:384], u[:, 384:512]
        k1 = _dot(ur + ui, inv_mat(2))
        d0, d1 = k1 + _dot(ui, inv_mat(4)), k1 - _dot(ur, inv_mat(3))
        p, q = e0 + e1, e0 - e1
        return [p + d0, q - d1, p - d0, q + d1]

    pending = idft128(0)
    for s in range(16):
        ahead = idft128(s + 1) if s < 15 else None
        y = [pltpu.bitcast(v.astype(bf16).astype(f32), u32) for v in irfft_rows(pending)]
        if s % 2:
            for j in range(4):
                ya[s // 2, :, 128 * j:128 * (j + 1)] = (even[j] >> 16) | y[j]
        pending, even = ahead, y

    def w_qkv(g, m, r):
        return pltpu.bitcast(t_qkv.bitcast(u32)[(m * NG + g) * NPR + INDEX[r]], bf16)

    def w_o(g, r):
        return pltpu.bitcast(t_o.bitcast(u32)[g * NPR + INDEX[r]], bf16)

    def stage_tokens(it):
        x = bx[pl.ds(it * RB if isinstance(it, int) else pl.multiple_of(it * RB, RB), RB), :].astype(f32)
        blocks = {(i, k): x[i * SEG:(i + 1) * SEG, k * 128:(k + 1) * 128] for i in range(G) for k in range(G)}
        for r, v in _pre(blocks, SU, PRODUCTS).items():
            tok_lhs[INDEX[r]] = v

    stage_tokens(0)
    start(sum(c_wo, []) + [c_bx])

    @pl.loop(0, 3)
    def _(m):
        shift = jnp.where(m == 1, SHIFT[1], SHIFT[0])

        @pl.loop(0, NG)
        def _(g):
            for i, src in enumerate((wq_h, wk_h, wv_h)):
                pl.when(m == i)(lambda i=i, src=src: wait(c_qkv(src, i, g)))
            for d0 in (0, 16, 48, 32, 64, 80, 112, 96):
                words = {(k, j): raw_qkv[m * (H // 2) + 2 * g + (j ^ (shift >> 1)), k * 128 + d0:k * 128 + d0 + 16, :]
                         for k in range(G) for j in range(2)}
                blocks = {(k, n): (_lo, _hi)[n % 2](words[(k, n // 2)]) for k in range(G) for n in range(G)}
                for r, v in _pre(blocks, SV, PRODUCTS).items():
                    t_qkv[(m * NG + g) * NPR + INDEX[r], d0:d0 + 16, :] = v.astype(bf16)

        for g in range(NG):
            for (i, n), v in _post({r: _dot(tok_lhs[INDEX[r]], w_qkv(g, m, r)) for r in PRODUCTS}).items():
                if i == G - 1:
                    tok_late[m, G * g + (n ^ shift)] = v
                else:
                    tok[m, G * g + (n ^ shift), i * SEG:(i + 1) * SEG, :] = v

    stage_tokens(1)

    @pl.loop(0, NG)
    def _(g):
        for at, copies in zip(wo_cuts, c_wo):
            pl.when(g == at)(lambda copies=copies: wait(copies))
        for e0 in range(0, E, 16):
            blocks = {(k, n): pltpu.bitcast(raw_o.bitcast(u32)[pl.ds(pl.multiple_of(
                (n * H + G * g + k) * (E // 2) + e0 // 2, 8), 8), :], bf16).astype(f32) for k in range(G) for n in range(G)}
            for r, v in _pre(blocks, SV, PRODUCTS).items():
                t_o[g * NPR + INDEX[r], e0:e0 + 16, :] = v.astype(bf16)

    start(c_ya)

    ri = lax.broadcasted_iota(jnp.int32, (L, L), 0)
    ci = lax.broadcasted_iota(jnp.int32, (L, L), 1)
    allowed = (ri < M) | (ri >= ci)
    log2e = np.float32(np.log2(np.e))
    slab = lambda i, rb: slice(i * SEG + rb * 8, i * SEG + rb * 8 + 8)

    def combine(p, prods):
        for rb in range(SEG // 8):
            here = {r: prods[r][rb * 8 - a:rb * 8 + 8 - a] for r, (a, b) in ROWS[p].items() if a <= rb * 8 < b}
            for (i, n), v in _post(here).items():
                yield i, n, rb, v

    def emit(p, prods, it):
        for i, n, rb, v in combine(p, prods):
            where = (slab(i, rb), slice(128 * n, 128 * (n + 1)))
            part_o[where] = v if p == ADDS[(i, n, rb)][0] else v + part_o[where]
        if p == G - 1:
            yb[pl.ds(jnp.maximum(it, 0) * (RB // 16), RB // 16)] = part_o[...].astype(bf16).reshape(RB // 16, 16, D)

    def emit_last(it):
        emit(G - 1, {r: acc_last[INDEX[r], 0:b - a, :] for r, (a, b) in ROWS[G - 1].items()}, it)

    def segment(p, mem, held, ahead=True):
        final = not ahead and p == G - 1
        prods = list(ROWS[p])
        mem_in = _pre({(p, k): mem[:, 128 * k:128 * (k + 1)] for k in range(G)}, SU, prods)
        result, mem_qkv, mem_att, mem_out, acc = {}, {}, {}, {}, {}

        def project(g, m, r):
            a, b = ROWS[p][r]
            lhs = jnp.concatenate([tok_lhs[INDEX[r], a:b, :], mem_in[r]], axis=0) if ahead else mem_in[r]
            result[(g, m, r)] = _dot(lhs, w_qkv(g, m, r))
            if any((g, m, q) not in result for q in prods):
                return
            for n in range(G):
                for rb in range(SEG // 8):
                    if ahead and p and ADDS[(p - 1, n, rb)][-1] == p - 1:
                        h = G * g + (n ^ SHIFT[m])
                        tok[m, h, slab(p - 1, rb), :] = held.pop((m, h, p - 1, rb))
            if p == G - 2:
                for h in range(G * g, G * g + G):
                    tok[m, h, (G - 1) * SEG:G * SEG, :] = tok_late[m, h]
            res = {q: result.pop((g, m, q)) for q in prods}
            for (_, n), v in _post({q: v[-M:] for q, v in res.items()}, p).items():
                mem_qkv[(m, G * g + (n ^ SHIFT[m]))] = v
            for i, n, rb, v in combine(p, res) if ahead else ():
                h, adds = G * g + (n ^ SHIFT[m]), ADDS[(i, n, rb)]
                assert adds[-1] >= i
                if p != adds[0]:
                    v = v + held.pop((m, h, i, rb))
                if p == adds[-1] and p != i:
                    tok[m, h, slab(i, rb), :] = v
                elif p == G - 1:
                    tok_late[m, h, slab(0, rb), :] = v
                else:
                    held[(m, h, i, rb)] = v

        def rows_of(m, h):
            tokens = tok[m, h, p * SEG:(p + 1) * SEG, :]
            return tokens if final and m == 0 else jnp.concatenate([mem_qkv[(m, h)], tokens], axis=0)

        skip = M if final else 0
        earlier = lambda g, r, a, b: att_lhs[g * NPR + INDEX[r], a:b, :] if ahead else held[(g, r)][a:b]

        def scores(h):
            s = _dot(rows_of(0, h), rows_of(1, h).astype(bf16), NT) * (np.float32(E ** -0.5) * log2e)
            s = jnp.where(allowed[skip:], s, np.float32(-1e9) * log2e)
            e = jnp.exp2(s - jnp.max(s, axis=-1, keepdims=True))
            total = jnp.sum(e, axis=-1, keepdims=True)
            probs[h, skip:, :] = e * pl.reciprocal(total, approx=False, full_range=False)

        def values(h):
            if p == 0 and h % G == 0:
                before = {(i, k): att[h + k, i * SEG:(i + 1) * SEG, :] for i in range(G) for k in range(G)}
                for r, v in _pre(before, SU, PRODUCTS).items():
                    if ahead:
                        att_lhs[h // G * NPR + INDEX[r]] = v
                    else:
                        held[(h // G, r)] = v
            o = _dot(probs[h, skip:, :], rows_of(2, h).astype(bf16))
            mem_att[h] = o[:M]
            if ahead:
                att[h, p * SEG:(p + 1) * SEG, :] = o[M:]
            else:
                held[('att', h, p)] = o[M - skip:]

        def output(gs, r):
            a, b = ROWS[p][r]
            for g in gs:
                if g not in mem_out:
                    mem_out[g] = _pre({(p, k): mem_att[G * g + k] for k in range(G)}, SU, prods)
            v = _dot(jnp.concatenate([jnp.concatenate([mem_out[g][r], earlier(g, r, a, b)], axis=0)
                                      for g in gs], axis=1),
                     jnp.concatenate([w_o(g, r) for g in gs], axis=0))
            if gs[0] > 0:
                v = v + acc_o[INDEX[r], 0:M + b - a, :]
            if gs[-1] < NG - 1:
                acc_o[INDEX[r], 0:M + b - a, :] = v
            acc[r] = v

        def final_output(gs, r):
            for g in gs:
                if g not in mem_out:
                    mem_out[g] = _pre({(i, k): held[('att', G * g + k, i)] for i in range(G) for k in range(G)}, SU, PRODUCTS)
            a, b = ROWS[p].get(r, (0, 0))
            rows = [jnp.concatenate([mem_out[g][r], earlier(g, r, a, b)], axis=0) if b else mem_out[g][r]
                    for g in gs]
            v = _dot(jnp.concatenate(rows, axis=1), jnp.concatenate([w_o(g, r) for g in gs], axis=0))
            acc[r] = acc[r] + v if gs[0] else v
            if gs[0] and b:
                result[r] = acc[r][SEG:]
                if all(q in result for q in prods):
                    emit(p, result, NIT - 2)
                    c_yb((S - 2 * RB) // 16, RB).start()

        run = {'project': project, 'scores': scores, 'values': values, 'output': final_output if final else output}
        for item in _schedule(p, ahead):
            run[item[0]](*item[1:])
        if final:
            return acc
        if p < G - 1:
            emit(p, {r: v[M:] for r, v in acc.items()}, None)
        else:
            for r, (a, b) in ROWS[p].items():
                acc_last[INDEX[r], 0:b - a, :] = acc[r][M:]
        new = _post({r: v[:M] for r, v in acc.items()}, p)
        return jnp.concatenate([new[(p, n)] for n in range(G)], axis=1)

    def iteration(it, mem):
        pl.when(it == 1)(c_bx.wait)
        pl.when(((it & 3) == 2) & (it > 2))(lambda: c_yb((it - 6) * (RB // 16), 4 * RB).start())
        emit_last(it - 2)
        held = {}
        for p in range(G):
            mem = segment(p, mem, held)
        stage_tokens(jnp.minimum(it + 2, NIT - 1))
        return mem

    mem = lax.fori_loop(0, NIT - 1, iteration, mem0[...].astype(f32))

    emit_last(NIT - 3)
    c_yb((S - 4 * RB) // 16, 2 * RB).start()
    held = {}
    for p in range(G - 1):
        mem = segment(p, mem, held, ahead=False)
    for (i, n), v in _post({r: v[:SEG] for r, v in segment(G - 1, mem, held, ahead=False).items()}).items():
        r0 = (S - RB + i * SEG) // 16
        yb[r0:r0 + SEG // 16, :, 128 * n:128 * (n + 1)] = v.astype(bf16).reshape(SEG // 16, 16, 128)
    c_yb((S - RB) // 16, RB).start()
    wait(c_ya)
    c_yb(0, S).wait()


def _scratch():
    vmem = pltpu.VMEM
    return [
        vmem((8, 128, D), u32), vmem((16 * 256, 128), bf16), vmem((16 * 256, 128), bf16),
        vmem((1, S), bf16), vmem((1, S), bf16),
        vmem(_DFT_ROWS.shape, u32), vmem(_DFT_TURNS.shape, f32), vmem((5 * 128, 128), bf16),
        vmem((16, 4, 128, 128), bf16),
        vmem((16, 2, 264, 128), f32), vmem((16, 2, 264, 128), f32), vmem((8, 128, D), u32),
        vmem((S, D), bf16), vmem((M, D), bf16),
        vmem((3 * H // 2, D, E), u32), vmem((G * H * E, 128), bf16),
        vmem((3 * NG * NPR, 128, E), bf16), vmem((NG * NPR, E, 128), bf16),
        vmem((NPR, SEG, 128), f32), vmem((3, H, RB, E), f32), vmem((3, H, SEG, E), f32),
        vmem((H, RB, E), f32), vmem((NG * NPR, SEG, E), f32), vmem((H, L, L), f32),
        vmem((NPR, L, 128), f32), vmem((NPR, SEG, 128), f32),
        vmem((RB, D), f32), vmem((S // 16, 16, D), bf16),
        pltpu.SemaphoreType.DMA((6,)), pltpu.SemaphoreType.DMA((8,)),
        pltpu.SemaphoreType.DMA((2,)), pltpu.SemaphoreType.DMA((3 * NG,)),
        pltpu.SemaphoreType.DMA((3,)),
    ]


@jax.jit
def pallas_concat_heads__spectral_gfnet__memory_aug_recurrent_mem_tr__prompt_kernel(
    A_x: jax.Array,
    A_w_r: jax.Array,
    A_w_i: jax.Array,
    B_x: jax.Array,
    B_mem0: jax.Array,
    B_Wq: jax.Array,
    B_Wk: jax.Array,
    B_Wv: jax.Array,
    B_Wo: jax.Array,
    B_seg_len: jax.Array,
):
    del B_seg_len
    hbm = pl.BlockSpec(memory_space=pl.ANY)
    out = pl.pallas_call(
        _kernel,
        out_shape=jax.ShapeDtypeStruct((S // 16, 16, 2 * D), bf16),
        in_specs=[hbm] * 11,
        out_specs=hbm,
        scratch_shapes=_scratch(),
        compiler_params=pltpu.CompilerParams(vmem_limit_bytes=120 * 2 ** 20),
    )(A_x.reshape(S // 16, 16, D), A_w_r.T, A_w_i.T, B_x.reshape(S, D), B_mem0.reshape(M, D),
      B_Wq, B_Wk, B_Wv, B_Wo.reshape(H * E, D), _DFT_ROWS, _DFT_TURNS)
    return out.reshape(1, S, 2 * D)
```

```python
import jax
import jax.numpy as jnp
import ml_dtypes
import numpy as np
from jax import lax
import jax.experimental.pallas as pl
import jax.experimental.pallas.tpu as pltpu

S, D, H, E, M, SEG = 2048, 512, 32, 128, 8, 32
L = M + SEG
G = 4
NG = H // G
RB = G * SEG
NIT = S // RB
SHIFT = (0, 2, 0)
f32, bf16, u32 = jnp.float32, jnp.bfloat16, jnp.uint32
NN = (((1,), (0,)), ((), ()))
NT = (((1,), (1,)), ((), ()))


def _dot(a, b, dims=NN):
    return lax.dot_general(a, b, dims, preferred_element_type=f32)


def _lo(u):
    return pltpu.bitcast(u << 16, f32)


def _hi(u):
    return pltpu.bitcast(u & np.uint32(0xFFFF0000), f32)


SU = {1: (((0, 0), 1), ((1, 1), 1)), 2: (((1, 0), 1), ((1, 1), 1)), 3: (((0, 0), 1),), 4: (((1, 1), 1),),
      5: (((0, 0), 1), ((0, 1), 1)), 6: (((1, 0), 1), ((0, 0), -1)), 7: (((0, 1), 1), ((1, 1), -1))}
SV = {1: (((0, 0), 1), ((1, 1), 1)), 2: (((0, 0), 1),), 3: (((0, 1), 1), ((1, 1), -1)),
      4: (((1, 0), 1), ((0, 0), -1)), 5: (((1, 1), 1),), 6: (((0, 0), 1), ((0, 1), 1)),
      7: (((1, 0), 1), ((1, 1), 1))}
SW = {(0, 0): ((1, 1), (4, 1), (7, 1), (5, -1)), (0, 1): ((3, 1), (5, 1)), (1, 0): ((2, 1), (4, 1)),
      (1, 1): ((1, 1), (3, 1), (6, 1), (2, -1))}
OWN = ((3, 1, 5, 7), (4, 1, 2, 6))


def _lin(terms):
    terms = [(v, c) for v, c in terms if v is not None]
    if not terms:
        return None
    pos = [v for v, c in terms if c > 0]
    neg = [v for v, c in terms if c < 0]
    if pos:
        acc = pos[0]
        for v in pos[1:]:
            acc = acc + v
    else:
        acc, neg = -neg[0], neg[1:]
    for v in neg:
        acc = acc - v
    return acc


def _pre(blocks, table, want):
    if not want[0]:
        return {(): blocks.get((0, 0))}
    h = 2 ** (len(want[0]) - 1)
    out = {}
    for r in sorted({w[0] for w in want}):
        sub = {(i, k): _lin([(blocks.get((a * h + i, b * h + k)), c) for (a, b), c in table[r]])
               for i in range(h) for k in range(h)}
        for rest, v in _pre(sub, table, sorted(w[1:] for w in want if w[0] == r)).items():
            out[(r,) + rest] = v
    return out


def _post(prods, row=None):
    if () in prods:
        return {(0, 0): prods[()]}
    h = 2 ** (len(next(iter(prods))) - 1)
    inner = {r: _post({w[1:]: v for w, v in prods.items() if w[0] == r}, None if row is None else row % h)
             for r in sorted({w[0] for w in prods})}
    out = {}
    for (a, b), terms in SW.items():
        for i in range(h):
            if row is None or row == a * h + i:
                for n in range(h):
                    v = _lin([(inner.get(r, {}).get((i, n)), c) for r, c in terms])
                    if v is not None:
                        out[(a * h + i, b * h + n)] = v
    return out


PRODUCTS = [(a, b) for a in range(1, 8) for b in range(1, 8)]
NPR = len(PRODUCTS)
INDEX = {r: i for i, r in enumerate(PRODUCTS)}


def _token_rows():
    phases = [[(a, b) for a in OWN[p >> 1] for b in OWN[p & 1]] for p in range(G)]
    rows = []
    for p in range(G):
        rows.append({})
        for r in phases[p]:
            users = [q for q in range(G) if r in phases[q]]
            n = SEG // len(users)
            rows[p][r] = (users.index(p) * n, (users.index(p) + 1) * n)
    return rows


def _contributors(rows):
    out = {}
    for p in range(G):
        for r, (a, b) in rows[p].items():
            for rb in range(a // 8, b // 8):
                for key in _post({r: np.zeros(1)}):
                    if p not in out.setdefault(key + (rb,), []):
                        out[key + (rb,)].append(p)
    return out


ROWS = _token_rows()
ADDS = _contributors(ROWS)


def _early(p, r):
    prev = (p - 1) % G
    return all(x in {(0, 1): (1, 3), (0, 0): (7,), (1, 1): (6,), (1, 0): (1, 4)}[(p >> s & 1, prev >> s & 1)]
               for x, s in zip(r, (1, 0)))


def _schedule_last(p):
    groups = sorted(((g, m) for g in range(NG) for m in ((1, 2) if p == G - 1 else (0, 1, 2))),
                    key=lambda gm: gm[0] + 2 * (gm[1] == 2))
    items = [('project', g, m, r) for g, m in groups for r in ROWS[p]]
    head = [it for it in items if _early(p, it[3])][:12]
    items = head + [it for it in items if it not in head]
    rounds = [items[i:i + 4] for i in range(0, len(items), 4)]
    done = {item[1:3]: t + 1 for t, rd in enumerate(rounds) for item in rd}
    soon = [((3, 5), (2, 4))[p >> s & 1] for s in (1, 0)]
    order = sorted(ROWS[p], key=lambda r: not (r[0] in soon[0] and r[1] in soon[1]))
    extra = {}

    def place(t, items):
        while t in extra:
            t += 1
        extra[t] = items
        return t

    step = 2 if p == G - 1 else 3
    scored = [place(done[(g, 1)] + 7, [('scores', G * g + n) for n in range(G)]) for g in range(NG)]
    for g in range(NG):
        t = place(max(done[(g, 2)] + 7, scored[g] + 17), [('values', G * g + n) for n in range(G)]) + 7
        for i in range(0, len(order), 4):
            t = place(t, [('output', g, r) for r in order[i:i + 4]]) + step
    return [item for t in range(max(extra) + 1) for item in extra.get(t, []) + (rounds[t] if t < len(rounds) else [])]


def _schedule(p):
    size = {r: b - a for r, (a, b) in ROWS[p].items()}
    long_ = [r for r in size if size[r] == SEG]
    short = [r for r in size if size[r] == SEG // 2]
    tiny = [r for r in size if size[r] == SEG // 4]
    lead = ([r for r in long_ if _early(p, r)] + [long_[8]])[0]
    pool = [lead, short[4], tiny[0], short[5]]
    rest = [r for r in long_ if r != lead]
    groups = [(g, m) for g in range(NG) for m in (0, 1)] + [(g, 2) for g in range(NG)]
    shared = lambda i, r: [('project', g, m, r) for (g, m) in groups[i:i + 4]]
    own = lambda i, rs: [('project',) + groups[i] + (r,) for r in rs]
    rounds = []
    for i in range(len(groups)):
        a, b, c = own(i, rest[:4]), own(i, short[:4]), own(i, rest[4:])
        if i == 0:
            rounds += [shared(0, pool[0]), shared(0, pool[1]), a, shared(0, pool[2]), c, b, shared(0, pool[3])]
        else:
            rounds += [a, b, c]
        if i // 4 * 4 + 4 < len(groups):
            rounds.append(shared(i // 4 * 4 + 4, pool[i % 4]))
    done = {item[1:3]: t + 1 for t, rd in enumerate(rounds) for item in rd}
    rest, mixed = list(long_), []
    fill = [r for r in size if size[r] < SEG]
    while rest or fill:
        mixed += rest[:1]
        rest = rest[1:]
        if fill and len(fill) >= len(rest) - 1:
            mixed.append(fill.pop(0))
    for g0 in range(0, NG, 4):
        rounds += [[('output', tuple(range(g0, g0 + 4)), r)] for r in mixed]
    extra = {}

    def place(t, items):
        while any(abs(t - u) < 3 for u in extra):
            t += 1
        extra[t] = items
        return t

    scored = [place(done[(g, 1)] + 6 + g % 2, [('scores', G * g + n) for n in range(G)]) for g in range(NG)]
    for g in range(NG):
        place(max(done[(g, 2)] + 6, scored[g] + 5), [('values', G * g + n) for n in range(G)])
    return [item for t, rd in enumerate(rounds) for item in extra.get(t, []) + rd]


def _dft_constants():
    n = np.arange(128)[None, :]
    m = np.arange(64)[:, None]
    angle = lambda k: 2 * np.pi * ((k * n) % D) / D
    even0 = np.concatenate([np.cos(angle(4 * m)), -np.sin(angle(4 * m))])
    even0[64] = np.cos(np.pi * n[0])
    even2 = np.concatenate([np.cos(angle(4 * m + 2)), -np.sin(angle(4 * m + 2))])
    cr = np.concatenate([np.cos(angle(4 * m + 1)), np.cos(angle(4 * m + 3))])
    ci = np.concatenate([-np.sin(angle(4 * m + 1)), np.sin(angle(4 * m + 3))])
    rows = np.concatenate([even0, even2, cr, cr + ci, ci - cr]).astype(np.float32).astype(ml_dtypes.bfloat16)
    rows = rows.view(np.uint16).astype(np.uint32)
    offsets = np.concatenate([128 * np.arange(16), 16 * np.arange(8), np.arange(16)])
    turn = 2 * np.pi * ((offsets[:, None] * n) % S) / S
    return rows[0::2] | (rows[1::2] << 16), np.concatenate([np.cos(turn), -np.sin(turn)]).astype(np.float32)


_DFT_ROWS, _DFT_TURNS = _dft_constants()


def _fft4(a, b, c, d, sign):
    t0 = (a[0] + c[0], a[1] + c[1])
    t1 = (a[0] - c[0], a[1] - c[1])
    t2 = (b[0] + d[0], b[1] + d[1])
    t3 = (b[0] - d[0], b[1] - d[1])
    y0 = (t0[0] + t2[0], t0[1] + t2[1])
    y2 = (t0[0] - t2[0], t0[1] - t2[1])
    p = (t1[0] + t3[1], t1[1] - t3[0])
    q = (t1[0] - t3[1], t1[1] + t3[0])
    return (y0, p, y2, q) if sign < 0 else (y0, q, y2, p)


def _rotate16(z, e, sign):
    if e == 0:
        return z
    r, i = z
    if e == 4:
        return (i, -r) if sign < 0 else (-i, r)
    h = np.float32(np.sqrt(0.5))
    if e == 2:
        return ((r + i) * h, (i - r) * h) if sign < 0 else ((r - i) * h, (r + i) * h)
    if e == 6:
        return ((i - r) * h, (r + i) * (-h)) if sign < 0 else ((r + i) * (-h), (r - i) * h)
    c = np.float32(np.cos(2 * np.pi * e / 16))
    s = np.float32(sign * np.sin(2 * np.pi * e / 16))
    return (r * c - i * s, r * s + i * c)


def _fft16(x, sign):
    col = [_fft4(x[n], x[4 + n], x[8 + n], x[12 + n], sign) for n in range(4)]
    y = [None] * 16
    for k1 in range(4):
        r = _fft4(*[_rotate16(col[n][k1], n * k1, sign) for n in range(4)], sign)
        for k2 in range(4):
            y[k1 + 4 * k2] = r[k2]
    return y


def _kernel(ax_h, wr_h, wi_h, bx_h, mem_h, wq_h, wk_h, wv_h, wo_h, rows_h, turns_h, out_h,
            ax, wr, wi, nyq_r, nyq_i, rows_v, turns, rows_inv, gmat, xs, ts, ya,
            bx, mem0, raw_qkv, raw_o, t_qkv, t_o, tok_lhs, tok, tok_late, att, att_lhs, probs, acc_o, acc_last,
            part_o, yb, sems, row_sems, filt_sems, qkv_sems, wo_sems):
    copy = pltpu.make_async_copy

    def start(copies):
        for c in copies:
            c.start()

    def wait(copies):
        for c in copies:
            c.wait()

    c_turns, c_rows = copy(turns_h, turns, sems.at[0]), copy(rows_h, rows_v, sems.at[2])
    c_ax = [copy(ax_h.bitcast(u32).at[:, j, :], ax.at[j], row_sems.at[j]) for j in range(8)]
    c_filt = [[copy(src.at[pl.ds(128 * b, 128), pl.ds(128 * k, 128)], dst.at[pl.ds(256 * k + 128 * b, 128)], filt_sems.at[b])
               for k in range(16) for src, dst in ((wr_h, wr), (wi_h, wi))] for b in range(2)]
    c_filt[0] += [copy(src.at[pl.ds(256, 1)], dst, filt_sems.at[0]) for src, dst in ((wr_h, nyq_r), (wi_h, nyq_i))]
    c_small = [copy(bx_h.at[pl.ds(0, 3 * RB)], bx.at[pl.ds(0, 3 * RB)], sems.at[1]), copy(mem_h, mem0, sems.at[1])]

    def c_qkv(src, m, g):
        return [copy(src.bitcast(u32).at[:, 2 * g + j, :], raw_qkv.at[m * (H // 2) + 2 * g + j], qkv_sems.at[m * NG + g])
                for j in range(2)]

    c_bx = copy(bx_h.at[pl.ds(3 * RB, S - 3 * RB)], bx.at[pl.ds(3 * RB, S - 3 * RB)], sems.at[3])
    c_ya = [copy(ya.at[j], out_h.bitcast(u32).at[:, j, pl.ds(0, D)], sems.at[4]) for j in range(8)]

    wo_cuts = (0, 4, NG - 1, NG)
    c_wo = [[copy(wo_h.at[pl.ds(a * G * E, (b - a) * G * E), pl.ds(128 * c, 128)],
                  raw_o.at[pl.ds((c * H + a * G) * E, (b - a) * G * E)], wo_sems.at[i]) for c in range(G)]
            for i, (a, b) in enumerate(zip(wo_cuts, wo_cuts[1:]))]

    def c_yb(tile, size):
        rows = pl.ds(tile, size // 16)
        return copy(yb.at[rows], out_h.at[rows, :, pl.ds(D, D)], sems.at[5])

    start([c_turns, c_rows] + c_ax + c_filt[0])
    for ref in (att, acc_last, part_o):
        ref[...] = jnp.zeros(ref.shape, f32)

    c_turns.wait()
    br, bi = turns[16:24, :], turns[56:64, :]
    for s in range(16):
        cr, ci = turns[24 + s:25 + s, :], turns[64 + s:65 + s, :]
        ar, ai = br * cr - bi * ci, br * ci + bi * cr
        gr = jnp.concatenate([ar * turns[a:a + 1, :] - ai * turns[40 + a:41 + a, :] for a in range(16)], axis=0)
        gi = jnp.concatenate([ar * turns[40 + a:41 + a, :] + ai * turns[a:a + 1, :] for a in range(16)], axis=0)
        for c, v in enumerate((gr, gi, gr + gi, gi - gr)):
            gmat[s, c] = v.astype(bf16)
    g_mat = lambda s, c: pltpu.bitcast(gmat.bitcast(u32)[s, c], bf16)
    row_mat = lambda i: pltpu.bitcast(rows_v[64 * i:64 * (i + 1)], bf16)
    inv_mat = lambda i: pltpu.bitcast(rows_inv.bitcast(u32)[64 * i:64 * (i + 1)], bf16)
    c_rows.wait()
    edge = lax.broadcasted_iota(jnp.int32, (128, 128), 0) % 64 == 0
    for i in range(5):
        gain = np.float32(2.0 / (S * D))
        rows_inv[128 * i:128 * (i + 1), :] = (row_mat(i).astype(f32) * (gain if i else jnp.where(edge, gain / 2, gain))).astype(bf16)
    first = lax.broadcasted_iota(jnp.int32, (8, 128), 0) == 0

    def rfft_rows(s):
        unpack = (_lo, _hi)[s % 2]
        x0, x1, x2, x3 = (unpack(ax[s // 2, :, 128 * j:128 * (j + 1)]) for j in range(4))
        s02, s13 = x0 + x2, x1 + x3
        xa = _dot(row_mat(0), (s02 + s13).astype(bf16), NT)
        xb = _dot(row_mat(1), (s02 - s13).astype(bf16), NT)
        d0, d1 = x0 - x2, x3 - x1
        k1 = _dot(row_mat(2), (d0 + d1).astype(bf16), NT)
        er = k1 - _dot(row_mat(3), d1.astype(bf16), NT)
        ei = k1 + _dot(row_mat(4), d0.astype(bf16), NT)
        nyq = xa[64:72]
        return (jnp.concatenate([xa[:64], xb[:64], er, nyq], axis=0),
                jnp.concatenate([jnp.where(first, 0.0, nyq), xa[72:], xb[64:], ei[:64], -ei[64:]], axis=0))

    def dft128(s, re, im):
        k1 = _dot(jnp.concatenate([re[:256] + im, re[256:]], axis=0), g_mat(s, 0))
        xs[s, 0, 0:256, :] = k1[:256] - _dot(im, g_mat(s, 2))
        xs[s, 0, 256:264, :] = k1[256:]
        xs[s, 1] = k1 + _dot(re, g_mat(s, 3))

    wait(c_ax[:2])
    pending = rfft_rows(0)
    for s in range(16):
        if s == 3:
            wait(c_ax[2:4])
            start(c_filt[1] + c_small)
        if s == 7:
            wait(c_ax[4:])
            start(sum((c_qkv(wq_h, 0, g) for g in range(NG)), []))
        ahead = rfft_rows(s + 1) if s < 15 else None
        dft128(s, *pending)
        pending = ahead

    wait(c_filt[0])
    start(sum((c_qkv(wk_h, 1, g) for g in range(NG)), []))

    def spectral_filter(r0, w):
        y = _fft16([(xs[s, 0, pl.ds(r0, 8), :], xs[s, 1, pl.ds(r0, 8), :]) for s in range(16)], -1)
        z = _fft16([(a * w[k][0] - b * w[k][1], a * w[k][1] + b * w[k][0]) for k, (a, b) in enumerate(y)], +1)
        for s in range(16):
            ts[s, 0, pl.ds(r0, 8), :] = z[s][0]
            ts[s, 1, pl.ds(r0, 8), :] = z[s][1]

    nr, ni = nyq_r[...].astype(f32), nyq_i[...].astype(f32)
    spectral_filter(256, [(jnp.broadcast_to(nr[:, 128 * k:128 * (k + 1)], (8, 128)),
                           jnp.broadcast_to(ni[:, 128 * k:128 * (k + 1)], (8, 128))) for k in range(16)])

    def filter_rows(i):
        for p in range(2):
            words = [[ref.bitcast(u32).at[pl.ds(128 * k + 16 * i, 16)][pl.ds(p, 8, stride=2), :]
                      for ref in (wr, wi)] for k in range(16)]
            for g, unpack in enumerate((_lo, _hi)):
                spectral_filter((2 * g + p) * 64 + 8 * i, [(unpack(a), unpack(b)) for a, b in words])

    for i in range(8):
        if i == 4:
            wait(c_filt[1])
        filter_rows(i)

    start(sum((c_qkv(wv_h, 2, g) for g in range(NG)), []))
    wait(c_small)

    def idft128(s):
        real, imag = [], []
        for g in range(4):
            tr, ti = ts[s, 0, 64 * g:64 * (g + 1), :], ts[s, 1, 64 * g:64 * (g + 1), :]
            a, b = (-ti, tr) if g == 3 else (ti, -tr)
            if g == 0:
                a = jnp.concatenate([jnp.where(first, ts[s, 0, 256:264, :], a[:8]), a[8:]], axis=0)
                b = jnp.concatenate([jnp.where(first, ts[s, 1, 256:264, :], b[:8]), b[8:]], axis=0)
            real.append(jnp.concatenate([tr, ti], axis=1))
            imag.append(jnp.concatenate([a, b], axis=1))
        rhs = jnp.concatenate([real[0], imag[0], real[1], imag[1], real[2], real[3], imag[2], imag[3]], axis=0)
        return _dot(jnp.concatenate([g_mat(s, 0), g_mat(s, 1)], axis=1), rhs.astype(bf16), NT)

    def irfft_rows(u):
        e0, e1 = _dot(u[:, 0:128], inv_mat(0)), _dot(u[:, 128:256], inv_mat(1))
        ur, ui = u[:, 256:384], u[:, 384:512]
        k1 = _dot(ur + ui, inv_mat(2))
        d0, d1 = k1 + _dot(ui, inv_mat(4)), k1 - _dot(ur, inv_mat(3))
        p, q = e0 + e1, e0 - e1
        return [p + d0, q - d1, p - d0, q + d1]

    pending = idft128(0)
    for s in range(16):
        ahead = idft128(s + 1) if s < 15 else None
        y = [pltpu.bitcast(v.astype(bf16).astype(f32), u32) for v in irfft_rows(pending)]
        if s % 2:
            for j in range(4):
                ya[s // 2, :, 128 * j:128 * (j + 1)] = (even[j] >> 16) | y[j]
        pending, even = ahead, y

    def w_qkv(g, m, r):
        return pltpu.bitcast(t_qkv.bitcast(u32)[(m * NG + g) * NPR + INDEX[r]], bf16)

    def w_o(g, r):
        return pltpu.bitcast(t_o.bitcast(u32)[g * NPR + INDEX[r]], bf16)

    def stage_tokens(it):
        x = bx[pl.ds(it * RB if isinstance(it, int) else pl.multiple_of(it * RB, RB), RB), :].astype(f32)
        blocks = {(i, k): x[i * SEG:(i + 1) * SEG, k * 128:(k + 1) * 128] for i in range(G) for k in range(G)}
        for r, v in _pre(blocks, SU, PRODUCTS).items():
            tok_lhs[INDEX[r]] = v

    stage_tokens(0)
    start(sum(c_wo, []) + [c_bx])

    @pl.loop(0, 3)
    def _(m):
        shift = jnp.where(m == 1, SHIFT[1], SHIFT[0])

        @pl.loop(0, NG)
        def _(g):
            for i, src in enumerate((wq_h, wk_h, wv_h)):
                pl.when(m == i)(lambda i=i, src=src: wait(c_qkv(src, i, g)))
            for d0 in (0, 16, 48, 32, 64, 80, 112, 96):
                words = {(k, j): raw_qkv[m * (H // 2) + 2 * g + (j ^ (shift >> 1)), k * 128 + d0:k * 128 + d0 + 16, :]
                         for k in range(G) for j in range(2)}
                blocks = {(k, n): (_lo, _hi)[n % 2](words[(k, n // 2)]) for k in range(G) for n in range(G)}
                for r, v in _pre(blocks, SV, PRODUCTS).items():
                    t_qkv[(m * NG + g) * NPR + INDEX[r], d0:d0 + 16, :] = v.astype(bf16)

        for g in range(NG):
            for (i, n), v in _post({r: _dot(tok_lhs[INDEX[r]], w_qkv(g, m, r)) for r in PRODUCTS}).items():
                if i == G - 1:
                    tok_late[m, G * g + (n ^ shift)] = v
                else:
                    tok[m, G * g + (n ^ shift), i * SEG:(i + 1) * SEG, :] = v

    stage_tokens(1)

    @pl.loop(0, NG)
    def _(g):
        for at, copies in zip(wo_cuts, c_wo):
            pl.when(g == at)(lambda copies=copies: wait(copies))
        for e0 in range(0, E, 16):
            blocks = {(k, n): pltpu.bitcast(raw_o.bitcast(u32)[pl.ds(pl.multiple_of(
                (n * H + G * g + k) * (E // 2) + e0 // 2, 8), 8), :], bf16).astype(f32) for k in range(G) for n in range(G)}
            for r, v in _pre(blocks, SV, PRODUCTS).items():
                t_o[g * NPR + INDEX[r], e0:e0 + 16, :] = v.astype(bf16)

    start(c_ya)

    ri = lax.broadcasted_iota(jnp.int32, (L, L), 0)
    ci = lax.broadcasted_iota(jnp.int32, (L, L), 1)
    allowed = (ri < M) | (ri >= ci)
    log2e = np.float32(np.log2(np.e))
    slab = lambda i, rb: slice(i * SEG + rb * 8, i * SEG + rb * 8 + 8)

    def combine(p, prods):
        for rb in range(SEG // 8):
            here = {r: prods[r][rb * 8 - a:rb * 8 + 8 - a] for r, (a, b) in ROWS[p].items() if a <= rb * 8 < b}
            for (i, n), v in _post(here).items():
                yield i, n, rb, v

    def emit(p, prods, it):
        for i, n, rb, v in combine(p, prods):
            where = (slab(i, rb), slice(128 * n, 128 * (n + 1)))
            part_o[where] = v if p == ADDS[(i, n, rb)][0] else v + part_o[where]
        if p == G - 1:
            yb[pl.ds(jnp.maximum(it, 0) * (RB // 16), RB // 16)] = part_o[...].astype(bf16).reshape(RB // 16, 16, D)

    def emit_last(it):
        emit(G - 1, {r: acc_last[INDEX[r], 0:b - a, :] for r, (a, b) in ROWS[G - 1].items()}, it)

    def segment(p, mem, held, ahead=True):
        final = not ahead and p == G - 1
        prods = list(ROWS[p])
        mem_in = _pre({(p, k): mem[:, 128 * k:128 * (k + 1)] for k in range(G)}, SU, prods)
        result, mem_qkv, mem_att, mem_out, acc = {}, {}, {}, {}, {}

        def project(g, m, r):
            a, b = ROWS[p][r]
            lhs = jnp.concatenate([tok_lhs[INDEX[r], a:b, :], mem_in[r]], axis=0) if ahead else mem_in[r]
            result[(g, m, r)] = _dot(lhs, w_qkv(g, m, r))
            if any((g, m, q) not in result for q in prods):
                return
            for n in range(G):
                for rb in range(SEG // 8):
                    if ahead and p and ADDS[(p - 1, n, rb)][-1] == p - 1:
                        h = G * g + (n ^ SHIFT[m])
                        tok[m, h, slab(p - 1, rb), :] = held.pop((m, h, p - 1, rb))
            if p == G - 2:
                for h in range(G * g, G * g + G):
                    tok[m, h, (G - 1) * SEG:G * SEG, :] = tok_late[m, h]
            res = {q: result.pop((g, m, q)) for q in prods}
            for (_, n), v in _post({q: v[-M:] for q, v in res.items()}, p).items():
                mem_qkv[(m, G * g + (n ^ SHIFT[m]))] = v
            for i, n, rb, v in combine(p, res) if ahead else ():
                h, adds = G * g + (n ^ SHIFT[m]), ADDS[(i, n, rb)]
                assert adds[-1] >= i
                if p != adds[0]:
                    v = v + held.pop((m, h, i, rb))
                if p == adds[-1] and p != i:
                    tok[m, h, slab(i, rb), :] = v
                elif p == G - 1:
                    tok_late[m, h, slab(0, rb), :] = v
                else:
                    held[(m, h, i, rb)] = v

        def rows_of(m, h):
            tokens = tok[m, h, p * SEG:(p + 1) * SEG, :]
            return tokens if final and m == 0 else jnp.concatenate([mem_qkv[(m, h)], tokens], axis=0)

        skip = M if final else 0

        def scores(h):
            s = _dot(rows_of(0, h), rows_of(1, h).astype(bf16), NT) * (np.float32(E ** -0.5) * log2e)
            s = jnp.where(allowed[skip:], s, np.float32(-1e9) * log2e)
            e = jnp.exp2(s - jnp.max(s, axis=-1, keepdims=True))
            total = jnp.sum(e, axis=-1, keepdims=True)
            probs[h, skip:, :] = e * pl.reciprocal(total, approx=False, full_range=False)

        def values(h):
            if p == 0 and h % G == 0:
                before = {(i, k): att[h + k, i * SEG:(i + 1) * SEG, :] for i in range(G) for k in range(G)}
                for r, v in _pre(before, SU, PRODUCTS).items():
                    if ahead:
                        att_lhs[h // G * NPR + INDEX[r]] = v
                    else:
                        held[(h // G, r)] = v
            o = _dot(probs[h, skip:, :], rows_of(2, h).astype(bf16))
            if ahead:
                mem_att[h] = o[:M]
                att[h, p * SEG:(p + 1) * SEG, :] = o[M:]
            else:
                mem_att[h] = o

        def output(gs, r):
            a, b = ROWS[p][r]
            for g in gs:
                if g not in mem_out:
                    mem_out[g] = _pre({(p, k): mem_att[G * g + k] for k in range(G)}, SU, prods)
            v = _dot(jnp.concatenate([jnp.concatenate([mem_out[g][r], att_lhs[g * NPR + INDEX[r], a:b, :]], axis=0)
                                      for g in gs], axis=1),
                     jnp.concatenate([w_o(g, r) for g in gs], axis=0))
            if gs[0] > 0:
                v = v + acc_o[INDEX[r], 0:M + b - a, :]
            if gs[-1] < NG - 1:
                acc_o[INDEX[r], 0:M + b - a, :] = v
            acc[r] = v

        def output_last(g, r):
            if g not in mem_out:
                mem_out[g] = _pre({(p, k): mem_att[G * g + k] for k in range(G)}, SU, prods)
            a, b = ROWS[p][r]
            v = _dot(jnp.concatenate([mem_out[g][r], held[(g, r)][a:b]], axis=0), w_o(g, r))
            acc[r] = acc[r] + v if g else v

        run = {'project': project, 'scores': scores, 'values': values, 'output': output if ahead else output_last}
        for item in _schedule(p) if ahead else _schedule_last(p):
            run[item[0]](*item[1:])
        if not ahead:
            emit(p, {r: v[L - skip:] for r, v in acc.items()}, NIT - 2)
            new = _post({r: v[:L - skip] for r, v in acc.items()}, p)
            new = jnp.concatenate([new[(p, n)] for n in range(G)], axis=1)
            r0 = (S - RB + p * SEG) // 16
            yb[r0:r0 + SEG // 16] = new[M - skip:].astype(bf16).reshape(SEG // 16, 16, D)
            return new[:M]
        if p < G - 1:
            emit(p, {r: v[M:] for r, v in acc.items()}, None)
        else:
            for r, (a, b) in ROWS[p].items():
                acc_last[INDEX[r], 0:b - a, :] = acc[r][M:]
        new = _post({r: v[:M] for r, v in acc.items()}, p)
        return jnp.concatenate([new[(p, n)] for n in range(G)], axis=1)

    def iteration(it, mem):
        pl.when(it == 1)(c_bx.wait)
        pl.when(((it & 3) == 2) & (it > 2))(lambda: c_yb((it - 6) * (RB // 16), 4 * RB).start())
        emit_last(it - 2)
        held = {}
        for p in range(G):
            mem = segment(p, mem, held)
        stage_tokens(jnp.minimum(it + 2, NIT - 1))
        return mem

    mem = lax.fori_loop(0, NIT - 1, iteration, mem0[...].astype(f32))

    emit_last(NIT - 3)
    c_yb((S - 4 * RB) // 16, 2 * RB).start()
    held = {}
    for p in range(G):
        mem = segment(p, mem, held, ahead=False)
        if p == G - 2:
            c_yb((S - RB) // 16, RB - SEG).start()
    c_yb((S - 2 * RB) // 16, RB).start()
    c_yb((S - SEG) // 16, SEG).start()
    wait(c_ya)
    c_yb(0, S).wait()


def _scratch():
    vmem = pltpu.VMEM
    return [
        vmem((8, 128, D), u32), vmem((16 * 256, 128), bf16), vmem((16 * 256, 128), bf16),
        vmem((1, S), bf16), vmem((1, S), bf16),
        vmem(_DFT_ROWS.shape, u32), vmem(_DFT_TURNS.shape, f32), vmem((5 * 128, 128), bf16),
        vmem((16, 4, 128, 128), bf16),
        vmem((16, 2, 264, 128), f32), vmem((16, 2, 264, 128), f32), vmem((8, 128, D), u32),
        vmem((S, D), bf16), vmem((M, D), bf16),
        vmem((3 * H // 2, D, E), u32), vmem((G * H * E, 128), bf16),
        vmem((3 * NG * NPR, 128, E), bf16), vmem((NG * NPR, E, 128), bf16),
        vmem((NPR, SEG, 128), f32), vmem((3, H, RB, E), f32), vmem((3, H, SEG, E), f32),
        vmem((H, RB, E), f32), vmem((NG * NPR, SEG, E), f32), vmem((H, L, L), f32),
        vmem((NPR, L, 128), f32), vmem((NPR, SEG, 128), f32),
        vmem((RB, D), f32), vmem((S // 16, 16, D), bf16),
        pltpu.SemaphoreType.DMA((6,)), pltpu.SemaphoreType.DMA((8,)),
        pltpu.SemaphoreType.DMA((2,)), pltpu.SemaphoreType.DMA((3 * NG,)),
        pltpu.SemaphoreType.DMA((3,)),
    ]


@jax.jit
def pallas_concat_heads__spectral_gfnet__memory_aug_recurrent_mem_tr__prompt_kernel(
    A_x: jax.Array,
    A_w_r: jax.Array,
    A_w_i: jax.Array,
    B_x: jax.Array,
    B_mem0: jax.Array,
    B_Wq: jax.Array,
    B_Wk: jax.Array,
    B_Wv: jax.Array,
    B_Wo: jax.Array,
    B_seg_len: jax.Array,
):
    del B_seg_len
    hbm = pl.BlockSpec(memory_space=pl.ANY)
    out = pl.pallas_call(
        _kernel,
        out_shape=jax.ShapeDtypeStruct((S // 16, 16, 2 * D), bf16),
        in_specs=[hbm] * 11,
        out_specs=hbm,
        scratch_shapes=_scratch(),
        compiler_params=pltpu.CompilerParams(vmem_limit_bytes=120 * 2 ** 20),
    )(A_x.reshape(S // 16, 16, D), A_w_r.T, A_w_i.T, B_x.reshape(S, D), B_mem0.reshape(M, D),
      B_Wq, B_Wk, B_Wv, B_Wo.reshape(H * E, D), _DFT_ROWS, _DFT_TURNS)
    return out.reshape(1, S, 2 * D)
```

```python
import jax
import jax.numpy as jnp
import ml_dtypes
import numpy as np
from jax import lax
import jax.experimental.pallas as pl
import jax.experimental.pallas.tpu as pltpu

S, D, H, E, M, SEG = 2048, 512, 32, 128, 8, 32
L = M + SEG
G = 4
NG = H // G
RB = G * SEG
NIT = S // RB
f32, bf16, u32 = jnp.float32, jnp.bfloat16, jnp.uint32
NN = (((1,), (0,)), ((), ()))
NT = (((1,), (1,)), ((), ()))


def _dot(a, b, dims=NN):
    return lax.dot_general(a, b, dims, preferred_element_type=f32)


def _lo(u):
    return pltpu.bitcast(u << 16, f32)


def _hi(u):
    return pltpu.bitcast(u & np.uint32(0xFFFF0000), f32)


SU = {1: (((0, 0), 1), ((1, 1), 1)), 2: (((1, 0), 1), ((1, 1), 1)), 3: (((0, 0), 1),), 4: (((1, 1), 1),),
      5: (((0, 0), 1), ((0, 1), 1)), 6: (((1, 0), 1), ((0, 0), -1)), 7: (((0, 1), 1), ((1, 1), -1))}
SV = {1: (((0, 0), 1), ((1, 1), 1)), 2: (((0, 0), 1),), 3: (((0, 1), 1), ((1, 1), -1)),
      4: (((1, 0), 1), ((0, 0), -1)), 5: (((1, 1), 1),), 6: (((0, 0), 1), ((0, 1), 1)),
      7: (((1, 0), 1), ((1, 1), 1))}
SW = {(0, 0): ((1, 1), (4, 1), (7, 1), (5, -1)), (0, 1): ((3, 1), (5, 1)), (1, 0): ((2, 1), (4, 1)),
      (1, 1): ((1, 1), (3, 1), (6, 1), (2, -1))}
OWN = ((3, 1, 5, 7), (4, 1, 2, 6))


def _lin(terms):
    terms = [(v, c) for v, c in terms if v is not None]
    if not terms:
        return None
    pos = [v for v, c in terms if c > 0]
    neg = [v for v, c in terms if c < 0]
    if pos:
        acc = pos[0]
        for v in pos[1:]:
            acc = acc + v
    else:
        acc, neg = -neg[0], neg[1:]
    for v in neg:
        acc = acc - v
    return acc


def _pre(blocks, table, want):
    if not want[0]:
        return {(): blocks.get((0, 0))}
    h = 2 ** (len(want[0]) - 1)
    out = {}
    for r in sorted({w[0] for w in want}):
        sub = {(i, k): _lin([(blocks.get((a * h + i, b * h + k)), c) for (a, b), c in table[r]])
               for i in range(h) for k in range(h)}
        for rest, v in _pre(sub, table, sorted(w[1:] for w in want if w[0] == r)).items():
            out[(r,) + rest] = v
    return out


def _post(prods, row=None):
    if () in prods:
        return {(0, 0): prods[()]}
    h = 2 ** (len(next(iter(prods))) - 1)
    inner = {r: _post({w[1:]: v for w, v in prods.items() if w[0] == r}, None if row is None else row % h)
             for r in sorted({w[0] for w in prods})}
    out = {}
    for (a, b), terms in SW.items():
        for i in range(h):
            if row is None or row == a * h + i:
                for n in range(h):
                    v = _lin([(inner.get(r, {}).get((i, n)), c) for r, c in terms])
                    if v is not None:
                        out[(a * h + i, b * h + n)] = v
    return out


PRODUCTS = [(a, b) for a in range(1, 8) for b in range(1, 8)]
NPR = len(PRODUCTS)
INDEX = {r: i for i, r in enumerate(PRODUCTS)}


def _token_rows():
    phases = [[(a, b) for a in OWN[p >> 1] for b in OWN[p & 1]] for p in range(G)]
    rows = []
    for p in range(G):
        rows.append({})
        for r in phases[p]:
            users = [q for q in range(G) if r in phases[q]]
            n = SEG // len(users)
            rows[p][r] = (users.index(p) * n, (users.index(p) + 1) * n)
    return rows


def _contributors(rows):
    out = {}
    for p in range(G):
        for r, (a, b) in rows[p].items():
            for rb in range(a // 8, b // 8):
                for key in _post({r: np.zeros(1)}):
                    if p not in out.setdefault(key + (rb,), []):
                        out[key + (rb,)].append(p)
    return out


ROWS = _token_rows()
ADDS = _contributors(ROWS)


def _early(p, r):
    prev = (p - 1) % G
    return all(x in {(0, 1): (1, 3), (0, 0): (7,), (1, 1): (6,), (1, 0): (1, 4)}[(p >> s & 1, prev >> s & 1)]
               for x, s in zip(r, (1, 0)))


def _schedule_last(p):
    groups = sorted(((g, m) for g in range(NG) for m in ((1, 2) if p == G - 1 else (0, 1, 2))),
                    key=lambda gm: gm[0] + 2 * (gm[1] == 2))
    items = [('project', g, m, r) for g, m in groups for r in ROWS[p]]
    head = [it for it in items if _early(p, it[3])][:12]
    items = head + [it for it in items if it not in head]
    rounds = [items[i:i + 4] for i in range(0, len(items), 4)]
    done = {item[1:3]: t + 1 for t, rd in enumerate(rounds) for item in rd}
    soon = [((3, 5), (2, 4))[p >> s & 1] for s in (1, 0)]
    order = sorted(ROWS[p], key=lambda r: not (r[0] in soon[0] and r[1] in soon[1]))
    extra = {}

    def place(t, items):
        while t in extra:
            t += 1
        extra[t] = items
        return t

    step = 2 if p == G - 1 else 3
    scored = [place(done[(g, 1)] + 7, [('scores', G * g + n) for n in range(G)]) for g in range(NG)]
    for g in range(NG):
        t = place(max(done[(g, 2)] + 7, scored[g] + 17), [('values', G * g + n) for n in range(G)]) + 7
        for i in range(0, len(order), 4):
            t = place(t, [('output', g, r) for r in order[i:i + 4]]) + step
    return [item for t in range(max(extra) + 1) for item in extra.get(t, []) + (rounds[t] if t < len(rounds) else [])]


def _schedule(p):
    size = {r: b - a for r, (a, b) in ROWS[p].items()}
    long_ = [r for r in size if size[r] == SEG]
    short = [r for r in size if size[r] == SEG // 2]
    tiny = [r for r in size if size[r] == SEG // 4]
    lead = ([r for r in long_ if _early(p, r)] + [long_[8]])[0]
    pool = [lead, short[4], tiny[0], short[5]]
    rest = [r for r in long_ if r != lead]
    groups = [(g, m) for g in range(NG) for m in (0, 1)] + [(g, 2) for g in range(NG)]
    shared = lambda i, r: [('project', g, m, r) for (g, m) in groups[i:i + 4]]
    own = lambda i, rs: [('project',) + groups[i] + (r,) for r in rs]
    rounds = []
    for i in range(len(groups)):
        a, b, c = own(i, rest[:4]), own(i, short[:4]), own(i, rest[4:])
        if i == 0:
            rounds += [shared(0, pool[0]), shared(0, pool[1]), a, shared(0, pool[2]), c, b, shared(0, pool[3])]
        else:
            rounds += [a, b, c]
        if i // 4 * 4 + 4 < len(groups):
            rounds.append(shared(i // 4 * 4 + 4, pool[i % 4]))
    done = {item[1:3]: t + 1 for t, rd in enumerate(rounds) for item in rd}
    rest, mixed = list(long_), []
    fill = [r for r in size if size[r] < SEG]
    while rest or fill:
        mixed += rest[:1]
        rest = rest[1:]
        if fill and len(fill) >= len(rest) - 1:
            mixed.append(fill.pop(0))
    for g0 in range(0, NG, 4):
        rounds += [[('output', tuple(range(g0, g0 + 4)), r)] for r in mixed]
    extra = {}

    def place(t, items):
        while any(abs(t - u) < 3 for u in extra):
            t += 1
        extra[t] = items
        return t

    scored = [place(done[(g, 1)] + 6 + g % 2, [('scores', G * g + n) for n in range(G)]) for g in range(NG)]
    for g in range(NG):
        place(max(done[(g, 2)] + 6, scored[g] + 5), [('values', G * g + n) for n in range(G)])
    return [item for t, rd in enumerate(rounds) for item in extra.get(t, []) + rd]


def _dft_constants():
    n = np.arange(128)[None, :]
    m = np.arange(64)[:, None]
    angle = lambda k: 2 * np.pi * ((k * n) % D) / D
    even0 = np.concatenate([np.cos(angle(4 * m)), -np.sin(angle(4 * m))])
    even0[64] = np.cos(np.pi * n[0])
    even2 = np.concatenate([np.cos(angle(4 * m + 2)), -np.sin(angle(4 * m + 2))])
    cr = np.concatenate([np.cos(angle(4 * m + 1)), np.cos(angle(4 * m + 3))])
    ci = np.concatenate([-np.sin(angle(4 * m + 1)), np.sin(angle(4 * m + 3))])
    rows = np.concatenate([even0, even2, cr, cr + ci, ci - cr]).astype(np.float32).astype(ml_dtypes.bfloat16)
    rows = rows.view(np.uint16).astype(np.uint32)
    offsets = np.concatenate([128 * np.arange(16), 16 * np.arange(8), np.arange(16)])
    turn = 2 * np.pi * ((offsets[:, None] * n) % S) / S
    return rows[0::2] | (rows[1::2] << 16), np.concatenate([np.cos(turn), -np.sin(turn)]).astype(np.float32)


_DFT_ROWS, _DFT_TURNS = _dft_constants()


def _fft4(a, b, c, d, sign):
    t0 = (a[0] + c[0], a[1] + c[1])
    t1 = (a[0] - c[0], a[1] - c[1])
    t2 = (b[0] + d[0], b[1] + d[1])
    t3 = (b[0] - d[0], b[1] - d[1])
    y0 = (t0[0] + t2[0], t0[1] + t2[1])
    y2 = (t0[0] - t2[0], t0[1] - t2[1])
    p = (t1[0] + t3[1], t1[1] - t3[0])
    q = (t1[0] - t3[1], t1[1] + t3[0])
    return (y0, p, y2, q) if sign < 0 else (y0, q, y2, p)


def _rotate16(z, e, sign):
    if e == 0:
        return z
    r, i = z
    if e == 4:
        return (i, -r) if sign < 0 else (-i, r)
    h = np.float32(np.sqrt(0.5))
    if e == 2:
        return ((r + i) * h, (i - r) * h) if sign < 0 else ((r - i) * h, (r + i) * h)
    if e == 6:
        return ((i - r) * h, (r + i) * (-h)) if sign < 0 else ((r + i) * (-h), (r - i) * h)
    c = np.float32(np.cos(2 * np.pi * e / 16))
    s = np.float32(sign * np.sin(2 * np.pi * e / 16))
    return (r * c - i * s, r * s + i * c)


def _fft16(x, sign):
    col = [_fft4(x[n], x[4 + n], x[8 + n], x[12 + n], sign) for n in range(4)]
    y = [None] * 16
    for k1 in range(4):
        r = _fft4(*[_rotate16(col[n][k1], n * k1, sign) for n in range(4)], sign)
        for k2 in range(4):
            y[k1 + 4 * k2] = r[k2]
    return y


def _kernel(ax_h, wr_h, wi_h, bx_h, mem_h, wq_h, wk_h, wv_h, wo_h, rows_h, turns_h, out_h,
            ax, wr, wi, nyq_r, nyq_i, rows_v, turns, rows_inv, gmat, xs, ts, ya,
            bx, mem0, raw_qkv, raw_o, t_qkv, t_o, tok_lhs, tok, tok_late, att, att_lhs, probs, acc_o, acc_last,
            part_o, yb, sems, row_sems, filt_sems, qkv_sems, wo_sems):
    copy = pltpu.make_async_copy

    def start(copies):
        for c in copies:
            c.start()

    def wait(copies):
        for c in copies:
            c.wait()

    c_turns, c_rows = copy(turns_h, turns, sems.at[0]), copy(rows_h, rows_v, sems.at[2])
    c_ax = [copy(ax_h.bitcast(u32).at[:, j, :], ax.at[j], row_sems.at[j]) for j in range(8)]
    c_filt = [[copy(src.at[pl.ds(128 * b, 128), pl.ds(128 * k, 128)], dst.at[pl.ds(256 * k + 128 * b, 128)], filt_sems.at[b])
               for k in range(16) for src, dst in ((wr_h, wr), (wi_h, wi))] for b in range(2)]
    c_filt[0] += [copy(src.at[pl.ds(256, 1)], dst, filt_sems.at[0]) for src, dst in ((wr_h, nyq_r), (wi_h, nyq_i))]
    c_small = [copy(bx_h.at[pl.ds(0, 3 * RB)], bx.at[pl.ds(0, 3 * RB)], sems.at[1]), copy(mem_h, mem0, sems.at[1])]

    def c_qkv(src, m, g):
        return [copy(src.bitcast(u32).at[:, 2 * g + j, :], raw_qkv.at[m * (H // 2) + 2 * g + j], qkv_sems.at[m * NG + g])
                for j in range(2)]

    c_bx = copy(bx_h.at[pl.ds(3 * RB, S - 3 * RB)], bx.at[pl.ds(3 * RB, S - 3 * RB)], sems.at[3])
    c_ya = [copy(ya.at[j], out_h.bitcast(u32).at[:, j, pl.ds(0, D)], sems.at[4]) for j in range(8)]

    wo_cuts = (0, 4, NG - 1, NG)
    c_wo = [[copy(wo_h.at[pl.ds(a * G * E, (b - a) * G * E), pl.ds(128 * c, 128)],
                  raw_o.at[pl.ds((c * H + a * G) * E, (b - a) * G * E)], wo_sems.at[i]) for c in range(G)]
            for i, (a, b) in enumerate(zip(wo_cuts, wo_cuts[1:]))]

    def c_yb(tile, size):
        rows = pl.ds(tile, size // 16)
        return copy(yb.at[rows], out_h.at[rows, :, pl.ds(D, D)], sems.at[5])

    start([c_turns, c_rows] + c_ax + c_filt[0])
    for ref in (att, acc_last, part_o):
        ref[...] = jnp.zeros(ref.shape, f32)

    c_turns.wait()
    br, bi = turns[16:24, :], turns[56:64, :]
    for s in range(16):
        cr, ci = turns[24 + s:25 + s, :], turns[64 + s:65 + s, :]
        ar, ai = br * cr - bi * ci, br * ci + bi * cr
        gr = jnp.concatenate([ar * turns[a:a + 1, :] - ai * turns[40 + a:41 + a, :] for a in range(16)], axis=0)
        gi = jnp.concatenate([ar * turns[40 + a:41 + a, :] + ai * turns[a:a + 1, :] for a in range(16)], axis=0)
        for c, v in enumerate((gr, gi, gr + gi, gi - gr)):
            gmat[s, c] = v.astype(bf16)
    g_mat = lambda s, c: pltpu.bitcast(gmat.bitcast(u32)[s, c], bf16)
    row_mat = lambda i: pltpu.bitcast(rows_v[64 * i:64 * (i + 1)], bf16)
    inv_mat = lambda i: pltpu.bitcast(rows_inv.bitcast(u32)[64 * i:64 * (i + 1)], bf16)
    c_rows.wait()
    edge = lax.broadcasted_iota(jnp.int32, (128, 128), 0) % 64 == 0
    for i in range(5):
        gain = np.float32(2.0 / (S * D))
        rows_inv[128 * i:128 * (i + 1), :] = (row_mat(i).astype(f32) * (gain if i else jnp.where(edge, gain / 2, gain))).astype(bf16)
    first = lax.broadcasted_iota(jnp.int32, (8, 128), 0) == 0

    def rfft_rows(s):
        unpack = (_lo, _hi)[s % 2]
        x0, x1, x2, x3 = (unpack(ax[s // 2, :, 128 * j:128 * (j + 1)]) for j in range(4))
        s02, s13 = x0 + x2, x1 + x3
        xa = _dot(row_mat(0), (s02 + s13).astype(bf16), NT)
        xb = _dot(row_mat(1), (s02 - s13).astype(bf16), NT)
        d0, d1 = x0 - x2, x3 - x1
        k1 = _dot(row_mat(2), (d0 + d1).astype(bf16), NT)
        er = k1 - _dot(row_mat(3), d1.astype(bf16), NT)
        ei = k1 + _dot(row_mat(4), d0.astype(bf16), NT)
        nyq = xa[64:72]
        return (jnp.concatenate([xa[:64], xb[:64], er, nyq], axis=0),
                jnp.concatenate([jnp.where(first, 0.0, nyq), xa[72:], xb[64:], ei[:64], -ei[64:]], axis=0))

    def dft128(s, re, im):
        k1 = _dot(jnp.concatenate([re[:256] + im, re[256:]], axis=0), g_mat(s, 0))
        xs[s, 0, 0:256, :] = k1[:256] - _dot(im, g_mat(s, 2))
        xs[s, 0, 256:264, :] = k1[256:]
        xs[s, 1] = k1 + _dot(re, g_mat(s, 3))

    wait(c_ax[:2])
    pending = rfft_rows(0)
    for s in range(16):
        if s == 3:
            wait(c_ax[2:4])
            start(c_filt[1] + c_small)
        if s == 7:
            wait(c_ax[4:])
            start(sum((c_qkv(wq_h, 0, g) for g in range(NG)), []))
        ahead = rfft_rows(s + 1) if s < 15 else None
        dft128(s, *pending)
        pending = ahead

    wait(c_filt[0])
    start(sum((c_qkv(wk_h, 1, g) for g in range(NG)), []))

    def spectral_filter(r0, w):
        y = _fft16([(xs[s, 0, pl.ds(r0, 8), :], xs[s, 1, pl.ds(r0, 8), :]) for s in range(16)], -1)
        z = _fft16([(a * w[k][0] - b * w[k][1], a * w[k][1] + b * w[k][0]) for k, (a, b) in enumerate(y)], +1)
        for s in range(16):
            ts[s, 0, pl.ds(r0, 8), :] = z[s][0]
            ts[s, 1, pl.ds(r0, 8), :] = z[s][1]

    nr, ni = nyq_r[...].astype(f32), nyq_i[...].astype(f32)
    spectral_filter(256, [(jnp.broadcast_to(nr[:, 128 * k:128 * (k + 1)], (8, 128)),
                           jnp.broadcast_to(ni[:, 128 * k:128 * (k + 1)], (8, 128))) for k in range(16)])

    def filter_rows(i):
        for p in range(2):
            words = [[ref.bitcast(u32).at[pl.ds(128 * k + 16 * i, 16)][pl.ds(p, 8, stride=2), :]
                      for ref in (wr, wi)] for k in range(16)]
            for g, unpack in enumerate((_lo, _hi)):
                spectral_filter((2 * g + p) * 64 + 8 * i, [(unpack(a), unpack(b)) for a, b in words])

    for i in range(8):
        if i == 4:
            wait(c_filt[1])
        filter_rows(i)

    start(sum((c_qkv(wv_h, 2, g) for g in range(NG)), []))
    wait(c_small)

    def idft128(s):
        real, imag = [], []
        for g in range(4):
            tr, ti = ts[s, 0, 64 * g:64 * (g + 1), :], ts[s, 1, 64 * g:64 * (g + 1), :]
            a, b = (-ti, tr) if g == 3 else (ti, -tr)
            if g == 0:
                a = jnp.concatenate([jnp.where(first, ts[s, 0, 256:264, :], a[:8]), a[8:]], axis=0)
                b = jnp.concatenate([jnp.where(first, ts[s, 1, 256:264, :], b[:8]), b[8:]], axis=0)
            real.append(jnp.concatenate([tr, ti], axis=1))
            imag.append(jnp.concatenate([a, b], axis=1))
        rhs = jnp.concatenate([real[0], imag[0], real[1], imag[1], real[2], real[3], imag[2], imag[3]], axis=0)
        return _dot(jnp.concatenate([g_mat(s, 0), g_mat(s, 1)], axis=1), rhs.astype(bf16), NT)

    def irfft_rows(u):
        e0, e1 = _dot(u[:, 0:128], inv_mat(0)), _dot(u[:, 128:256], inv_mat(1))
        ur, ui = u[:, 256:384], u[:, 384:512]
        k1 = _dot(ur + ui, inv_mat(2))
        d0, d1 = k1 + _dot(ui, inv_mat(4)), k1 - _dot(ur, inv_mat(3))
        p, q = e0 + e1, e0 - e1
        return [p + d0, q - d1, p - d0, q + d1]

    pending = idft128(0)
    for s in range(16):
        ahead = idft128(s + 1) if s < 15 else None
        y = [pltpu.bitcast(v.astype(bf16).astype(f32), u32) for v in irfft_rows(pending)]
        if s % 2:
            for j in range(4):
                ya[s // 2, :, 128 * j:128 * (j + 1)] = (even[j] >> 16) | y[j]
        pending, even = ahead, y

    def w_qkv(g, m, r):
        return pltpu.bitcast(t_qkv.bitcast(u32)[(m * NG + g) * NPR + INDEX[r]], bf16)

    def w_o(g, r):
        return pltpu.bitcast(t_o.bitcast(u32)[g * NPR + INDEX[r]], bf16)

    def stage_tokens(it):
        x = bx[pl.ds(it * RB if isinstance(it, int) else pl.multiple_of(it * RB, RB), RB), :].astype(f32)
        blocks = {(i, k): x[i * SEG:(i + 1) * SEG, k * 128:(k + 1) * 128] for i in range(G) for k in range(G)}
        for r, v in _pre(blocks, SU, PRODUCTS).items():
            tok_lhs[INDEX[r]] = v

    stage_tokens(0)
    start(sum(c_wo, []) + [c_bx])

    @pl.loop(0, 3)
    def _(m):
        @pl.loop(0, NG)
        def _(g):
            for i, src in enumerate((wq_h, wk_h, wv_h)):
                pl.when(m == i)(lambda i=i, src=src: wait(c_qkv(src, i, g)))
            for d0 in (0, 16, 48, 32, 64, 80, 112, 96):
                words = {(k, j): raw_qkv[m * (H // 2) + 2 * g + j, k * 128 + d0:k * 128 + d0 + 16, :]
                         for k in range(G) for j in range(2)}
                blocks = {(k, n): (_lo, _hi)[n % 2](words[(k, n // 2)]) for k in range(G) for n in range(G)}
                for r, v in _pre(blocks, SV, PRODUCTS).items():
                    t_qkv[(m * NG + g) * NPR + INDEX[r], d0:d0 + 16, :] = v.astype(bf16)

        for g in range(NG):
            for (i, n), v in _post({r: _dot(tok_lhs[INDEX[r]], w_qkv(g, m, r)) for r in PRODUCTS}).items():
                if i == G - 1:
                    tok_late[m, G * g + n] = v
                else:
                    tok[m, G * g + n, i * SEG:(i + 1) * SEG, :] = v

    stage_tokens(1)

    @pl.loop(0, NG)
    def _(g):
        for at, copies in zip(wo_cuts, c_wo):
            pl.when(g == at)(lambda copies=copies: wait(copies))
        for e0 in range(0, E, 16):
            blocks = {(k, n): pltpu.bitcast(raw_o.bitcast(u32)[pl.ds(pl.multiple_of(
                (n * H + G * g + k) * (E // 2) + e0 // 2, 8), 8), :], bf16).astype(f32) for k in range(G) for n in range(G)}
            for r, v in _pre(blocks, SV, PRODUCTS).items():
                t_o[g * NPR + INDEX[r], e0:e0 + 16, :] = v.astype(bf16)

    start(c_ya)

    ri = lax.broadcasted_iota(jnp.int32, (L, L), 0)
    ci = lax.broadcasted_iota(jnp.int32, (L, L), 1)
    allowed = (ri < M) | (ri >= ci)
    log2e = np.float32(np.log2(np.e))
    slab = lambda i, rb: slice(i * SEG + rb * 8, i * SEG + rb * 8 + 8)

    def combine(p, prods):
        for rb in range(SEG // 8):
            here = {r: prods[r][rb * 8 - a:rb * 8 + 8 - a] for r, (a, b) in ROWS[p].items() if a <= rb * 8 < b}
            for (i, n), v in _post(here).items():
                yield i, n, rb, v

    def emit(p, prods, it):
        for i, n, rb, v in combine(p, prods):
            where = (slab(i, rb), slice(128 * n, 128 * (n + 1)))
            part_o[where] = v if p == ADDS[(i, n, rb)][0] else v + part_o[where]
        if p == G - 1:
            yb[pl.ds(jnp.maximum(it, 0) * (RB // 16), RB // 16)] = part_o[...].astype(bf16).reshape(RB // 16, 16, D)

    def emit_last(it):
        emit(G - 1, {r: acc_last[INDEX[r], 0:b - a, :] for r, (a, b) in ROWS[G - 1].items()}, it)

    def segment(p, mem, held, ahead=True):
        final = not ahead and p == G - 1
        prods = list(ROWS[p])
        mem_in = _pre({(p, k): mem[:, 128 * k:128 * (k + 1)] for k in range(G)}, SU, prods)
        result, mem_qkv, mem_att, mem_out, acc = {}, {}, {}, {}, {}

        def project(g, m, r):
            a, b = ROWS[p][r]
            lhs = jnp.concatenate([tok_lhs[INDEX[r], a:b, :], mem_in[r]], axis=0) if ahead else mem_in[r]
            result[(g, m, r)] = _dot(lhs, w_qkv(g, m, r))
            if any((g, m, q) not in result for q in prods):
                return
            for n in range(G):
                for rb in range(SEG // 8):
                    if ahead and p and ADDS[(p - 1, n, rb)][-1] == p - 1:
                        h = G * g + n
                        tok[m, h, slab(p - 1, rb), :] = held.pop((m, h, p - 1, rb))
            if p == G - 2:
                for h in range(G * g, G * g + G):
                    tok[m, h, (G - 1) * SEG:G * SEG, :] = tok_late[m, h]
            res = {q: result.pop((g, m, q)) for q in prods}
            for (_, n), v in _post({q: v[-M:] for q, v in res.items()}, p).items():
                mem_qkv[(m, G * g + n)] = v
            for i, n, rb, v in combine(p, res) if ahead else ():
                h, adds = G * g + n, ADDS[(i, n, rb)]
                assert adds[-1] >= i
                if p != adds[0]:
                    v = v + held.pop((m, h, i, rb))
                if p == adds[-1] and p != i:
                    tok[m, h, slab(i, rb), :] = v
                elif p == G - 1:
                    tok_late[m, h, slab(0, rb), :] = v
                else:
                    held[(m, h, i, rb)] = v

        def rows_of(m, h):
            tokens = tok[m, h, p * SEG:(p + 1) * SEG, :]
            return tokens if final and m == 0 else jnp.concatenate([mem_qkv[(m, h)], tokens], axis=0)

        skip = M if final else 0

        def scores(h):
            s = _dot(rows_of(0, h), rows_of(1, h).astype(bf16), NT) * (np.float32(E ** -0.5) * log2e)
            s = jnp.where(allowed[skip:], s, np.float32(-1e9) * log2e)
            e = jnp.exp2(s - jnp.max(s, axis=-1, keepdims=True))
            total = jnp.sum(e, axis=-1, keepdims=True)
            probs[h, skip:, :] = e * pl.reciprocal(total, approx=False, full_range=False)

        def values(h):
            if p == 0 and h % G == 0:
                before = {(i, k): att[h + k, i * SEG:(i + 1) * SEG, :] for i in range(G) for k in range(G)}
                for r, v in _pre(before, SU, PRODUCTS).items():
                    if ahead:
                        att_lhs[h // G * NPR + INDEX[r]] = v
                    else:
                        held[(h // G, r)] = v
            o = _dot(probs[h, skip:, :], rows_of(2, h).astype(bf16))
            if ahead:
                mem_att[h] = o[:M]
                att[h, p * SEG:(p + 1) * SEG, :] = o[M:]
            else:
                mem_att[h] = o

        def output(gs, r):
            a, b = ROWS[p][r]
            for g in gs:
                if g not in mem_out:
                    mem_out[g] = _pre({(p, k): mem_att[G * g + k] for k in range(G)}, SU, prods)
            v = _dot(jnp.concatenate([jnp.concatenate([mem_out[g][r], att_lhs[g * NPR + INDEX[r], a:b, :]], axis=0)
                                      for g in gs], axis=1),
                     jnp.concatenate([w_o(g, r) for g in gs], axis=0))
            if gs[0] > 0:
                v = v + acc_o[INDEX[r], 0:M + b - a, :]
            if gs[-1] < NG - 1:
                acc_o[INDEX[r], 0:M + b - a, :] = v
            acc[r] = v

        def output_last(g, r):
            if g not in mem_out:
                mem_out[g] = _pre({(p, k): mem_att[G * g + k] for k in range(G)}, SU, prods)
            a, b = ROWS[p][r]
            v = _dot(jnp.concatenate([mem_out[g][r], held[(g, r)][a:b]], axis=0), w_o(g, r))
            acc[r] = acc[r] + v if g else v

        run = {'project': project, 'scores': scores, 'values': values, 'output': output if ahead else output_last}
        for item in _schedule(p) if ahead else _schedule_last(p):
            run[item[0]](*item[1:])
        if not ahead:
            emit(p, {r: v[L - skip:] for r, v in acc.items()}, NIT - 2)
            new = _post({r: v[:L - skip] for r, v in acc.items()}, p)
            new = jnp.concatenate([new[(p, n)] for n in range(G)], axis=1)
            r0 = (S - RB + p * SEG) // 16
            yb[r0:r0 + SEG // 16] = new[M - skip:].astype(bf16).reshape(SEG // 16, 16, D)
            return new[:M]
        if p < G - 1:
            emit(p, {r: v[M:] for r, v in acc.items()}, None)
        else:
            for r, (a, b) in ROWS[p].items():
                acc_last[INDEX[r], 0:b - a, :] = acc[r][M:]
        new = _post({r: v[:M] for r, v in acc.items()}, p)
        return jnp.concatenate([new[(p, n)] for n in range(G)], axis=1)

    def iteration(it, mem):
        pl.when(it == 1)(c_bx.wait)
        pl.when(((it & 3) == 2) & (it > 2))(lambda: c_yb((it - 6) * (RB // 16), 4 * RB).start())
        emit_last(it - 2)
        held = {}
        for p in range(G):
            mem = segment(p, mem, held)
        stage_tokens(jnp.minimum(it + 2, NIT - 1))
        return mem

    mem = lax.fori_loop(0, NIT - 1, iteration, mem0[...].astype(f32))

    emit_last(NIT - 3)
    c_yb((S - 4 * RB) // 16, 2 * RB).start()
    held = {}
    for p in range(G):
        mem = segment(p, mem, held, ahead=False)
        if p == G - 2:
            c_yb((S - RB) // 16, RB - SEG).start()
    c_yb((S - 2 * RB) // 16, RB).start()
    c_yb((S - SEG) // 16, SEG).start()
    wait(c_ya)
    c_yb(0, S).wait()


def _scratch():
    vmem = pltpu.VMEM
    return [
        vmem((8, 128, D), u32), vmem((16 * 256, 128), bf16), vmem((16 * 256, 128), bf16),
        vmem((1, S), bf16), vmem((1, S), bf16),
        vmem(_DFT_ROWS.shape, u32), vmem(_DFT_TURNS.shape, f32), vmem((5 * 128, 128), bf16),
        vmem((16, 4, 128, 128), bf16),
        vmem((16, 2, 264, 128), f32), vmem((16, 2, 264, 128), f32), vmem((8, 128, D), u32),
        vmem((S, D), bf16), vmem((M, D), bf16),
        vmem((3 * H // 2, D, E), u32), vmem((G * H * E, 128), bf16),
        vmem((3 * NG * NPR, 128, E), bf16), vmem((NG * NPR, E, 128), bf16),
        vmem((NPR, SEG, 128), f32), vmem((3, H, RB, E), f32), vmem((3, H, SEG, E), f32),
        vmem((H, RB, E), f32), vmem((NG * NPR, SEG, E), f32), vmem((H, L, L), f32),
        vmem((NPR, L, 128), f32), vmem((NPR, SEG, 128), f32),
        vmem((RB, D), f32), vmem((S // 16, 16, D), bf16),
        pltpu.SemaphoreType.DMA((6,)), pltpu.SemaphoreType.DMA((8,)),
        pltpu.SemaphoreType.DMA((2,)), pltpu.SemaphoreType.DMA((3 * NG,)),
        pltpu.SemaphoreType.DMA((3,)),
    ]


@jax.jit
def pallas_concat_heads__spectral_gfnet__memory_aug_recurrent_mem_tr__prompt_kernel(
    A_x: jax.Array,
    A_w_r: jax.Array,
    A_w_i: jax.Array,
    B_x: jax.Array,
    B_mem0: jax.Array,
    B_Wq: jax.Array,
    B_Wk: jax.Array,
    B_Wv: jax.Array,
    B_Wo: jax.Array,
    B_seg_len: jax.Array,
):
    del B_seg_len
    hbm = pl.BlockSpec(memory_space=pl.ANY)
    out = pl.pallas_call(
        _kernel,
        out_shape=jax.ShapeDtypeStruct((S // 16, 16, 2 * D), bf16),
        in_specs=[hbm] * 11,
        out_specs=hbm,
        scratch_shapes=_scratch(),
        compiler_params=pltpu.CompilerParams(vmem_limit_bytes=120 * 2 ** 20),
    )(A_x.reshape(S // 16, 16, D), A_w_r.T, A_w_i.T, B_x.reshape(S, D), B_mem0.reshape(M, D),
      B_Wq, B_Wk, B_Wv, B_Wo.reshape(H * E, D), _DFT_ROWS, _DFT_TURNS)
    return out.reshape(1, S, 2 * D)
```
